```python
import jax
import jax.numpy as jnp

def _softmax(x, axis=-1):
    return jax.nn.softmax(x, axis=axis)

def _gelu(x):
    return jax.nn.gelu(x, approximate=True)

def _silu(x):
    return jax.nn.silu(x)

def _sigmoid(x):
    return jax.nn.sigmoid(x)

def _layernorm(x, axis=-1, eps=1e-05):
    m = jnp.mean(x, axis=axis, keepdims=True)
    v = jnp.var(x, axis=axis, keepdims=True)
    return (x - m) / jnp.sqrt(v + eps)

def _scatter_add(tgt, idx, src, axis=0):
    return tgt.at[idx].add(src)

def _segment_sum(src, seg, n):
    return jax.ops.segment_sum(src, seg, n)

class _Rng:

    def __init__(self, key):
        self._k = key

    def _next(self):
        self._k, sub = jax.random.split(self._k)
        return sub

    def normal(self, shape):
        return jax.random.normal(self._next(), shape, dtype=jnp.bfloat16)

    def randint(self, lo, hi, shape):
        return jax.random.randint(self._next(), shape, lo, hi, dtype=jnp.int32)

    def uniform(self, shape, lo=0.0, hi=1.0):
        return jax.random.uniform(self._next(), shape, jnp.bfloat16, lo, hi)

    def permutation(self, n):
        return jax.random.permutation(self._next(), n)
kernel_name = 'adaLN_cond__gqa_block_cached__moe_arch_mod__prompt'

def setup_inputs():
    _rng = _Rng(jax.random.key(int.from_bytes(__import__("os").urandom(4), "little")))
    _w = lambda a: (lambda t: t.astype(jnp.bfloat16) if jnp.issubdtype(t.dtype, jnp.floating) else t)(jnp.asarray(a))

    def _A_setup():
        B, Sq, D = (1, 2048, 576)
        Hq, Hkv, Sk, Dh = (32, 16, 2048, 128)
        assert Hq % Hkv == 0, (Hq, Hkv)
        return {'x': _w((lambda *s: _rng.normal(s) * 0.05)(B, Sq, D)), 'k_cache': _w((lambda *s: _rng.normal(s) * 0.05)(B, Hkv, Sk, Dh)), 'v_cache': _w((lambda *s: _rng.normal(s) * 0.05)(B, Hkv, Sk, Dh)), 'wq': _w((lambda *s: _rng.normal(s) * 0.05)(D, Hq * Dh) * D ** (-0.5)), 'wo': _w((lambda *s: _rng.normal(s) * 0.05)(Hq * Dh, D) * (Hq * Dh) ** (-0.5))}
    _A_in = _A_setup()

    def _B_setup():
        B, S, D, F, C = (1, 2048, 576, 4608, 8)
        return {'x': _w((lambda *s: _rng.normal(s) * 0.05)(B, S, D)), 'w_r': _w((lambda *s: _rng.normal(s) * 0.05)(D)), 'w_gate': _w((lambda *s: _rng.normal(s) * 0.05)(D, F)), 'w_up': _w((lambda *s: _rng.normal(s) * 0.05)(D, F)), 'w_down': _w((lambda *s: _rng.normal(s) * 0.05)(F, D))}
    _B_in = _B_setup()
    return {'A_x': _A_in['x'], 'A_k_cache': _A_in['k_cache'], 'A_v_cache': _A_in['v_cache'], 'A_wq': _A_in['wq'], 'A_wo': _A_in['wo'], 'B_x': _B_in['x'], 'B_w_r': _B_in['w_r'], 'B_w_gate': _B_in['w_gate'], 'B_w_up': _B_in['w_up'], 'B_w_down': _B_in['w_down'], 'c': _w((lambda *s: _rng.normal(s) * 0.05)(1, 576)), 'w_mod': _w((lambda *s: _rng.normal(s) * 0.05)(576, 6 * 576) * 576 ** (-0.5))}

def reference(A_x, A_k_cache, A_v_cache, A_wq, A_wo, B_x, B_w_r, B_w_gate, B_w_up, B_w_down, c, w_mod):

    def _A_ref(x, k_cache, v_cache, wq, wo):
        B, Sq, D = x.shape
        Hq, Dh = (32, 128)
        Hkv = k_cache.shape[1]
        rep = Hq // Hkv
        q = (lambda x, *d: x.transpose(*d))((x @ wq).reshape(B, Sq, Hq, Dh), 0, 2, 1, 3)
        k = jnp.repeat(k_cache, rep, axis=1)
        v = jnp.repeat(v_cache, rep, axis=1)
        scores = jnp.einsum('bhqd,bhkd->bhqk', q, k) * Dh ** (-0.5)
        p = _softmax(scores, axis=-1)
        o = jnp.einsum('bhqk,bhkd->bhqd', p, v)
        return (lambda x, *d: x.transpose(*d))(o, 0, 2, 1, 3).reshape(B, Sq, Hq * Dh) @ wo

    def _B_ref(x, w_r, w_gate, w_up, w_down):
        B, S, D = x.shape
        C = 8
        r = x @ w_r
        idx = jnp.argsort(-r, axis=-1)[:, :C]
        idx_e = jnp.repeat(idx.reshape(B, C, 1), D, axis=2)
        x_sel = jnp.take_along_axis(x, idx_e, axis=1)
        g = _silu(x_sel @ w_gate)
        u = x_sel @ w_up
        y = g * u @ w_down
        r_sel = _sigmoid(jnp.take_along_axis(r, idx, axis=1))
        y = y * r_sel.reshape(B, C, 1)
        b_off = (jnp.arange(B) * S).reshape(B, 1)
        flat_idx = (idx + b_off).reshape(B * C)
        zero = (x * 0.0).reshape(B * S, D)
        upd = _scatter_add(zero, flat_idx, y.reshape(B * C, D), axis=0)
        return x + upd.reshape(B, S, D)
    x = A_x
    mod = (_silu(c) @ w_mod).reshape(c.shape[0], 6, 1, -1)
    sa, ca, ga, sb, cb, gb = (mod[:, 0].copy(), mod[:, 1].copy(), mod[:, 2].copy(), mod[:, 3].copy(), mod[:, 4].copy(), mod[:, 5].copy())
    h = _layernorm(x, axis=-1) * (1 + ca) + sa
    x = x + ga * _A_ref(h, A_k_cache, A_v_cache, A_wq, A_wo)
    h = _layernorm(x, axis=-1) * (1 + cb) + sb
    x = x + gb * _B_ref(h, B_w_r, B_w_gate, B_w_up, B_w_down)
    return x
```

```python
import functools

import jax
import jax.numpy as jnp
import jax.experimental.pallas as pl
import jax.experimental.pallas.tpu as pltpu

HQ = 32
DH = 128
TOPC = 8
LN_EPS = 1e-05
LOG2E = 1.4426950408889634

F32 = jnp.float32
BF16 = jnp.bfloat16


def _rnd(v):
    return v.astype(BF16).astype(F32)


def _layernorm_mod(x, scale1p, shift):
    d = x.shape[-1]
    mean = jnp.sum(x, axis=-1, keepdims=True) * (1.0 / d)
    xc = x - mean
    var = jnp.sum(xc * xc, axis=-1, keepdims=True) * (1.0 / d)
    den = _rnd(jnp.sqrt(_rnd(_rnd(var) + LN_EPS)))
    y = _rnd(_rnd(x - _rnd(mean)) / den)
    return _rnd(_rnd(y * scale1p) + shift)


def _kernel(x_ref, k_ref, v_ref, wq_ref, wo_ref, wr_ref, c_ref, wmod_ref,
            wg_hbm, wu_hbm, wd_hbm,
            out_ref,
            h_scr, acc_scr, mod_scr, h2_scr, wg_v, wu_v, wd_v, sems,
            *, tq, n_groups, rep):
    g = pl.program_id(0)
    s_len, d = x_ref.shape
    n_tiles = s_len // tq

    def moe_copies():
        return (pltpu.make_async_copy(wg_hbm, wg_v, sems.at[0]),
                pltpu.make_async_copy(wu_hbm, wu_v, sems.at[1]),
                pltpu.make_async_copy(wd_hbm, wd_v, sems.at[2]))

    @pl.when(g == 0)
    def _prologue():
        for cp in moe_copies():
            cp.start()
        cf = c_ref[...].astype(F32)
        sc = (cf * jax.nn.sigmoid(cf)).astype(BF16)
        sc8 = jnp.broadcast_to(sc, (8, d))
        mod = _rnd(jnp.dot(sc8, wmod_ref[...], preferred_element_type=F32))
        for j in range(6):
            mod_scr[j] = mod[:, j * d:(j + 1) * d]
        sa = mod_scr[0][0:1]
        ca1 = _rnd(1.0 + mod_scr[1][0:1])

        def ln_body(t, carry):
            rows = pl.ds(pl.multiple_of(t * tq, tq), tq)
            xt = x_ref[rows, :].astype(F32)
            h_scr[rows, :] = _layernorm_mod(xt, ca1, sa).astype(BF16)
            acc_scr[rows, :] = jnp.zeros((tq, d), F32)
            return carry

        jax.lax.fori_loop(0, n_tiles, ln_body, 0)

    qscale = (DH ** -0.5) * LOG2E

    def attn_body(t, carry):
        rows = pl.ds(pl.multiple_of(t * tq, tq), tq)
        q = jnp.dot(h_scr[rows, :], wq_ref[...], preferred_element_type=F32)
        q = (q * qscale).astype(BF16)
        q2 = jnp.concatenate([q[:, r * DH:(r + 1) * DH] for r in range(rep)], axis=0)
        s = jax.lax.dot_general(q2, k_ref[...], (((1,), (1,)), ((), ())),
                                preferred_element_type=F32)
        m = jnp.max(s, axis=1, keepdims=True)
        p = jnp.exp2(s - m)
        l = jnp.sum(p, axis=1, keepdims=True)
        o = jnp.dot(p.astype(BF16), v_ref[...], preferred_element_type=F32)
        o = (o / l).astype(BF16)
        o2 = jnp.concatenate([o[r * tq:(r + 1) * tq] for r in range(rep)], axis=1)
        acc_scr[rows, :] += jnp.dot(o2, wo_ref[...], preferred_element_type=F32)
        return carry

    jax.lax.fori_loop(0, n_tiles, attn_body, 0)

    @pl.when(g == n_groups - 1)
    def _epilogue():
        ga = mod_scr[2][0:1]
        sb = mod_scr[3][0:1]
        cb1 = _rnd(1.0 + mod_scr[4][0:1])
        gb = mod_scr[5][0:1]

        def ln_body(t, carry):
            rows = pl.ds(pl.multiple_of(t * tq, tq), tq)
            xt = x_ref[rows, :].astype(F32)
            x1 = _rnd(xt + _rnd(ga * _rnd(acc_scr[rows, :])))
            h2 = _layernorm_mod(x1, cb1, sb)
            acc_scr[rows, :] = x1
            h2_scr[rows, :] = h2
            h_scr[rows, :] = h2.astype(BF16)
            out_ref[rows, :] = (x1 + _rnd(gb * h2)).astype(BF16)
            return carry

        jax.lax.fori_loop(0, n_tiles, ln_body, 0)

        wr8 = jnp.broadcast_to(wr_ref[...], (8, d))
        r = _rnd(jax.lax.dot_general(wr8, h_scr[...], (((1,), (1,)), ((), ())),
                                     preferred_element_type=F32))
        r = r[0:1]
        pos = jax.lax.broadcasted_iota(jnp.int32, r.shape, 1)
        idxs, vals = [], []
        taken = jnp.zeros(r.shape, jnp.int32)
        for _ in range(TOPC):
            live = jnp.where(taken > 0, -jnp.inf, r)
            mx = jnp.max(live, axis=1, keepdims=True)
            cand = jnp.where((live == mx) & (taken == 0), pos, s_len - 1)
            ix = jnp.min(cand)
            taken = jnp.where(pos == ix, 1, taken)
            idxs.append(ix)
            vals.append(mx)

        sub = jax.lax.broadcasted_iota(jnp.int32, (TOPC, d), 0)
        x_sel = jnp.zeros((TOPC, d), F32)
        x1_sel = jnp.zeros((TOPC, d), F32)
        r_sel = jnp.zeros((TOPC, 1), F32)
        for cidx in range(TOPC):
            row = pl.ds(idxs[cidx], 1)
            x_sel = jnp.where(sub == cidx, h2_scr[row, :], x_sel)
            x1_sel = jnp.where(sub == cidx, acc_scr[row, :], x1_sel)
            r_sel = jnp.where(sub[:, 0:1] == cidx, vals[cidx], r_sel)

        for cp in moe_copies():
            cp.wait()
        xs = x_sel.astype(BF16)
        gt = _rnd(jnp.dot(xs, wg_v[...], preferred_element_type=F32))
        gt = _rnd(gt * jax.nn.sigmoid(gt))
        up = _rnd(jnp.dot(xs, wu_v[...], preferred_element_type=F32))
        gu = (gt * up).astype(BF16)
        y = _rnd(jnp.dot(gu, wd_v[...], preferred_element_type=F32))
        y = _rnd(y * _rnd(jax.nn.sigmoid(r_sel)))
        new_rows = x1_sel + _rnd(gb * _rnd(x_sel + y))

        sub16 = jax.lax.broadcasted_iota(jnp.int32, (16, d), 0)
        for cidx in range(TOPC):
            base = pl.multiple_of((idxs[cidx] // 16) * 16, 16)
            blk = out_ref[pl.ds(base, 16), :].astype(F32)
            blk = jnp.where(sub16 == idxs[cidx] - base, new_rows[cidx:cidx + 1], blk)
            out_ref[pl.ds(base, 16), :] = blk.astype(BF16)


@jax.jit
def pallas_adaLN_cond__gqa_block_cached__moe_arch_mod__prompt_kernel(
    A_x: jax.Array,
    A_k_cache: jax.Array,
    A_v_cache: jax.Array,
    A_wq: jax.Array,
    A_wo: jax.Array,
    B_x: jax.Array,
    B_w_r: jax.Array,
    B_w_gate: jax.Array,
    B_w_up: jax.Array,
    B_w_down: jax.Array,
    c: jax.Array,
    w_mod: jax.Array,
):
    b, s_len, d = A_x.shape
    assert b == 1
    hkv, sk = A_k_cache.shape[1], A_k_cache.shape[2]
    rep = HQ // hkv
    f = B_w_gate.shape[1]
    tq = 256

    x2 = A_x.reshape(s_len, d)
    k3 = A_k_cache.reshape(hkv, sk, DH)
    v3 = A_v_cache.reshape(hkv, sk, DH)
    wr2 = B_w_r.reshape(1, d)

    const2 = lambda g: (0, 0)
    in_specs = [
        pl.BlockSpec((s_len, d), const2),
        pl.BlockSpec((None, sk, DH), lambda g: (g, 0, 0)),
        pl.BlockSpec((None, sk, DH), lambda g: (g, 0, 0)),
        pl.BlockSpec((d, rep * DH), lambda g: (0, g)),
        pl.BlockSpec((rep * DH, d), lambda g: (g, 0)),
        pl.BlockSpec((1, d), const2),
        pl.BlockSpec((1, d), const2),
        pl.BlockSpec((d, 6 * d), const2),
        pl.BlockSpec(memory_space=pl.ANY),
        pl.BlockSpec(memory_space=pl.ANY),
        pl.BlockSpec(memory_space=pl.ANY),
    ]
    scratch = [
        pltpu.VMEM((s_len, d), BF16),
        pltpu.VMEM((s_len, d), F32),
        pltpu.VMEM((6, 8, d), F32),
        pltpu.VMEM((s_len, d), F32),
        pltpu.VMEM((d, f), BF16),
        pltpu.VMEM((d, f), BF16),
        pltpu.VMEM((f, d), BF16),
        pltpu.SemaphoreType.DMA((3,)),
    ]
    out = pl.pallas_call(
        functools.partial(_kernel, tq=tq, n_groups=hkv, rep=rep),
        grid=(hkv,),
        in_specs=in_specs,
        out_specs=pl.BlockSpec((s_len, d), const2),
        out_shape=jax.ShapeDtypeStruct((s_len, d), BF16),
        scratch_shapes=scratch,
        compiler_params=pltpu.CompilerParams(
            dimension_semantics=("arbitrary",),
            vmem_limit_bytes=100 * 1024 * 1024,
        ),
    )(x2, k3, v3, A_wq, A_wo, wr2, c, w_mod, B_w_gate, B_w_up, B_w_down)
    return out.reshape(b, s_len, d)
```

```python
import functools

import jax
import jax.numpy as jnp
import jax.experimental.pallas as pl
import jax.experimental.pallas.tpu as pltpu

HQ = 32
DH = 128
TOPC = 8
LN_EPS = 1e-05
LOG2E = 1.4426950408889634
F32 = jnp.float32
BF16 = jnp.bfloat16
NT = (((1,), (1,)), ((), ()))


def _rnd(v):
    return v.astype(BF16).astype(F32)


def _normalize_t(xt):
    d = xt.shape[0]
    mean = jnp.sum(xt, axis=0, keepdims=True) * (1.0 / d)
    xc = xt - mean
    var = jnp.sum(xc * xc, axis=0, keepdims=True) * (1.0 / d)
    den = _rnd(jnp.sqrt(_rnd(_rnd(var) + LN_EPS)))
    return _rnd(_rnd(xt - _rnd(mean)) / den)


def _kernel(xt_ref, k_ref, v_ref, wq_ref, wot_ref, wr_ref, c_ref, wmod_ref,
            wg_hbm, wu_hbm, wdt_hbm,
            out_ref,
            h_scr, acc_scr, col_scr, gb_scr, vt_scr, h2_scr, r_scr, wg_v, wu_v, wdt_v, s0_scr, s1_scr, z_scr, sems,
            *, tq, kq, ahead, order, qh, oh, lw, ki, n_groups, rep, tl, kc):
    g = pl.program_id(0)
    s_bufs = (s0_scr, s1_scr)
    d, s_len = xt_ref.shape
    n_tiles = s_len // tq

    def moe_copies():
        return (pltpu.make_async_copy(wg_hbm, wg_v, sems.at[0]),
                pltpu.make_async_copy(wu_hbm, wu_v, sems.at[1]),
                pltpu.make_async_copy(wdt_hbm, wdt_v, sems.at[2]))

    @pl.when(g == 0)
    def _prologue():
        for cp in moe_copies():
            cp.start()
        for i in range(8):
            z_scr[i] = 0
        cf = c_ref[...].astype(F32)
        sc = (cf * jax.nn.sigmoid(cf)).astype(BF16)
        sc8 = jnp.broadcast_to(sc, (8, d))
        mod = _rnd(jnp.dot(sc8, wmod_ref[...], preferred_element_type=F32))
        piece = lambda j: mod[0:1, j * d:(j + 1) * d]
        sa = piece(0)
        ca1 = _rnd(1.0 + piece(1))
        gb_scr[...] = jnp.broadcast_to(piece(5), (8, d))
        rows = [piece(2), piece(3), _rnd(1.0 + piece(4)), piece(5), wr_ref[...].astype(F32)]
        for j, row in enumerate(rows):
            col_scr[j] = jnp.broadcast_to(row, (128, d)).T

        def ln_body(t, carry):
            off = pl.multiple_of(t * tl, tl)
            y = _normalize_t(xt_ref[:, pl.ds(off, tl)].astype(F32)).T
            h_scr[pl.ds(off, tl), :] = (_rnd(y * ca1) + sa).astype(BF16)
            acc_scr[:, pl.ds(off, tl)] = jnp.zeros((d, tl), F32)
            return carry

        jax.lax.fori_loop(0, s_len // tl, ln_body, 0)

    qscale = (DH ** -0.5) * LOG2E
    sk = k_ref.shape[0]
    tg = 512 // rep
    nu = 4
    nc = sk // kc
    nq = sk // kq

    if n_tiles > 1:
        vt_scr[...] = v_ref[...].T

    def attn_body(t, carry):
        off = pl.multiple_of(t * tq, tq) if n_tiles > 1 else 0
        if n_tiles == 1:
            vt_scr[...] = v_ref[...].T
        zero = z_scr[0]
        zvec = jnp.full((8, 128), zero, jnp.int32)
        ng = tq // tg
        clock = [0]
        hist = []

        def step(result, nrows):
            hist.append((clock[0], nrows, result))
            clock[0] += nrows

        def after(x, ahead):
            want = clock[0] - ahead - 128
            for start, nrows, res in reversed(hist):
                if start <= want:
                    row = min((want - start) * res.shape[0] // nrows // 8 * 8, res.shape[0] - 8)
                    bits = pltpu.bitcast(res[row:row + 8, 0:128], jnp.int32) & zvec
                    return pltpu.bitcast(pltpu.bitcast(x, jnp.int32) | bits, F32)
            return x

        def tok_rows(i, lo, n):
            if n_tiles == 1:
                return pl.ds(i * tg + lo, n)
            return pl.ds(pl.multiple_of(off + i * tg + lo, n), n)

        def qproj(i):
            parts = []
            for hb in range(tg // qh):
                q = jnp.dot(h_scr[tok_rows(i, hb * qh, qh), :], wq_ref[...],
                            preferred_element_type=F32)
                step(q, qh * 10 // 4)
                parts.append((q * qscale).astype(BF16))
            return jnp.concatenate([p[:, r * DH:(r + 1) * DH] for r in range(rep) for p in parts],
                                   axis=0)

        def qk_chunk(qg, buf, j, m, cols=slice(0, 512), adv=True, kq=kq):
            st = jax.lax.dot_general(k_ref[j * kq:(j + 1) * kq, :], qg[cols], NT,
                                     preferred_element_type=F32)
            s_bufs[buf][zero, j * kq:(j + 1) * kq, cols] = st
            step(st, kq)
            if not adv:
                clock[0] -= kq
            mj = jnp.max(st.reshape(kq // 8, 8, st.shape[1]), axis=0)
            return mj if m is None else jnp.maximum(m, mj)

        def max_fin(m):
            return jnp.broadcast_to(jnp.max(m, axis=0, keepdims=True), m.shape)

        def qk(qg, buf):
            m = None
            for j in range(nq):
                m = qk_chunk(qg, buf, j, m)
            return max_fin(m)

        def pv_step(buf, m, u, j, st8, kc=kc, dur=None):
            cs = slice(u * 128, (u + 1) * 128)
            mu = after(m[:, cs], ahead)
            sj = s_bufs[buf][0, j * kc:(j + 1) * kc, cs].reshape(kc // 8, 8, 128)
            p = jnp.exp2(sj - mu[None])
            lj = jnp.sum(p.reshape(kc // lw, lw, 128), axis=0)
            oj = jnp.dot(vt_scr[:, j * kc:(j + 1) * kc], p.reshape(kc, 128).astype(BF16),
                         preferred_element_type=F32)
            step(oj, dur or kc // 4)
            return (oj, lj) if st8 is None else (st8[0] + oj, st8[1] + lj)

        def pv_fin(st8):
            return (st8[0] / jnp.sum(st8[1], axis=0, keepdims=True)).astype(BF16)

        def gather_out(outs):
            per = nu // rep
            return jnp.concatenate(
                [jnp.concatenate(outs[r * per:(r + 1) * per], axis=1) for r in range(rep)], axis=0)

        def pv(buf, m):
            outs = []
            for u in range(nu):
                st8 = None
                for j in range(nc):
                    st8 = pv_step(buf, m, u, j, st8)
                outs.append(pv_fin(st8))
            return gather_out(outs)

        def pv_qk_mixed(buf, m, qn, nbuf):
            outs, mn, n, jq = [], None, 0, 0
            nqi = sk // ki
            every = nu * nc // nqi
            for u in range(nu):
                st8 = None
                for j in range(nc):
                    if n % every == 0:
                        mn = qk_chunk(qn, nbuf, jq, mn, kq=ki)
                        jq += 1
                    st8 = pv_step(buf, m, u, j, st8)
                    n += 1
                outs.append(pv_fin(st8))
            return gather_out(outs), max_fin(mn)

        def pv_qk_split(buf, m, qn, nbuf):
            outs, mns = [], []
            for half in range(2):
                mns.append(qk_chunk(qn, nbuf, 0, None, cols=slice(half * 256, (half + 1) * 256),
                                    adv=False, kq=sk))
                for u in range(2 * half, 2 * half + 2):
                    st8 = None
                    for j in range(sk // 256):
                        st8 = pv_step(buf, m, u, j, st8, kc=256, dur=128)
                    outs.append(pv_fin(st8))
            return gather_out(outs), max_fin(jnp.concatenate(mns, axis=1))

        def oproj(i, ot):
            cols = tok_rows(i, 0, tg)
            for rb in range(d // oh):
                rows = slice(rb * oh, (rb + 1) * oh)
                res = jnp.dot(wot_ref[rows, :], ot, preferred_element_type=F32)
                step(res, oh)
                acc_scr[rows, cols] += res

        qs, ots, ms = {}, {}, {}
        qs[0] = qproj(0)
        qs[1] = qproj(1)
        if order == 0:
            for i in range(ng):
                m = qk(qs[i], i % 2)
                if i >= 2:
                    oproj(i - 2, ots[i - 2])
                if i + 2 < ng:
                    qs[i + 2] = qproj(i + 2)
                ots[i] = pv(i % 2, m)
        elif order in (2, 3):
            fn = pv_qk_mixed if order == 2 else pv_qk_split
            ms[0] = qk(qs[0], 0)
            for i in range(ng):
                if i >= 2:
                    oproj(i - 2, ots[i - 2])
                if i + 2 < ng:
                    qs[i + 2] = qproj(i + 2)
                if i + 1 < ng:
                    ots[i], ms[i + 1] = fn(i % 2, ms[i], qs[i + 1], (i + 1) % 2)
                else:
                    ots[i] = pv(i % 2, ms[i])
        else:
            ms[0] = qk(qs[0], 0)
            for i in range(ng):
                if i + 1 < ng:
                    ms[i + 1] = qk(qs[i + 1], (i + 1) % 2)
                if i >= 2:
                    oproj(i - 2, ots[i - 2])
                if i + 2 < ng:
                    qs[i + 2] = qproj(i + 2)
                ots[i] = pv(i % 2, ms[i])
        oproj(ng - 2, ots[ng - 2])
        oproj(ng - 1, ots[ng - 1])
        return carry

    if n_tiles == 1:
        attn_body(0, 0)
    else:
        jax.lax.fori_loop(0, n_tiles, attn_body, 0)

    @pl.when(g == n_groups - 1)
    def _epilogue():
        def ln_body(t, carry):
            cols = pl.ds(pl.multiple_of(t * 128, 128), 128)
            xt = xt_ref[:, cols].astype(F32)
            x1 = _rnd(xt + _rnd(col_scr[0] * _rnd(acc_scr[:, cols])))
            h2 = _rnd(_rnd(_normalize_t(x1) * col_scr[2]) + col_scr[1])
            acc_scr[:, cols] = x1
            h2_scr[:, cols] = h2.astype(BF16)
            r_scr[:, cols] = jnp.sum(h2 * col_scr[4], axis=0, keepdims=True)
            return carry

        jax.lax.fori_loop(0, s_len // 128, ln_body, 0)

        r = _rnd(r_scr[...])
        pos = jax.lax.broadcasted_iota(jnp.int32, r.shape, 1)
        sub = jax.lax.broadcasted_iota(jnp.int32, (TOPC, s_len), 0)
        sub1 = jax.lax.broadcasted_iota(jnp.int32, (TOPC, 1), 0)
        taken = jnp.zeros(r.shape, jnp.int32)
        onehot = jnp.zeros((TOPC, s_len), F32)
        r_sel = jnp.zeros((TOPC, 1), F32)
        for cidx in range(TOPC):
            live = jnp.where(taken > 0, -jnp.inf, r)
            mx = jnp.max(live, axis=1, keepdims=True)
            cand = jnp.where((live == mx) & (taken == 0), pos, s_len - 1)
            ix = jnp.min(cand, axis=1, keepdims=True)
            hit = pos == ix
            taken = jnp.where(hit, 1, taken)
            onehot = jnp.where(hit & (sub == cidx), 1.0, onehot)
            r_sel = jnp.where(sub1 == cidx, mx, r_sel)
        oh = onehot.astype(BF16)
        x_sel = jax.lax.dot_general(oh, h2_scr[...], NT, preferred_element_type=F32)

        for cp in moe_copies():
            cp.wait()
        xs = x_sel.astype(BF16)
        gt = _rnd(jnp.dot(xs, wg_v[...], preferred_element_type=F32))
        gt = _rnd(gt * jax.nn.sigmoid(gt))
        up = _rnd(jnp.dot(xs, wu_v[...], preferred_element_type=F32))
        gu = (gt * up).astype(BF16)
        y = _rnd(jax.lax.dot_general(gu, wdt_v[...], NT, preferred_element_type=F32))
        y = (y * _rnd(jax.nn.sigmoid(r_sel))).astype(BF16)
        ypad = jnp.concatenate([y.astype(F32), jnp.zeros((128 - TOPC, d), F32)], axis=0)
        yt = ypad.T.astype(BF16)
        ohpad = jnp.concatenate([onehot, jnp.zeros((128 - TOPC, s_len), F32)], axis=0).astype(BF16)

        for t in range(s_len // 128):
            cols = slice(t * 128, (t + 1) * 128)
            upd = jnp.dot(yt, ohpad[:, cols], preferred_element_type=F32)
            hb = _rnd(h2_scr[:, cols].astype(F32) + upd)
            out_ref[:, cols] = (acc_scr[:, cols] + _rnd(col_scr[3] * hb)).astype(BF16)


def build(tq=2048, kq=512, ahead=384, order=3, qh=128, oh=144, tl=256, kc=512, lw=32, ki=128):
    gw = 512
    @jax.jit
    def fn(A_x, A_k_cache, A_v_cache, A_wq, A_wo, B_x, B_w_r, B_w_gate, B_w_up, B_w_down, c, w_mod):
        b, s_len, d = A_x.shape
        hkv, sk = A_k_cache.shape[1], A_k_cache.shape[2]
        rep = HQ // hkv
        f = B_w_gate.shape[1]
        xt = A_x.reshape(s_len, d).T
        k3 = A_k_cache.reshape(hkv, sk, DH)
        v3 = A_v_cache.reshape(hkv, sk, DH)
        wr2 = B_w_r.reshape(1, d)
        const2 = lambda g: (0, 0)
        in_specs = [
            pl.BlockSpec((d, s_len), const2),
            pl.BlockSpec((None, sk, DH), lambda g: (g, 0, 0)),
            pl.BlockSpec((None, sk, DH), lambda g: (g, 0, 0)),
            pl.BlockSpec((d, rep * DH), lambda g: (0, g)),
            pl.BlockSpec((d, rep * DH), lambda g: (0, g)),
            pl.BlockSpec((1, d), const2),
            pl.BlockSpec((1, d), const2),
            pl.BlockSpec((d, 6 * d), const2),
            pl.BlockSpec(memory_space=pl.ANY),
            pl.BlockSpec(memory_space=pl.ANY),
            pl.BlockSpec(memory_space=pl.ANY),
        ]
        scratch = [
            pltpu.VMEM((s_len, d), BF16),
            pltpu.VMEM((d, s_len), F32),
            pltpu.VMEM((5, d, 128), F32),
            pltpu.VMEM((8, d), F32),
            pltpu.VMEM((DH, sk), BF16),
            pltpu.VMEM((d, s_len), BF16),
            pltpu.VMEM((1, s_len), F32),
            pltpu.VMEM((d, f), BF16),
            pltpu.VMEM((d, f), BF16),
            pltpu.VMEM((d, f), BF16),
            pltpu.VMEM((1, sk, gw), F32),
            pltpu.VMEM((1, sk, gw), F32),
            pltpu.SMEM((8,), jnp.int32),
            pltpu.SemaphoreType.DMA((3,)),
        ]
        out = pl.pallas_call(
            functools.partial(_kernel, tq=tq, kq=kq, ahead=ahead, order=order, qh=qh, oh=oh, lw=lw, ki=ki, n_groups=hkv, rep=rep, tl=tl, kc=kc),
            grid=(hkv,),
            in_specs=in_specs,
            out_specs=pl.BlockSpec((d, s_len), const2),
            out_shape=jax.ShapeDtypeStruct((d, s_len), BF16),
            scratch_shapes=scratch,
            compiler_params=pltpu.CompilerParams(
                dimension_semantics=("arbitrary",),
                vmem_limit_bytes=100 * 1024 * 1024,
            ),
        )(xt, k3, v3, A_wq, A_wo.T, wr2, c, w_mod, B_w_gate, B_w_up, B_w_down.T)
        return out.T.reshape(b, s_len, d)
    return fn


pallas_adaLN_cond__gqa_block_cached__moe_arch_mod__prompt_kernel = build()
```

```python
import contextlib
import functools

import jax
import jax.numpy as jnp
import jax.experimental.pallas as pl
import jax.experimental.pallas.tpu as pltpu

HQ = 32
DH = 128
TOPC = 8
LN_EPS = 1e-05
LOG2E = 1.4426950408889634
F32 = jnp.float32
BF16 = jnp.bfloat16
I32 = jnp.int32
NT = (((1,), (1,)), ((), ()))
LANES = 128
GW = 512


def _rnd(v):
    return v.astype(BF16).astype(F32)


def _fold8(v):
    return jnp.sum(v.reshape(v.shape[0] // 8, 8, v.shape[1]), axis=0)


def _ln_stats(shift, s1, s2, d):
    e1 = jnp.sum(s1, axis=0, keepdims=True) * (1.0 / d)
    e2 = jnp.sum(s2, axis=0, keepdims=True) * (1.0 / d)
    var = jnp.maximum(e2 - e1 * e1, 0.0)
    den = _rnd(jnp.sqrt(_rnd(_rnd(var) + LN_EPS)))
    return _rnd(shift + e1), 1.0 / den


def _kernel(xt_hbm, k_hbm, v_hbm, wq_hbm, wot_hbm, wr_hbm, c_hbm, wmod_hbm,
            wg_hbm, wu_hbm, wdt_hbm,
            out_hbm,
            xt_v, kbuf, vbuf, wqbuf, wobuf, wr_v, c_v, wmod_v, wg_v, wu_v, wdt_v, out_v,
            h_scr, acc_scr, row_scr, col_scr, vt_scr, xh_scr, r_scr, st_scr, s0_scr, s1_scr, z_scr,
            gsem, msem, osem, xsem,
            *, n_groups, rep, ahead, qh, oh, lw, x0, prof, mid, lb, l1, rch, pm, gl):
    _, d, s_len = xt_v.shape
    sk = kbuf.shape[1]
    gcols = rep * DH
    tg = GW // rep
    ng = s_len // tg
    nblk = s_len // LANES
    s_bufs = (s0_scr, s1_scr)
    qscale = (DH ** -0.5) * LOG2E

    def group_copies(g, slot):
        cols = pl.ds(pl.multiple_of(g * gcols, gcols), gcols)
        return (pltpu.make_async_copy(wq_hbm.at[:, cols], wqbuf.at[slot], gsem.at[slot, 0]),
                pltpu.make_async_copy(k_hbm.at[g], kbuf.at[slot], gsem.at[slot, 1]),
                pltpu.make_async_copy(v_hbm.at[g], vbuf.at[slot], gsem.at[slot, 2]),
                pltpu.make_async_copy(wot_hbm.at[:, cols], wobuf.at[slot], gsem.at[slot, 3]))

    cp_c = pltpu.make_async_copy(c_hbm, c_v, msem.at[0])
    cp_wr = pltpu.make_async_copy(wr_hbm, wr_v, msem.at[1])
    cp_m0 = pltpu.make_async_copy(wmod_hbm.at[:, 0:2 * d], wmod_v.at[:, 0:2 * d], msem.at[4])
    cp_m1 = pltpu.make_async_copy(wmod_hbm.at[:, 2 * d:6 * d], wmod_v.at[:, 2 * d:6 * d], msem.at[5])
    cp_moe = (pltpu.make_async_copy(wg_hbm, wg_v, msem.at[6]),
              pltpu.make_async_copy(wu_hbm, wu_v, msem.at[7]),
              pltpu.make_async_copy(wdt_hbm, wdt_v, msem.at[8]))

    def out_copy(b):
        cols = slice(b * LANES, (b + 1) * LANES)
        return pltpu.make_async_copy(out_v.at[0, :, cols], out_hbm.at[:, cols], osem.at[b])

    def silu_c8():
        cf = c_v[...].astype(F32)
        sc = (cf * jax.nn.sigmoid(cf)).astype(BF16)
        return jnp.broadcast_to(sc, (8, d))

    def moments(chunk_fn):
        shift = s1 = s2 = None
        for rc in range(d // rch):
            v = chunk_fn(slice(rc * rch, (rc + 1) * rch))
            if shift is None:
                shift = v[0:1]
            dv = v - shift
            a, b = _fold8(dv), _fold8(dv * dv)
            s1, s2 = (a, b) if s1 is None else (s1 + a, s2 + b)
        return _ln_stats(shift, s1, s2, d)

    def ln1_norm(lo, n):
        mean, rinv = moments(lambda rows: xt_v[0, rows, lo:lo + n].astype(F32))
        z = z_scr[0]
        return ((xt_v[z, :, lo:lo + n].astype(F32) - mean) * rinv).astype(BF16).T

    def ln1_mod(lo, n, y):
        h = y.astype(F32) * row_scr[1][0:1] + row_scr[0][0:1]
        h_scr[lo:lo + n, :] = h.astype(BF16)

    def ln2_pass_a(b):
        nb = lb // LANES
        cols = pl.ds(pl.multiple_of(b * lb, lb), lb)

        def chunk(rows):
            ga = jnp.concatenate([col_scr[0, rows, :]] * nb, axis=1)
            x1b = (xt_v[0, rows, cols].astype(F32) + ga * acc_scr[rows, cols]).astype(BF16)
            xh_scr[0, pl.ds(d + rows.start, rch), cols] = x1b
            return x1b.astype(F32)

        mean, rinv = moments(chunk)
        st_scr[0, :, cols] = jnp.broadcast_to(mean, (8, lb))
        st_scr[1, :, cols] = jnp.broadcast_to(rinv, (8, lb))

    def ln2_pass_c(b):
        nb = lb // LANES
        cols = pl.ds(pl.multiple_of(b * lb, lb), lb)
        mean, rinv = st_scr[0, 0:1, cols], st_scr[1, 0:1, cols]
        racc = None
        for rc in range(d // rch):
            rows = slice(rc * rch, (rc + 1) * rch)
            col = lambda j: jnp.concatenate([col_scr[j, rows, :]] * nb, axis=1)
            x1 = xh_scr[0, pl.ds(d + rows.start, rch), cols].astype(F32)
            y = _rnd(_rnd(x1 - mean) * rinv)
            h2b = (_rnd(y * col(2)) + col(1)).astype(BF16)
            h2 = h2b.astype(F32)
            xh_scr[0, rows, cols] = h2b
            part = _fold8(h2 * col(4))
            racc = part if racc is None else racc + part
        r = jnp.sum(racc, axis=0, keepdims=True)
        for j in range(nb):
            r_scr[pl.ds(b * nb + j, 1), :] = r[:, j * LANES:(j + 1) * LANES]

    def attn_group(slot, first, last, barrier=None):
        k_ref, v_ref = kbuf.at[slot], vbuf.at[slot]
        wq_ref, wot_ref = wqbuf.at[slot], wobuf.at[slot]
        zero = z_scr[0]
        zvec = jnp.full((8, LANES), zero, I32)
        clock = [0]
        hist = []

        def step(result, dur, adv=True):
            hist.append((clock[0], dur, result))
            if adv:
                clock[0] += dur

        def after(x):
            want = clock[0] - ahead - 128
            for start, dur, res in reversed(hist):
                if start <= want:
                    row = min((want - start) * res.shape[0] // dur // 8 * 8, res.shape[0] - 8)
                    bits = pltpu.bitcast(res[row:row + 8, 0:LANES], I32) & zvec
                    return pltpu.bitcast(pltpu.bitcast(x, I32) | bits, F32)
            return x

        def qproj(i):
            parts = []
            for hb in range(tg // qh):
                lo = i * tg + hb * qh
                q = jnp.dot(h_scr[lo:lo + qh, :], wq_ref[...], preferred_element_type=F32)
                step(q, qh * 10 // 4)
                parts.append((q * qscale).astype(BF16))
            return jnp.concatenate([p[:, r * DH:(r + 1) * DH] for r in range(rep) for p in parts],
                                   axis=0)

        def qk_part(qg, buf, rows, cols, adv):
            st = jax.lax.dot_general(k_ref[rows, :], qg[cols], NT, preferred_element_type=F32)
            s_bufs[buf][zero, rows, cols] = st
            step(st, st.shape[0], adv)
            return jnp.max(st.reshape(st.shape[0] // 8, 8, st.shape[1]), axis=0)

        def max_fin(m):
            return jnp.broadcast_to(jnp.max(m, axis=0, keepdims=True), m.shape)

        def qk(qg, buf):
            m = None
            for j in range(4):
                mj = qk_part(qg, buf, slice(j * sk // 4, (j + 1) * sk // 4), slice(0, GW), True)
                m = mj if m is None else jnp.maximum(m, mj)
            return max_fin(m)

        def pv_unit(buf, m, u, kc):
            cs = slice(u * LANES, (u + 1) * LANES)
            o = l = None
            for j in range(sk // kc):
                mu = after(m[:, cs])
                sj = s_bufs[buf][0, j * kc:(j + 1) * kc, cs].reshape(kc // 8, 8, LANES)
                p = jnp.exp2(sj - mu[None])
                lj = jnp.sum(p.reshape(kc // lw, lw, LANES), axis=0)
                oj = jnp.dot(vt_scr[:, j * kc:(j + 1) * kc], p.reshape(kc, LANES).astype(BF16),
                             preferred_element_type=F32)
                step(oj, DH)
                o = oj if o is None else o + oj
                l = lj if l is None else l + lj
            return (o / jnp.sum(l, axis=0, keepdims=True)).astype(BF16)

        def gather_out(outs):
            per = 4 // rep
            return jnp.concatenate(
                [jnp.concatenate(outs[r * per:(r + 1) * per], axis=1) for r in range(rep)], axis=0)

        def pv(buf, m):
            return gather_out([pv_unit(buf, m, u, 512) for u in range(4)])

        def pv_qk(buf, m, qn, nbuf):
            outs, mns = [], []
            for half in range(2):
                mns.append(qk_part(qn, nbuf, slice(0, sk), slice(half * 256, (half + 1) * 256), False))
                outs += [pv_unit(buf, m, u, 256) for u in (2 * half, 2 * half + 1)]
            return gather_out(outs), max_fin(jnp.concatenate(mns, axis=1))

        def oproj(i, ot):
            cols = slice(i * tg, (i + 1) * tg)
            parts = []
            for rb in range(d // oh):
                rows = slice(rb * oh, (rb + 1) * oh)
                res = jnp.dot(wot_ref[rows, :], ot, preferred_element_type=F32)
                step(res, oh)
                if not first:
                    res = res + acc_scr[rows, cols]
                if last:
                    parts.append(res)
                else:
                    acc_scr[rows, cols] = res
            if last:
                attn = jnp.concatenate(parts, axis=0)
                for bb in range(tg // LANES):
                    ln2_block(i * tg // LANES + bb, attn[:, bb * LANES:(bb + 1) * LANES])

        qs, ots, ms = {}, {}, {}
        if barrier is None:
            vt_scr[...] = v_ref[...].T
        qs[0] = qproj(0)
        qs[1] = qproj(1)
        ms[0] = qk(qs[0], 0)
        if barrier is not None:
            barrier()
            hist.clear()
            vt_scr[...] = v_ref[...].T
        for i in range(ng):
            if i >= 2:
                oproj(i - 2, ots[i - 2])
            if i + 2 < ng:
                qs[i + 2] = qproj(i + 2)
            if i + 1 < ng:
                ots[i], ms[i + 1] = pv_qk(i % 2, ms[i], qs[i + 1], (i + 1) % 2)
            else:
                ots[i] = pv(i % 2, ms[i])
        oproj(ng - 2, ots[ng - 2])
        oproj(ng - 1, ots[ng - 1])

    es = contextlib.ExitStack()
    def scope(name):
        es.close()
        if prof:
            es.enter_context(jax.named_scope(name))

    scope('p0_start')
    g0 = group_copies(0, 0)
    nxc = s_len // x0
    cp_x = [pltpu.make_async_copy(xt_hbm.at[:, j * x0:(j + 1) * x0], xt_v.at[0, :, j * x0:(j + 1) * x0],
                                  xsem.at[j]) for j in range(nxc)]
    cp_c.start()
    cp_m0.start()
    cp_x[0].start()
    cp_wr.start()
    for i in range(z_scr.shape[0]):
        z_scr[i] = 0
    acc_scr[...] = jnp.zeros(acc_scr.shape, F32)
    per = x0 // l1
    scope('p1_waitx0')
    cp_x[0].wait()
    cp_x[1].start()
    cp_x[2].start()
    scope('p1_norm0')
    ys = [ln1_norm(i * l1, l1) for i in range(per)]
    scope('p1_waitmod')
    cp_c.wait()
    cp_m0.wait()
    cp_x[3].start()
    scope('p2_mod')
    mod = _rnd(jnp.dot(silu_c8(), wmod_v[:, 0:2 * d], preferred_element_type=F32))
    row_scr[0] = mod[:, 0:d]
    row_scr[1] = _rnd(1.0 + mod[:, d:2 * d])
    for i in range(per):
        ln1_mod(i * l1, l1, ys[i])
    for j in range(1, nxc):
        scope('p3_waitx%d' % j)
        cp_x[j].wait()
        if j <= 2:
            g0[2 * j - 2].start()
            g0[2 * j - 1].start()
        scope('p4_ln%d' % j)
        for i in range(j * per, (j + 1) * per):
            ln1_mod(i * l1, l1, ln1_norm(i * l1, l1))

    def mid_body(g, carry):
        slot = g % 2
        for cp in group_copies(g, slot):
            cp.wait()

        @pl.when(g + 1 < n_run)
        def _():
            for cp in group_copies(g + 1, 1 - slot):
                cp.start()

        @pl.when(g == 0)
        def _():
            cp_m1.start()
            for cp in cp_moe:
                cp.start()

        if mid:
            attn_group(slot, False, False)
        else:
            acc_scr[0:16, 0:512] += h_scr[pl.ds(pl.multiple_of(z_scr[0] * 16, 16), 16), 0:512].astype(F32)
        return carry

    n_run = n_groups if mid else 2
    scope('q_loop')
    jax.lax.fori_loop(0, n_run, mid_body, 0)

    scope('r0_mod2')
    cp_m1.wait()
    cp_wr.wait()
    for cp in cp_moe:
        cp.wait()
    mod = _rnd(jnp.dot(silu_c8(), wmod_v[:, 2 * d:6 * d], preferred_element_type=F32))
    piece = lambda j: mod[0:1, j * d:(j + 1) * d]
    rows = [piece(0), piece(1), _rnd(1.0 + piece(2)), piece(3), wr_v[...].astype(F32)]
    for j, row in enumerate(rows):
        col_scr[j] = jnp.broadcast_to(row, (LANES, d)).T
    row_scr[2] = mod[:, 3 * d:4 * d]

    scope('r1_ln2a')
    jax.lax.fori_loop(0, s_len // lb, lambda b, c: (ln2_pass_a(b), c)[1], 0)
    scope('r1_ln2c')
    jax.lax.fori_loop(0, s_len // lb, lambda b, c: (ln2_pass_c(b), c)[1], 0)
    scope('r2_topk')

    zero = z_scr[0]
    zvec = jnp.full((8, LANES), zero, I32)
    ow = s_len // TOPC

    def out_piece(b, zg):
        cols = slice(b * ow, (b + 1) * ow)
        for rc in range(d // rch):
            rows = slice(rc * rch, (rc + 1) * rch)
            gb = jnp.concatenate([col_scr[3 + zg, rows, :]] * (ow // LANES), axis=1)
            x1 = xh_scr[zg, d + rc * rch:d + (rc + 1) * rch, cols].astype(F32)
            out_v[0, rows, cols] = (x1 + gb * xh_scr[zg, rows, cols].astype(F32)).astype(BF16)
        return pltpu.bitcast(out_v[zero, 0:16, 0:LANES], I32) & zvec

    ibits = (s_len - 1).bit_length()
    imask = (1 << ibits) - 1
    bits = pltpu.bitcast(_rnd(r_scr[...]), I32)
    pos = (jax.lax.broadcasted_iota(I32, bits.shape, 0) * LANES
           + jax.lax.broadcasted_iota(I32, bits.shape, 1))
    order = ((bits ^ ((bits >> 31) & 0x7FFFFFFF)) >> 16) + 0x8000
    key = pltpu.bitcast((order << ibits) + (imask - pos) + 0x20000000, F32)
    sub = jax.lax.broadcasted_iota(I32, (TOPC, LANES), 0)
    lane = jax.lax.broadcasted_iota(I32, (TOPC, LANES), 1)
    idxs, blks = [], []
    keyv = jnp.zeros((TOPC, LANES), I32)
    xh_sel = jnp.zeros((TOPC, 2 * d), F32)
    for cidx in range(TOPC):
        top = jnp.max(jnp.max(key, axis=0, keepdims=True), axis=1, keepdims=True)
        topi = pltpu.bitcast(jnp.broadcast_to(top, (TOPC, LANES)), I32) | out_piece(cidx, zero & (idxs[cidx - gl] if cidx >= gl else cidx))
        key = jnp.where(key == pltpu.bitcast(topi, F32)[0:1], 0.0, key)
        keyv = jnp.where(sub == cidx, topi, keyv)
        ixv = imask - (topi & imask)
        ix = ixv[0, 0]
        idxs.append(ix)
        blks.append(ix >> 7)
        cols = pl.ds(pl.multiple_of(blks[cidx] * LANES, LANES), LANES)
        oh1 = jnp.where((lane == (ixv & (LANES - 1))) & (sub == cidx), 1.0, 0.0).astype(BF16)
        xh_sel = xh_sel + jax.lax.dot_general(oh1, xh_scr[0, :, cols], NT, preferred_element_type=F32)

    for b in range(nblk):
        hit = blks[0] == b
        for bb in blks[1:]:
            hit = jnp.logical_or(hit, bb == b)

        @pl.when(jnp.logical_not(hit))
        def _(b=b):
            out_copy(b).start()

    scope('r4_moe')
    x_sel = xh_sel[:, 0:d]
    x1_sel = xh_sel[:, d:2 * d]
    ob = (((keyv - 0x20000000) >> ibits) - 0x8000) << 16
    r_sel = pltpu.bitcast((ob ^ ((ob >> 31) & 0x7FFFFFFF)) & ~0xFFFF, F32)[:, 0:1]
    xs = x_sel.astype(BF16)
    gt = _rnd(jnp.dot(xs, wg_v[...], preferred_element_type=F32))
    gt = _rnd(gt * jax.nn.sigmoid(gt))
    up = _rnd(jnp.dot(xs, wu_v[...], preferred_element_type=F32))
    gu = (gt * up).astype(BF16)
    y = _rnd(jax.lax.dot_general(gu, wdt_v[...], NT, preferred_element_type=F32))
    y = _rnd(y * _rnd(jax.nn.sigmoid(r_sel)))
    new = x1_sel + _rnd(row_scr[2] * _rnd(x_sel + y))
    scope('r5_patch')
    newt = jnp.concatenate([new, jnp.zeros((LANES - TOPC, d), F32)], axis=0).astype(BF16).T
    lane_d = jax.lax.broadcasted_iota(I32, (d // 2, LANES), 1)
    newt32 = pltpu.bitcast(newt, jnp.uint32)
    out32 = out_v.bitcast(jnp.uint32) if pm else None
    for cidx in range(TOPC):
        cols = pl.ds(pl.multiple_of(blks[cidx] * LANES, LANES), LANES)
        ln = idxs[cidx] & (LANES - 1)
        moved = pltpu.roll(newt32, (ln - cidx) & (LANES - 1), 1)
        if pm:
            pltpu.store(out32.at[0, :, cols], moved, mask=lane_d == ln)
        else:
            cur = pltpu.bitcast(out_v[0, :, cols], jnp.uint32)
            out_v[0, :, cols] = pltpu.bitcast(jnp.where(lane_d == ln, moved, cur), BF16)
        again = False
        for later in blks[cidx + 1:]:
            again = jnp.logical_or(again, later == blks[cidx])

        @pl.when(jnp.logical_not(again))
        def _(cidx=cidx, cols=cols):
            pltpu.make_async_copy(out_v.at[0, :, cols], out_hbm.at[:, cols],
                                  osem.at[blks[cidx]]).start()

    scope('r6_outwait')
    for b in range(nblk):
        out_copy(b).wait()
    es.close()


def build(ahead=384, qh=128, oh=144, lw=32, x0=512, prof=0, mid=1, lb=512, l1=512, rch=32, pm=1, gl=2):
    @jax.jit
    def fn(A_x, A_k_cache, A_v_cache, A_wq, A_wo, B_x, B_w_r, B_w_gate, B_w_up, B_w_down, c, w_mod):
        b, s_len, d = A_x.shape
        hkv, sk = A_k_cache.shape[1], A_k_cache.shape[2]
        rep = HQ // hkv
        f = B_w_gate.shape[1]
        xt = A_x.reshape(s_len, d).T
        k3 = A_k_cache.reshape(hkv, sk, DH)
        v3 = A_v_cache.reshape(hkv, sk, DH)
        wr2 = B_w_r.reshape(1, d)
        nblk = s_len // LANES
        scratch = [
            pltpu.VMEM((1, d, s_len), BF16),
            pltpu.VMEM((2, sk, DH), BF16),
            pltpu.VMEM((2, sk, DH), BF16),
            pltpu.VMEM((2, d, rep * DH), BF16),
            pltpu.VMEM((2, d, rep * DH), BF16),
            pltpu.VMEM((1, d), BF16),
            pltpu.VMEM((1, d), BF16),
            pltpu.VMEM((d, 6 * d), BF16),
            pltpu.VMEM((d, f), BF16),
            pltpu.VMEM((d, f), BF16),
            pltpu.VMEM((d, f), BF16),
            pltpu.VMEM((1, d, s_len), BF16),
            pltpu.VMEM((s_len, d), BF16),
            pltpu.VMEM((d, s_len), F32),
            pltpu.VMEM((3, 8, d), F32),
            pltpu.VMEM((5, d, LANES), F32),
            pltpu.VMEM((DH, sk), BF16),
            pltpu.VMEM((1, 2 * d, s_len), BF16),
            pltpu.VMEM((nblk, LANES), F32),
            pltpu.VMEM((2, 8, s_len), F32),
            pltpu.VMEM((1, sk, GW), F32),
            pltpu.VMEM((1, sk, GW), F32),
            pltpu.SMEM((1,), I32),
            pltpu.SemaphoreType.DMA((2, 4)),
            pltpu.SemaphoreType.DMA((9,)),
            pltpu.SemaphoreType.DMA((nblk,)),
            pltpu.SemaphoreType.DMA((s_len // x0,)),
        ]
        out = pl.pallas_call(
            functools.partial(_kernel, n_groups=hkv, rep=rep, ahead=ahead, qh=qh, oh=oh, lw=lw,
                              x0=x0, prof=prof, mid=mid, lb=lb, l1=l1, rch=rch, pm=pm, gl=gl),
            in_specs=[pl.BlockSpec(memory_space=pl.ANY)] * 11,
            out_specs=pl.BlockSpec(memory_space=pl.ANY),
            out_shape=jax.ShapeDtypeStruct((d, s_len), BF16),
            scratch_shapes=scratch,
            compiler_params=pltpu.CompilerParams(vmem_limit_bytes=100 * 1024 * 1024),
        )(xt, k3, v3, A_wq, A_wo.T, wr2, c, w_mod, B_w_gate, B_w_up, B_w_down.T)
        return out.T.reshape(b, s_len, d)
    return fn


pallas_adaLN_cond__gqa_block_cached__moe_arch_mod__prompt_kernel = build()
```

```python
import contextlib
import functools

import jax
import jax.numpy as jnp
import jax.experimental.pallas as pl
import jax.experimental.pallas.tpu as pltpu

HQ = 32
DH = 128
TOPC = 8
LN_EPS = 1e-05
LOG2E = 1.4426950408889634
F32 = jnp.float32
BF16 = jnp.bfloat16
I32 = jnp.int32
NT = (((1,), (1,)), ((), ()))
LANES = 128
GW = 512
MXU_LAT = 128


def _rnd(v):
    return v.astype(BF16).astype(F32)


def _by8(v):
    return v.reshape(v.shape[0] // 8, 8, v.shape[1])


def _ln_stats(shift, s1, s2, d):
    e1 = jnp.sum(s1, axis=0, keepdims=True) * (1.0 / d)
    e2 = jnp.sum(s2, axis=0, keepdims=True) * (1.0 / d)
    var = jnp.maximum(e2 - e1 * e1, 0.0)
    den = _rnd(jnp.sqrt(_rnd(_rnd(var) + LN_EPS)))
    return _rnd(shift + e1), jnp.broadcast_to(1.0 / den, shift.shape)


class _Moments:
    def __init__(self):
        self.shift = self.s1 = self.s2 = None

    def add(self, v, gate=lambda t: t):
        if self.shift is None:
            self.shift = jnp.broadcast_to(v[0:1], (8, v.shape[1]))
        dv = _by8(v) - gate(self.shift)[None]
        a, b = jnp.sum(dv, axis=0), jnp.sum(dv * dv, axis=0)
        self.s1, self.s2 = (a, b) if self.s1 is None else (self.s1 + a, self.s2 + b)

    def stats(self, d):
        return _ln_stats(self.shift, self.s1, self.s2, d)


def _kernel(xt_hbm, k_hbm, v_hbm, wq_hbm, wot_hbm, wr_hbm, c_hbm, wmod_hbm,
            wg_hbm, wu_hbm, wdt_hbm,
            out_hbm,
            xt_v, kbuf, vbuf, wqbuf, wobuf,
            wr_v, c_v, wmod_v, wg_v, wu_v, wdt_v, out_v,
            h_scr, acc_scr, row_scr, col_scr, vt_scr, xh_scr, r_scr, st_scr, s0_scr, s1_scr, z_scr, zv_scr,
            msem, osem, *,
            n_groups, rep, ahead, qh, oh, lw, nf, prof, mid, dt1, dt2, dl, ra, ra2, rc2, marg, sub, spause, sched_f, sched_l, kcp, ahp, vmode, vch):
    _, d, s_len = xt_v.shape
    sk = kbuf.shape[1]
    gcols = rep * DH
    tg = GW // rep
    ng = s_len // tg
    nblk = s_len // LANES
    nlt = tg // LANES
    s_bufs = (s0_scr, s1_scr)
    qscale = (DH ** -0.5) * LOG2E
    ident = lambda t: t

    def steady(n):
        return 'V Q0 Q1 K0 ' + ' '.join(
            ('O%d ' % (i - 2) if i >= 2 else '') + ('Q%d ' % (i + 2) if i + 2 < n else '')
            + ('S%d' % i if i + 1 < n else 'P%d' % i) for i in range(n)) + ' O%d O%d' % (n - 2, n - 1)

    es = contextlib.ExitStack()

    def scope(name):
        es.close()
        if prof:
            es.enter_context(jax.named_scope(name))

    def group_copies(g, slot):
        cols = pl.ds(pl.multiple_of(g * gcols, gcols), gcols)
        return (pltpu.make_async_copy(wq_hbm.at[:, cols], wqbuf.at[slot], msem.at[16 + slot * 4]),
                pltpu.make_async_copy(k_hbm.at[g], kbuf.at[slot], msem.at[17 + slot * 4]),
                pltpu.make_async_copy(v_hbm.at[g], vbuf.at[slot], msem.at[18 + slot * 4]),
                pltpu.make_async_copy(wot_hbm.at[:, cols], wobuf.at[slot], msem.at[19 + slot * 4]))

    def x_copy(lo, hi, sem):
        return pltpu.make_async_copy(xt_hbm.at[:, lo:hi], xt_v.at[0, :, lo:hi], msem.at[sem])

    cp_c = pltpu.make_async_copy(c_hbm, c_v, msem.at[0])
    cp_wr = pltpu.make_async_copy(wr_hbm, wr_v, msem.at[1])
    nxc = 4
    xw = s_len // nxc
    cp_x = [x_copy(j * xw, (j + 1) * xw, 9 + j) for j in range(nxc)]
    cp_m0 = pltpu.make_async_copy(wmod_hbm.at[:, 0:2 * d], wmod_v.at[:, 0:2 * d], msem.at[4])
    cp_m1 = pltpu.make_async_copy(wmod_hbm.at[:, 2 * d:6 * d], wmod_v.at[:, 2 * d:6 * d], msem.at[5])
    cp_moe = (pltpu.make_async_copy(wg_hbm, wg_v, msem.at[6]),
              pltpu.make_async_copy(wu_hbm, wu_v, msem.at[7]),
              pltpu.make_async_copy(wdt_hbm, wdt_v, msem.at[8]))

    def out_copy(b):
        cols = slice(b * LANES, (b + 1) * LANES)
        return pltpu.make_async_copy(out_v.at[:, cols], out_hbm.at[:, cols], osem.at[b])

    def silu_c8():
        cf = c_v[...].astype(F32)
        sc = (cf * jax.nn.sigmoid(cf)).astype(BF16)
        return jnp.broadcast_to(sc, (8, d))

    def tspan(i, lo, n):
        if isinstance(i, int):
            return slice(i * tg + lo, i * tg + lo + n)
        return pl.ds(pl.multiple_of(i * tg + lo, n), n)

    def tcols(i):
        return tspan(i, 0, tg)

    def col(j, rows):
        return jnp.concatenate([col_scr[j, rows, :]] * nlt, axis=1)

    def ln1_norm_piece(i, lt, rows, mean, rinv):
        ls = slice(lt * LANES, (lt + 1) * LANES)
        xv = _by8(xt_v[z_scr[0, 0], rows, tspan(i, lt * LANES, LANES)].astype(F32))
        y = (xv - mean[:, ls][None]) * rinv[:, ls][None]
        return y.reshape(rows.stop - rows.start, LANES).astype(BF16).T

    def ln1_mod_piece(i, lt, rows, y):
        h = y.astype(F32) * row_scr[1, 0:1, rows] + row_scr[0, 0:1, rows]
        h_scr[0, tspan(i, lt * LANES, LANES), rows] = h.astype(BF16)

    fch = [slice(lo, min(lo + LANES, d)) for lo in range(0, d, LANES)]

    def ln1_job(i):
        gate = yield
        mo = _Moments()
        for r0 in range(0, d, ra):
            mo.add(xt_v[0, r0:r0 + ra, tcols(i)].astype(F32), gate)
            if r0 + ra < d:
                gate = yield mo.s2
        mean, rinv = mo.stats(d)
        gate = yield rinv, spause
        for lt in range(nlt):
            for rows in fch:
                ln1_mod_piece(i, lt, rows, ln1_norm_piece(i, lt, rows, gate(mean), rinv))
                gate = yield None

    def ln2_x1(i, rows, attn, mo):
        ga = col(0, rows)
        x1b = (xt_v[0, rows, tcols(i)].astype(F32) + ga * attn).astype(BF16)
        xh_scr[d + rows.start:d + rows.stop, tcols(i)] = x1b
        mo.add(x1b.astype(F32))

    def ln2_stats(i, mo):
        mean, rinv = mo.stats(d)
        st_scr[0, :, tcols(i)] = mean
        st_scr[1, :, tcols(i)] = rinv

    def ln2_job(i):
        gate = yield
        mean, rinv = st_scr[0, :, tcols(i)], st_scr[1, :, tcols(i)]
        racc = None
        for r0 in range(0, d, rc2):
            rows = slice(r0, r0 + rc2)
            x1 = xh_scr[d + r0:d + r0 + rc2, tcols(i)].astype(F32)
            xc = (_by8(x1) - gate(mean)[None]).reshape(x1.shape)
            y = _rnd((_by8(_rnd(xc)) * rinv[None]).reshape(x1.shape))
            h2b = (_rnd(y * col(2, rows)) + col(1, rows)).astype(BF16)
            h2 = h2b.astype(F32)
            xh_scr[rows, tcols(i)] = h2b
            out_v[rows, tcols(i)] = (x1 + col(3, rows) * h2).astype(BF16)
            part = jnp.sum(_by8(h2 * col(4, rows)), axis=0)
            racc = part if racc is None else racc + part
            if r0 + rc2 == d:
                r = jnp.sum(racc, axis=0, keepdims=True)
                for lt in range(nlt):
                    r_scr[pl.ds(i * nlt + lt, 1), :] = r[:, lt * LANES:(lt + 1) * LANES]
            gate = yield racc

    def vt_job(v_ref):
        gate = yield
        for k0 in range(0, sk, vch):
            v32 = pltpu.bitcast(v_ref[k0:k0 + vch, :], F32)
            v32 = gate(_by8(v32)).reshape(v32.shape)
            vt = pltpu.bitcast(v32, BF16).T
            vt_scr[z_scr[0, 0], :, k0:k0 + vch] = pltpu.bitcast(vt, F32)
            gate = yield vt_scr[0, 0:8, 0:LANES]

    def run_all(job):
        next(job)
        try:
            while True:
                job.send(ident)
        except StopIteration:
            pass

    def attn_group(refs, toks, sched, first=False, last=False, barriers=None, jobs=None, dt=128):
        wq_ref, k_ref, v_ref, wot_ref = refs
        barriers = barriers or {}
        jobs = jobs or {}
        n = len(toks)
        st = dict(zero=None, zvec=None, clock=0, nxt=0, on=False)
        hist = []
        queue = []
        due = []

        def fresh():
            st['zero'] = z_scr[0, 0]
            st['zvec'] = jnp.full((8, LANES), st['zero'], I32)

        def token(when):
            want = when - MXU_LAT
            for start, dur, res in reversed(hist):
                if start <= want:
                    row = min((want - start) * res.shape[0] // dur // 8 * 8, res.shape[0] - 8)
                    return pltpu.bitcast(res[row:row + 8, 0:LANES], I32) & st['zvec']
            return None

        def tie(x, tok):
            if tok is None:
                return x
            reps = x.shape[-1] // LANES
            if reps > 1:
                tok = jnp.concatenate([tok] * reps, axis=1)
            if x.ndim == 3:
                tok = tok[None]
            return pltpu.bitcast(pltpu.bitcast(x, I32) | tok, F32)

        def side(upto=None):
            upto = st['clock'] if upto is None else upto
            while queue and st['on'] and st['nxt'] <= upto:
                tok = token(st['nxt'] + MXU_LAT)
                try:
                    v = queue[0].send(lambda x, tok=tok: tie(x, tok))
                except StopIteration:
                    queue.pop(0)
                    continue
                v, pause = v if isinstance(v, tuple) else (v, 0)
                if dl and v is not None:
                    due.append((st['nxt'] + dl + pause, v))
                st['nxt'] += dt + pause

        def release(gens):
            for gen in gens:
                next(gen)
                queue.append(gen)
            st['nxt'] = max(st['nxt'], st['clock'])

        def drain():
            while queue:
                try:
                    queue[0].send(ident)
                except StopIteration:
                    queue.pop(0)

        def mark(tag):
            if tag in barriers:
                drain()
                barriers[tag]()
                hist.clear()
                due.clear()
                fresh()
            release(jobs.get(tag, []))

        def step(result, dur, adv=True):
            hist.append((st['clock'], dur, result))
            if adv:
                st['clock'] += dur
                side()

        def after(x, ahead):
            return tie_due(tie(x, token(st['clock'] - ahead)), st['clock'] - ahead)

        def tie_due(x, now):
            while due and due[0][0] <= now:
                v = pltpu.bitcast(due.pop(0)[1], I32)
                bits = v[:, 0:LANES]
                for j in range(1, v.shape[1] // LANES):
                    bits = bits | v[:, j * LANES:(j + 1) * LANES]
                x = tie(x, bits & st['zvec'])
            return x

        def qproj(i):
            parts = []
            for hb in range(tg // qh):
                q = jnp.dot(h_scr[0, tspan(toks[i], hb * qh, qh), :], wq_ref[...],
                            preferred_element_type=F32)
                step(q, qh * 10 // 4)
                parts.append((q * qscale).astype(BF16))
            return jnp.concatenate([p[:, r * DH:(r + 1) * DH] for r in range(rep) for p in parts],
                                   axis=0)

        def qk_part(qg, buf, rows, cols, adv):
            s = jax.lax.dot_general(k_ref[rows, :], qg[cols], NT, preferred_element_type=F32)
            s_bufs[buf][st['zero'], rows, cols] = s
            m = jnp.max(_by8(s), axis=0)
            step(s, s.shape[0], adv)
            return m

        def max_fin(m):
            return jnp.broadcast_to(jnp.max(m, axis=0, keepdims=True), m.shape)

        def qk(qg, buf):
            m = None
            if not queue:
                for j in range(4):
                    mj = qk_part(qg, buf, slice(j * sk // 4, (j + 1) * sk // 4), slice(0, GW), True)
                    m = mj if m is None else jnp.maximum(m, mj)
                return max_fin(m)
            was, st['on'] = st['on'], True
            st['nxt'] = max(st['nxt'], st['clock'])
            stop = st['clock'] + sk - marg
            for j in range(4):
                rows = slice(j * sk // 4, (j + 1) * sk // 4)
                sc = jax.lax.dot_general(k_ref[rows, :], qg, NT, preferred_element_type=F32)
                s_bufs[buf][st['zero'], rows, :] = sc
                t_start = st['clock']
                hist.append((t_start, sc.shape[0], sc))
                for r0 in range(0, sc.shape[0], sub):
                    mj = jnp.max(_by8(sc[r0:r0 + sub]), axis=0)
                    if m is not None:
                        m0 = tie_due(m[:, 0:LANES], t_start + r0)
                        mj = jnp.maximum(jnp.concatenate([m0, m[:, LANES:]], axis=1), mj)
                    m = mj
                    side(min(t_start + r0 + sub - 1, stop))
                st['clock'] += sc.shape[0]
            st['on'] = was
            return max_fin(m)

        def pv_unit(buf, m, u, kc, dur, ahead):
            cs = slice(u * LANES, (u + 1) * LANES)
            o = l = None
            for j in range(sk // kc):
                mu = after(m[:, cs], ahead)
                p = jnp.exp2(_by8(s_bufs[buf][0, j * kc:(j + 1) * kc, cs]) - mu[None])
                lj = jnp.sum(p.reshape(kc // lw, lw, LANES), axis=0)
                oj = jnp.dot(pltpu.bitcast(vt_scr[0, :, j * kc:(j + 1) * kc], BF16),
                             p.reshape(kc, LANES).astype(BF16),
                             preferred_element_type=F32)
                o = oj if o is None else o + oj
                l = lj if l is None else l + lj
                hist.append((st['clock'], DH, oj))
                st['clock'] += dur
                side()
            return (o / jnp.sum(l, axis=0, keepdims=True)).astype(BF16)

        def gather_out(outs):
            return jnp.concatenate(
                [jnp.concatenate(outs[r * nlt:(r + 1) * nlt], axis=1) for r in range(rep)], axis=0)

        def pv(buf, m):
            return gather_out([pv_unit(buf, m, u, kcp, kcp // 4, ahp) for u in range(4)])

        def pv_qk(buf, m, qn, nbuf):
            outs, mns = [], []
            for half in range(2):
                mns.append(qk_part(qn, nbuf, slice(0, sk), slice(half * 256, (half + 1) * 256), False))
                outs += [pv_unit(buf, m, u, 256, DH, ahead) for u in (2 * half, 2 * half + 1)]
            return gather_out(outs), max_fin(jnp.concatenate(mns, axis=1))

        def oproj(i, ot):
            cols = tcols(toks[i])
            mo = _Moments()
            for rb in range(d // oh):
                rows = slice(rb * oh, (rb + 1) * oh)
                res = jnp.dot(wot_ref[rows, :], ot, preferred_element_type=F32)
                tot = res if first else res + acc_scr[rows, cols]
                if last:
                    ln2_x1(toks[i], rows, tot, mo)
                else:
                    acc_scr[rows, cols] = tot
                step(res, oh)
            if last:
                ln2_stats(toks[i], mo)

        qs, ots, ms, bufs = {}, {}, {}, {}
        free = [0, 1]
        fresh()
        for item in sched.split():
            kind, arg = item[0], item[1:]
            if kind == '|':
                mark(arg)
                continue
            if kind == 'V':
                if vmode == 0:
                    vt_scr[0] = pltpu.bitcast(v_ref[...].T, F32)
                elif vmode == 1:
                    vt_scr[st['zero']] = pltpu.bitcast(v_ref[...].T, F32)
                else:
                    gen = vt_job(v_ref)
                    next(gen)
                    queue.insert(0, gen)
                continue
            if kind == '+':
                st['on'] = True
                st['nxt'] = max(st['nxt'], st['clock'])
                continue
            i = int(arg)
            if kind == 'Q':
                qs[i] = qproj(i)
            elif kind == 'K':
                bufs[i] = free.pop(0)
                ms[i] = qk(qs[i], bufs[i])
            elif kind == 'P':
                ots[i] = pv(bufs[i], ms[i])
                free.append(bufs[i])
            elif kind == 'S':
                bufs[i + 1] = free.pop(0)
                ots[i], ms[i + 1] = pv_qk(bufs[i], ms[i], qs[i + 1], bufs[i + 1])
                free.append(bufs[i])
            elif kind == 'O':
                oproj(i, ots[i])
        drain()

    scope('p0_start')
    zv_scr[...] = jnp.zeros(zv_scr.shape, I32)
    cp_z = pltpu.make_async_copy(zv_scr, z_scr, msem.at[2])
    for cp in ((cp_z, cp_c, cp_x[0], cp_m0) + tuple(cp_x[1:]) + group_copies(0, 0) + (cp_wr,)):
        cp.start()

    def zero_body(j, carry):
        acc_scr[pl.ds(pl.multiple_of(j * 64, 64), 64), :] = jnp.zeros((64, s_len), F32)
        return carry

    jax.lax.fori_loop(0, d // 64, zero_body, 0)
    xh_scr[d:2 * d, s_len - 2 * tg:s_len] = jnp.zeros((d, 2 * tg), BF16)
    st_scr[...] = jnp.zeros(st_scr.shape, F32)
    scope('p1_waitx')
    cp_z.wait()
    cp_x[0].wait()
    scope('p1_norm')
    per = xw // tg
    ys = {}
    for i in range(per):
        mo = _Moments()
        for r0 in range(0, d, 64):
            mo.add(xt_v[0, r0:r0 + 64, tcols(i)].astype(F32))
        mean, rinv = mo.stats(d)
        for lt in range(nlt):
            for rows in fch:
                ys[i, lt, rows.start] = ln1_norm_piece(i, lt, rows, mean, rinv)
    scope('p2_waitmod')
    cp_c.wait()
    cp_m0.wait()
    scope('p2_mod')
    mod = _rnd(jnp.dot(silu_c8(), wmod_v[:, 0:2 * d], preferred_element_type=F32))
    row_scr[0] = mod[:, 0:d]
    row_scr[1] = _rnd(1.0 + mod[:, d:2 * d])
    for i in range(per):
        for lt in range(nlt):
            for rows in fch:
                ln1_mod_piece(i, lt, rows, ys[i, lt, rows.start])
    scope('p3_ln1')

    def ln1_body(j, carry):
        pltpu.make_async_copy(xt_hbm.at[:, 0:xw], xt_v.at[0, :, pl.ds(pl.multiple_of(j * xw, xw), xw)],
                              msem.at[9 + j]).wait()
        for i in range(per):
            run_all(ln1_job(j * per + i))
        return carry

    jax.lax.fori_loop(1, nxc, ln1_body, 0)

    def mid_body(g, carry):
        slot = g % 2
        with (jax.named_scope('q1_wait') if prof else contextlib.nullcontext()):
            for cp in group_copies(g, slot):
                cp.wait()
        for cp in group_copies(g + 1, 1 - slot):
            cp.start()
        for j, cp in enumerate((cp_m1,) + cp_moe):
            @pl.when(g == (1 + j if mid else 0))
            def _(cp=cp):
                cp.start()

        if mid:
            with (jax.named_scope('q2_body') if prof else contextlib.nullcontext()):
                attn_group((wqbuf.at[slot], kbuf.at[slot], vbuf.at[slot], wobuf.at[slot]),
                           list(range(ng)), steady(ng))
        return carry

    lastg = n_groups - 1 if mid else 1
    scope('q_loop')
    jax.lax.fori_loop(0, lastg, mid_body, 0)

    scope('r0_wait')
    ls = lastg % 2
    for cp in group_copies(lastg, ls) + (cp_m1, cp_wr) + cp_moe:
        cp.wait()
    scope('r0_mod2')
    mod = _rnd(jnp.dot(silu_c8(), wmod_v[:, 2 * d:6 * d], preferred_element_type=F32))
    piece = lambda j: mod[0:1, j * d:(j + 1) * d]
    rows5 = [piece(0), piece(1), _rnd(1.0 + piece(2)), piece(3), wr_v[...].astype(F32)]
    for j, row in enumerate(rows5):
        col_scr[j] = jnp.broadcast_to(row, (LANES, d)).T
    row_scr[2] = mod[:, 3 * d:4 * d]
    npair = ng // 2

    def last_body(t, carry):
        prev = (t + npair - 1) % npair
        attn_group((wqbuf.at[ls], kbuf.at[ls], vbuf.at[ls], wobuf.at[ls]),
                   [2 * t, 2 * t + 1], sched_l, last=True,
                   jobs=dict(a=[ln2_job(2 * prev), ln2_job(2 * prev + 1)]), dt=dt2)
        return carry

    scope('r1_last')
    jax.lax.fori_loop(0, npair, last_body, 0)
    scope('r1_ln2')
    run_all(ln2_job(ng - 2))
    run_all(ln2_job(ng - 1))

    scope('r2_topk')
    ibits = (s_len - 1).bit_length()
    imask = (1 << ibits) - 1
    bits = pltpu.bitcast(_rnd(r_scr[...]), I32)
    pos = (jax.lax.broadcasted_iota(I32, bits.shape, 0) * LANES
           + jax.lax.broadcasted_iota(I32, bits.shape, 1))
    order = ((bits ^ ((bits >> 31) & 0x7FFFFFFF)) >> 16) + 0x8000
    key = pltpu.bitcast((order << ibits) + (imask - pos) + 0x20000000, F32)
    sub = jax.lax.broadcasted_iota(I32, (TOPC, LANES), 0)
    lane = jax.lax.broadcasted_iota(I32, (TOPC, LANES), 1)
    idxs, blks = [], []
    keyv = jnp.zeros((TOPC, LANES), I32)
    xh_sel = jnp.zeros((TOPC, 2 * d), F32)
    for cidx in range(TOPC):
        top = jnp.max(jnp.max(key, axis=0, keepdims=True), axis=1, keepdims=True)
        key = jnp.where(key == top, 0.0, key)
        topi = pltpu.bitcast(jnp.broadcast_to(top, (TOPC, LANES)), I32)
        keyv = jnp.where(sub == cidx, topi, keyv)
        ixv = imask - (topi & imask)
        ix = ixv[0, 0]
        idxs.append(ix)
        blks.append(ix >> 7)
        cols = pl.ds(pl.multiple_of(blks[cidx] * LANES, LANES), LANES)
        oh1 = jnp.where((lane == (ixv & (LANES - 1))) & (sub == cidx), 1.0, 0.0).astype(BF16)
        xh_sel = xh_sel + jax.lax.dot_general(oh1, xh_scr[:, cols], NT, preferred_element_type=F32)

    for b in range(nblk):
        hit = blks[0] == b
        for bb in blks[1:]:
            hit = jnp.logical_or(hit, bb == b)

        @pl.when(jnp.logical_not(hit))
        def _(b=b):
            out_copy(b).start()

    scope('r4_moe')
    x_sel = xh_sel[:, 0:d]
    x1_sel = xh_sel[:, d:2 * d]
    ob = (((keyv - 0x20000000) >> ibits) - 0x8000) << 16
    r_sel = pltpu.bitcast((ob ^ ((ob >> 31) & 0x7FFFFFFF)) & ~0xFFFF, F32)[:, 0:1]
    xs = x_sel.astype(BF16)
    gt = _rnd(jnp.dot(xs, wg_v[...], preferred_element_type=F32))
    gt = _rnd(gt * jax.nn.sigmoid(gt))
    up = _rnd(jnp.dot(xs, wu_v[...], preferred_element_type=F32))
    gu = (gt * up).astype(BF16)
    y = _rnd(jax.lax.dot_general(gu, wdt_v[...], NT, preferred_element_type=F32))
    y = _rnd(y * _rnd(jax.nn.sigmoid(r_sel)))
    new = x1_sel + _rnd(row_scr[2] * _rnd(x_sel + y))
    scope('r5_patch')
    newt = jnp.concatenate([new, jnp.zeros((LANES - TOPC, d), F32)], axis=0).astype(BF16).T
    lane_d = jax.lax.broadcasted_iota(I32, (d // 2, LANES), 1)
    newt32 = pltpu.bitcast(newt, jnp.uint32)
    out32 = out_v.bitcast(jnp.uint32)
    for cidx in range(TOPC):
        cols = pl.ds(pl.multiple_of(blks[cidx] * LANES, LANES), LANES)
        ln = idxs[cidx] & (LANES - 1)
        moved = pltpu.roll(newt32, (ln - cidx) & (LANES - 1), 1)
        pltpu.store(out32.at[:, cols], moved, mask=lane_d == ln)
        again = False
        for later in blks[cidx + 1:]:
            again = jnp.logical_or(again, later == blks[cidx])

        @pl.when(jnp.logical_not(again))
        def _(cidx=cidx, cols=cols):
            pltpu.make_async_copy(out_v.at[:, cols], out_hbm.at[:, cols],
                                  osem.at[blks[cidx]]).start()

    scope('r6_outwait')
    for b in range(nblk):
        out_copy(b).wait()
    es.close()


def build(ahead=384, qh=128, oh=144, lw=32, nf=3, prof=0, mid=1, dt1=48, dt2=96, dl=192, ra=96,
          ra2=64, rc2=32, marg=128, sub=64, spause=128, kcp=256, ahp=320, vmode=1, vch=256,
          sched_f='|a Q0 Q1 |b K0 |c V Q2 P0 |d K1 K2 O0 P1 P2 O1 O2',
          sched_l='|a V Q0 Q1 K0 K1 P0 P1 O0 O1'):
    @jax.jit
    def fn(A_x, A_k_cache, A_v_cache, A_wq, A_wo, B_x, B_w_r, B_w_gate, B_w_up, B_w_down, c, w_mod):
        b, s_len, d = A_x.shape
        hkv, sk = A_k_cache.shape[1], A_k_cache.shape[2]
        rep = HQ // hkv
        f = B_w_gate.shape[1]
        xt = A_x.reshape(s_len, d).T
        k3 = A_k_cache.reshape(hkv, sk, DH)
        v3 = A_v_cache.reshape(hkv, sk, DH)
        wr2 = B_w_r.reshape(1, d)
        nblk = s_len // LANES
        tg = GW // rep
        scratch = [
            pltpu.VMEM((1, d, s_len), BF16),
            pltpu.VMEM((2, sk, DH), BF16),
            pltpu.VMEM((2, sk, DH), BF16),
            pltpu.VMEM((2, d, rep * DH), BF16),
            pltpu.VMEM((2, d, rep * DH), BF16),
            pltpu.VMEM((1, d), BF16),
            pltpu.VMEM((1, d), BF16),
            pltpu.VMEM((d, 6 * d), BF16),
            pltpu.VMEM((d, f), BF16),
            pltpu.VMEM((d, f), BF16),
            pltpu.VMEM((d, f), BF16),
            pltpu.VMEM((d, s_len), BF16),
            pltpu.VMEM((1, s_len, d), BF16),
            pltpu.VMEM((d, s_len), F32),
            pltpu.VMEM((3, 8, d), F32),
            pltpu.VMEM((5, d, LANES), F32),
            pltpu.VMEM((1, DH // 2, sk), F32),
            pltpu.VMEM((2 * d, s_len), BF16),
            pltpu.VMEM((nblk, LANES), F32),
            pltpu.VMEM((2, 8, s_len), F32),
            pltpu.VMEM((1, sk, GW), F32),
            pltpu.VMEM((1, sk, GW), F32),
            pltpu.SMEM((8, LANES), I32),
            pltpu.VMEM((8, LANES), I32),
            pltpu.SemaphoreType.DMA((24,)),
            pltpu.SemaphoreType.DMA((nblk,)),
        ]
        out = pl.pallas_call(
            functools.partial(_kernel, n_groups=hkv, rep=rep, ahead=ahead, qh=qh, oh=oh, lw=lw,
                              nf=nf, prof=prof, mid=mid, dt1=dt1, dt2=dt2, dl=dl, ra=ra, ra2=ra2, rc2=rc2,
                              marg=marg, sub=sub, spause=spause, sched_f=sched_f, sched_l=sched_l, kcp=kcp, ahp=ahp, vmode=vmode, vch=vch),
            in_specs=[pl.BlockSpec(memory_space=pl.ANY)] * 11,
            out_specs=pl.BlockSpec(memory_space=pl.ANY),
            out_shape=jax.ShapeDtypeStruct((d, s_len), BF16),
            scratch_shapes=scratch,
            compiler_params=pltpu.CompilerParams(vmem_limit_bytes=100 * 1024 * 1024),
        )(xt, k3, v3, A_wq, A_wo.T, wr2, c, w_mod, B_w_gate, B_w_up, B_w_down.T)
        return out.T.reshape(b, s_len, d)
    return fn


pallas_adaLN_cond__gqa_block_cached__moe_arch_mod__prompt_kernel = build()
```

```python
import contextlib
import functools

import jax
import jax.numpy as jnp
import jax.experimental.pallas as pl
import jax.experimental.pallas.tpu as pltpu

HQ = 32
DH = 128
TOPC = 8
LN_EPS = 1e-05
LOG2E = 1.4426950408889634
F32 = jnp.float32
BF16 = jnp.bfloat16
I32 = jnp.int32
NT = (((1,), (1,)), ((), ()))
LANES = 128
GW = 512
MXU_LAT = 128


def _rnd(v):
    return v.astype(BF16).astype(F32)


def _by8(v):
    return v.reshape(v.shape[0] // 8, 8, v.shape[1])


def _ln_stats(shift, s1, s2, d):
    e1 = jnp.sum(s1, axis=0, keepdims=True) * (1.0 / d)
    e2 = jnp.sum(s2, axis=0, keepdims=True) * (1.0 / d)
    var = jnp.maximum(e2 - e1 * e1, 0.0)
    den = _rnd(jnp.sqrt(_rnd(_rnd(var) + LN_EPS)))
    return _rnd(shift + e1), jnp.broadcast_to(1.0 / den, shift.shape)


class _Moments:
    def __init__(self):
        self.shift = self.s1 = self.s2 = None

    def add(self, v, gate=lambda t: t):
        if self.shift is None:
            self.shift = jnp.broadcast_to(v[0:1], (8, v.shape[1]))
        dv = _by8(v) - gate(self.shift)[None]
        a, b = jnp.sum(dv, axis=0), jnp.sum(dv * dv, axis=0)
        self.s1, self.s2 = (a, b) if self.s1 is None else (self.s1 + a, self.s2 + b)

    def stats(self, d):
        return _ln_stats(self.shift, self.s1, self.s2, d)


def _kernel(xt_hbm, k_hbm, v_hbm, wq_hbm, wot_hbm, wr_hbm, c_hbm, wmod_hbm,
            wg_hbm, wu_hbm, wdt_hbm,
            out_hbm,
            xt_v, kbuf, vbuf, wqbuf, wobuf, wql_v, q_scr,
            wr_v, c_v, wmod_v, wg_v, wu_v, wdt_v, wd_scr, out_v,
            h_scr, acc_scr, row_scr, col_scr, vt_scr, xh_scr, r_scr, st_scr, s0_scr, s1_scr, z_scr, zv_scr, new_scr,
            msem, *,
            n_groups, rep, ahead, qh, oh, lw, nf, prof, mid, dt1, dt2, dl, ra, ra2, rc2, marg, sub, spause, sched_f, sched_l, kcp, ahp, vmode, vch, l1mode, wpause, cuts):
    _, d, s_len = xt_v.shape
    sk = kbuf.shape[1]
    gcols = rep * DH
    tg = GW // rep
    ng = s_len // tg
    nblk = s_len // LANES
    nlt = tg // LANES
    s_bufs = (s0_scr, s1_scr)
    qscale = (DH ** -0.5) * LOG2E
    ident = lambda t: t

    def steady(n):
        return 'V Q0 Q1 K0 ! ' + ' '.join(
            ('O%d ' % (i - 2) if i >= 2 else '') + ('Q%d ' % (i + 2) if i + 2 < n else '')
            + ('S%d' % i if i + 1 < n else 'P%d' % i) for i in range(n)) + ' O%d O%d' % (n - 2, n - 1)

    es = contextlib.ExitStack()

    def scope(name):
        es.close()
        if prof:
            es.enter_context(jax.named_scope(name))

    def group_copies(g, slot):
        cols = pl.ds(pl.multiple_of(g * gcols, gcols), gcols)
        return (pltpu.make_async_copy(wq_hbm.at[:, cols], wqbuf.at[slot], msem.at[5 + slot]),
                pltpu.make_async_copy(k_hbm.at[g], kbuf.at[slot], msem.at[5 + slot]),
                pltpu.make_async_copy(v_hbm.at[g], vbuf.at[slot], msem.at[5 + slot]),
                pltpu.make_async_copy(wot_hbm.at[:, cols], wobuf.at[slot], msem.at[5 + slot]))

    def x_copy(lo, hi, sem):
        return pltpu.make_async_copy(xt_hbm.at[:, lo:hi], xt_v.at[0, :, lo:hi], msem.at[sem])

    cp_c = pltpu.make_async_copy(c_hbm, c_v, msem.at[1])
    cp_wr = pltpu.make_async_copy(wr_hbm, wr_v, msem.at[0])
    nxc = 4
    xw = s_len // nxc
    cp_x = [x_copy(j * xw, (j + 1) * xw, j + 1 if j else 0) for j in range(nxc)]
    cp_m0 = pltpu.make_async_copy(wmod_hbm.at[:, 0:2 * d], wmod_v.at[:, 0:2 * d], msem.at[1])
    cp_m1 = pltpu.make_async_copy(wmod_hbm.at[:, 2 * d:6 * d], wmod_v.at[:, 2 * d:6 * d], msem.at[0])
    cp_moe = (pltpu.make_async_copy(wg_hbm, wg_v, msem.at[0]),
              pltpu.make_async_copy(wu_hbm, wu_v, msem.at[0]),
              pltpu.make_async_copy(wdt_hbm, wdt_v, msem.at[0]))

    lastg = n_groups - 1 if mid else 1
    cp_wql = pltpu.make_async_copy(wq_hbm.at[:, lastg * gcols:(lastg + 1) * gcols], wql_v, msem.at[2])

    def out_copy(b):
        cols = slice(b * LANES, (b + 1) * LANES)
        return pltpu.make_async_copy(out_v.at[:, cols], out_hbm.at[:, cols], msem.at[1])

    def silu_c8():
        cf = c_v[...].astype(F32)
        sc = (cf * jax.nn.sigmoid(cf)).astype(BF16)
        return jnp.broadcast_to(sc, (8, d))

    def tspan(i, lo, n):
        if isinstance(i, int):
            return slice(i * tg + lo, i * tg + lo + n)
        return pl.ds(pl.multiple_of(i * tg + lo, n), n)

    def tcols(i):
        return tspan(i, 0, tg)

    def col(j, rows):
        return jnp.concatenate([col_scr[j, rows, :]] * nlt, axis=1)

    def ln1_norm_piece(i, lt, rows, mean, rinv):
        ls = slice(lt * LANES, (lt + 1) * LANES)
        xv = _by8(xt_v[z_scr[0, 0], rows, tspan(i, lt * LANES, LANES)].astype(F32))
        y = (xv - mean[:, ls][None]) * rinv[:, ls][None]
        return y.reshape(rows.stop - rows.start, LANES).astype(BF16).T

    def ln1_mod_piece(i, lt, rows, y):
        h = y.astype(F32) * row_scr[1, 0:1, rows] + row_scr[0, 0:1, rows]
        h_scr[0, tspan(i, lt * LANES, LANES), rows] = h.astype(BF16)

    fch = [slice(lo, min(lo + LANES, d)) for lo in range(0, d, LANES)]

    def ln1_job(i, dst):
        gate = yield
        mo = _Moments()
        for r0 in range(0, d, ra):
            mo.add(xt_v[0, r0:r0 + ra, tcols(i)].astype(F32), gate)
            if r0 + ra < d:
                gate = yield mo.s2
        mean, rinv = mo.stats(d)
        gate = yield rinv, spause
        for lt in range(nlt):
            for rows in fch:
                ln1_mod_piece(dst, lt, rows, ln1_norm_piece(i, lt, rows, gate(mean), rinv))
                gate = yield None

    def ln2_x1(i, rows, attn, mo):
        ga = col(0, rows)
        x1b = (xt_v[0, rows, tcols(i)].astype(F32) + ga * attn).astype(BF16)
        xh_scr[d + rows.start:d + rows.stop, tcols(i)] = x1b
        mo.add(x1b.astype(F32))

    def ln2_stats(i, mo):
        mean, rinv = mo.stats(d)
        st_scr[0, :, tcols(i)] = mean
        st_scr[1, :, tcols(i)] = rinv

    def ln2_job(i):
        gate = yield
        mean, rinv = st_scr[0, :, tcols(i)], st_scr[1, :, tcols(i)]
        racc = None
        for r0 in range(0, d, rc2):
            rows = slice(r0, r0 + rc2)
            x1 = xh_scr[d + r0:d + r0 + rc2, tcols(i)].astype(F32)
            xc = (_by8(x1) - gate(mean)[None]).reshape(x1.shape)
            y = _rnd((_by8(_rnd(xc)) * rinv[None]).reshape(x1.shape))
            h2b = (_rnd(y * col(2, rows)) + col(1, rows)).astype(BF16)
            h2 = h2b.astype(F32)
            xh_scr[rows, tcols(i)] = h2b
            out_v[rows, tcols(i)] = (x1 + col(3, rows) * h2).astype(BF16)
            part = jnp.sum(_by8(h2 * col(4, rows)), axis=0)
            racc = part if racc is None else racc + part
            if r0 + rc2 == d:
                r = jnp.sum(racc, axis=0, keepdims=True)
                for lt in range(nlt):
                    r_scr[pl.ds(i * nlt + lt, 1), :] = r[:, lt * LANES:(lt + 1) * LANES]
            gate = yield racc

    def project_q(tok, wq_ref, step=lambda *a: None):
        parts = []
        for hb in range(tg // qh):
            q = jnp.dot(h_scr[0, tspan(tok, hb * qh, qh), :], wq_ref[...],
                        preferred_element_type=F32)
            step(q, qh * 10 // 4)
            parts.append((q * qscale).astype(BF16))
        return jnp.concatenate([p[:, r * DH:(r + 1) * DH] for r in range(rep) for p in parts],
                               axis=0)

    def vt_job(v_ref):
        gate = yield
        for k0 in range(0, sk, vch):
            v32 = pltpu.bitcast(v_ref[k0:k0 + vch, :], F32)
            v32 = gate(_by8(v32)).reshape(v32.shape)
            vt = pltpu.bitcast(v32, BF16).T
            vt_scr[z_scr[0, 0], :, k0:k0 + vch] = pltpu.bitcast(vt, F32)
            gate = yield vt_scr[0, 0:8, 0:LANES]

    def wd_job(t, parts):
        gate = yield
        fw = wdt_v.shape[1] // parts
        for f0 in range(0, fw, LANES):
            lo = pl.multiple_of(t * fw + f0, LANES)
            w32 = pltpu.bitcast(wdt_v[:, pl.ds(lo, LANES)], F32)
            w32 = gate(_by8(w32)).reshape(w32.shape)
            wd = pltpu.bitcast(w32, BF16).T
            half = pl.multiple_of(t * (fw // 2) + f0 // 2, LANES // 2)
            wd_scr[pl.ds(half, LANES // 2), :] = pltpu.bitcast(wd, F32)
            gate = yield wd_scr[0:8, 0:LANES], wpause

    def mix(a, b, every):
        next(a)
        next(b)
        gate = yield
        n, live = 0, [a, b]
        while live:
            n += 1
            job = b if (b in live and (n % (every + 1) == 0 or a not in live)) else a
            try:
                v = job.send(gate)
            except StopIteration:
                live.remove(job)
                continue
            gate = yield v

    def chain(*jobs):
        gate = yield
        for job in jobs:
            next(job)
            while True:
                try:
                    v = job.send(gate)
                except StopIteration:
                    break
                gate = yield v

    def run_all(job):
        next(job)
        try:
            while True:
                job.send(ident)
        except StopIteration:
            pass

    def attn_group(refs, toks, sched, first=False, last=False, barriers=None, jobs=None, dt=128,
                   hook=None):
        wq_ref, k_ref, v_ref, wot_ref = refs
        barriers = barriers or {}
        jobs = jobs or {}
        n = len(toks)
        st = dict(zero=None, zvec=None, clock=0, nxt=0, on=False)
        hist = []
        queue = []
        due = []

        def fresh():
            st['zero'] = z_scr[0, 0]
            st['zvec'] = jnp.full((8, LANES), st['zero'], I32)

        def token(when):
            want = when - MXU_LAT
            for start, dur, res in reversed(hist):
                if start <= want:
                    row = min((want - start) * res.shape[0] // dur // 8 * 8, res.shape[0] - 8)
                    return pltpu.bitcast(res[row:row + 8, 0:LANES], I32) & st['zvec']
            return None

        def tie(x, tok):
            if tok is None:
                return x
            reps = x.shape[-1] // LANES
            if reps > 1:
                tok = jnp.concatenate([tok] * reps, axis=1)
            if x.ndim == 3:
                tok = tok[None]
            return pltpu.bitcast(pltpu.bitcast(x, I32) | tok, F32)

        def side(upto=None):
            upto = st['clock'] if upto is None else upto
            while queue and st['on'] and st['nxt'] <= upto:
                tok = token(st['nxt'] + MXU_LAT)
                try:
                    v = queue[0].send(lambda x, tok=tok: tie(x, tok))
                except StopIteration:
                    queue.pop(0)
                    continue
                v, pause = v if isinstance(v, tuple) else (v, 0)
                if dl and v is not None:
                    due.append((st['nxt'] + dl + pause, v))
                st['nxt'] += dt + pause

        def release(gens):
            for gen in gens:
                next(gen)
                queue.append(gen)
            st['nxt'] = max(st['nxt'], st['clock'])

        def drain():
            while queue:
                try:
                    queue[0].send(ident)
                except StopIteration:
                    queue.pop(0)

        def mark(tag):
            if tag in barriers:
                drain()
                barriers[tag]()
                hist.clear()
                due.clear()
                fresh()
            release(jobs.get(tag, []))

        def step(result, dur, adv=True):
            hist.append((st['clock'], dur, result))
            if adv:
                st['clock'] += dur
                side()

        def after(x, ahead):
            return tie_due(tie(x, token(st['clock'] - ahead)), st['clock'] - ahead)

        def tie_due(x, now):
            while due and due[0][0] <= now:
                v = pltpu.bitcast(due.pop(0)[1], I32)
                bits = v[:, 0:LANES]
                for j in range(1, v.shape[1] // LANES):
                    bits = bits | v[:, j * LANES:(j + 1) * LANES]
                x = tie(x, bits & st['zvec'])
            return x

        def qk_part(qg, buf, rows, cols, adv):
            s = jax.lax.dot_general(k_ref[rows, :], qg[cols], NT, preferred_element_type=F32)
            s_bufs[buf][st['zero'], rows, cols] = s
            m = jnp.max(_by8(s), axis=0)
            step(s, s.shape[0], adv)
            return m

        def max_fin(m):
            return jnp.broadcast_to(jnp.max(m, axis=0, keepdims=True), m.shape)

        def qk(qg, buf):
            m = None
            if not queue:
                for j in range(4):
                    mj = qk_part(qg, buf, slice(j * sk // 4, (j + 1) * sk // 4), slice(0, GW), True)
                    m = mj if m is None else jnp.maximum(m, mj)
                return max_fin(m)
            was, st['on'] = st['on'], True
            st['nxt'] = max(st['nxt'], st['clock'])
            stop = st['clock'] + sk - marg
            for j in range(4):
                rows = slice(j * sk // 4, (j + 1) * sk // 4)
                sc = jax.lax.dot_general(k_ref[rows, :], qg, NT, preferred_element_type=F32)
                s_bufs[buf][st['zero'], rows, :] = sc
                t_start = st['clock']
                hist.append((t_start, sc.shape[0], sc))
                for r0 in range(0, sc.shape[0], sub):
                    mj = jnp.max(_by8(sc[r0:r0 + sub]), axis=0)
                    if m is not None:
                        m0 = tie_due(m[:, 0:LANES], t_start + r0)
                        mj = jnp.maximum(jnp.concatenate([m0, m[:, LANES:]], axis=1), mj)
                    m = mj
                    side(min(t_start + r0 + sub - 1, stop))
                st['clock'] += sc.shape[0]
            st['on'] = was
            return max_fin(m)

        def pv_unit(buf, m, u, kc, dur, ahead):
            cs = slice(u * LANES, (u + 1) * LANES)
            o = l = None
            for j in range(sk // kc):
                mu = after(m[:, cs], ahead)
                p = jnp.exp2(_by8(s_bufs[buf][0, j * kc:(j + 1) * kc, cs]) - mu[None])
                lj = jnp.sum(p.reshape(kc // lw, lw, LANES), axis=0)
                oj = jnp.dot(pltpu.bitcast(vt_scr[0, :, j * kc:(j + 1) * kc], BF16),
                             p.reshape(kc, LANES).astype(BF16),
                             preferred_element_type=F32)
                o = oj if o is None else o + oj
                l = lj if l is None else l + lj
                hist.append((st['clock'], DH, oj))
                st['clock'] += dur
                side()
            return (o / jnp.sum(l, axis=0, keepdims=True)).astype(BF16)

        def gather_out(outs):
            return jnp.concatenate(
                [jnp.concatenate(outs[r * nlt:(r + 1) * nlt], axis=1) for r in range(rep)], axis=0)

        def pv(buf, m):
            return gather_out([pv_unit(buf, m, u, kcp, kcp // 4, ahp) for u in range(4)])

        def pv_qk(buf, m, qn, nbuf):
            outs, mns = [], []
            for half in range(2):
                mns.append(qk_part(qn, nbuf, slice(0, sk), slice(half * 256, (half + 1) * 256), False))
                outs += [pv_unit(buf, m, u, 256, DH, ahead) for u in (2 * half, 2 * half + 1)]
            return gather_out(outs), max_fin(jnp.concatenate(mns, axis=1))

        def oproj(i, ot):
            cols = tcols(toks[i])
            mo = _Moments()
            for rb in range(d // oh):
                rows = slice(rb * oh, (rb + 1) * oh)
                res = jnp.dot(wot_ref[rows, :], ot, preferred_element_type=F32)
                tot = res if first else res + acc_scr[rows, cols]
                if last:
                    ln2_x1(toks[i], rows, tot, mo)
                else:
                    acc_scr[rows, cols] = tot
                step(res, oh)
            if last:
                ln2_stats(toks[i], mo)

        qs, ots, ms, bufs = {}, {}, {}, {}
        free = [0, 1]
        fresh()
        for item in sched.split():
            kind, arg = item[0], item[1:]
            if kind == '|':
                mark(arg)
                continue
            if kind == '!':
                hook()
                continue
            if kind == 'V':
                if vmode == 0:
                    vt_scr[0] = pltpu.bitcast(v_ref[...].T, F32)
                elif vmode == 1:
                    vt_scr[st['zero']] = pltpu.bitcast(v_ref[...].T, F32)
                else:
                    gen = vt_job(v_ref)
                    next(gen)
                    queue.insert(0, gen)
                continue
            if kind == '+':
                st['on'] = True
                st['nxt'] = max(st['nxt'], st['clock'])
                continue
            i = int(arg)
            if kind == 'Q':
                qs[i] = project_q(toks[i], wq_ref, step)
            elif kind == 'L':
                qs[i] = q_scr[toks[i]]
            elif kind == 'K':
                bufs[i] = free.pop(0)
                ms[i] = qk(qs[i], bufs[i])
            elif kind == 'P':
                ots[i] = pv(bufs[i], ms[i])
                free.append(bufs[i])
            elif kind == 'S':
                bufs[i + 1] = free.pop(0)
                ots[i], ms[i + 1] = pv_qk(bufs[i], ms[i], qs[i + 1], bufs[i + 1])
                free.append(bufs[i])
            elif kind == 'O':
                oproj(i, ots[i])
        drain()

    scope('p0_start')
    zv_scr[...] = jnp.zeros(zv_scr.shape, I32)
    cp_z = pltpu.make_async_copy(zv_scr, z_scr, msem.at[0])
    for cp in ((cp_z, cp_c, cp_x[0], cp_m0, cp_wql) + tuple(cp_x[1:]) + group_copies(0, 0)):
        cp.start()

    def zero_body(j, carry):
        acc_scr[pl.ds(pl.multiple_of(j * 64, 64), 64), :] = jnp.zeros((64, s_len), F32)
        return carry

    jax.lax.fori_loop(0, d // 64, zero_body, 0)
    xh_scr[d:2 * d, s_len - 2 * tg:s_len] = jnp.zeros((d, 2 * tg), BF16)
    st_scr[...] = jnp.zeros(st_scr.shape, F32)
    scope('p1_waitx')
    cp_z.wait()
    cp_x[0].wait()
    scope('p1_norm')
    per = xw // tg
    ys = {}
    for i in range(per):
        mo = _Moments()
        for r0 in range(0, d, 64):
            mo.add(xt_v[0, r0:r0 + 64, tcols(i)].astype(F32))
        mean, rinv = mo.stats(d)
        for lt in range(nlt):
            for rows in fch:
                ys[i, lt, rows.start] = ln1_norm_piece(i, lt, rows, mean, rinv)
    scope('p2_waitmod')
    cp_c.wait()
    cp_m0.wait()
    scope('p2_mod')
    mod = _rnd(jnp.dot(silu_c8(), wmod_v[:, 0:2 * d], preferred_element_type=F32))
    row_scr[0] = mod[:, 0:d]
    row_scr[1] = _rnd(1.0 + mod[:, d:2 * d])
    for i in range(per):
        for lt in range(nlt):
            for rows in fch:
                ln1_mod_piece(i, lt, rows, ys[i, lt, rows.start])
    scope('p3_ln1')

    cp_wql.wait()

    def ln1_body(j, carry):
        pltpu.make_async_copy(xt_hbm.at[:, 0:xw],
                              xt_v.at[0, :, pl.ds(pl.multiple_of((j + 1) * xw, xw), xw)],
                              msem.at[2 + j]).wait()
        base = j * per
        for i in range(per):
            q_scr[base + i] = project_q(base + i, wql_v)
        if l1mode == 0:
            for i in range(per):
                run_all(ln1_job(base + per + i, base + per + i))
        else:
            cols = pl.ds(pl.multiple_of(j * xw + xw, xw), xw)
            mo = _Moments()
            for r0 in range(0, d, 32):
                mo.add(xt_v[0, r0:r0 + 32, cols].astype(F32))
            mean, rinv = mo.stats(d)
            y = (_by8(xt_v[z_scr[0, 0], :, cols].astype(F32)) - mean[None]) * rinv[None]
            y = y.reshape(d, xw).astype(BF16).T
            h = y.astype(F32) * row_scr[1, 0:1, :] + row_scr[0, 0:1, :]
            h_scr[0, cols, :] = h.astype(BF16)
        return carry

    jax.lax.fori_loop(0, nxc - 1, ln1_body, 0)

    def mid_body(g, carry):
        slot = g & 1
        with (jax.named_scope('q1_wait') if prof else contextlib.nullcontext()):
            for cp in group_copies(g, slot):
                cp.wait()

        def prefetch():
            for cp in group_copies(g + 1, 1 - slot):
                cp.start()
            for j, cp in enumerate((cp_m1, cp_wr) + cp_moe):
                @pl.when(g == (1 + j if mid else 0))
                def _(cp=cp):
                    cp.start()

        if mid:
            with (jax.named_scope('q2_body') if prof else contextlib.nullcontext()):
                attn_group((wqbuf.at[slot], kbuf.at[slot], vbuf.at[slot], wobuf.at[slot]),
                           list(range(ng)), steady(ng), hook=prefetch)
        else:
            prefetch()
        return carry

    scope('q_loop')
    jax.lax.fori_loop(0, lastg, mid_body, 0)

    scope('r0_wait')
    ls = lastg % 2
    for cp in group_copies(lastg, ls) + (cp_m1, cp_wr) + cp_moe:
        cp.wait()
    scope('r0_mod2')
    mod = _rnd(jnp.dot(silu_c8(), wmod_v[:, 2 * d:6 * d], preferred_element_type=F32))
    piece = lambda j: mod[0:1, j * d:(j + 1) * d]
    rows5 = [piece(0), piece(1), _rnd(1.0 + piece(2)), piece(3), wr_v[...].astype(F32).reshape(1, d)]
    for j, row in enumerate(rows5):
        col_scr[j] = jnp.broadcast_to(row, (LANES, d)).T
    row_scr[2] = mod[:, 3 * d:4 * d]
    for i in range(ng - per, ng):
        q_scr[i] = project_q(i, wql_v)
    npair = ng // 2

    def last_body(t, carry):
        prev = (t + npair - 1) % npair
        attn_group((wqbuf.at[ls], kbuf.at[ls], vbuf.at[ls], wobuf.at[ls]),
                   [2 * t, 2 * t + 1], sched_l, last=True,
                   jobs=dict(a=[mix(chain(ln2_job(2 * prev), ln2_job(2 * prev + 1)),
                                    wd_job(t, npair), 4)]), dt=dt2)
        return carry

    scope('r1_last')
    jax.lax.fori_loop(0, npair, last_body, 0)
    scope('r1_ln2')
    run_all(ln2_job(ng - 2))
    run_all(ln2_job(ng - 1))

    scope('r2_topk')
    ibits = (s_len - 1).bit_length()
    imask = (1 << ibits) - 1
    bits = pltpu.bitcast(_rnd(r_scr[...]), I32)
    pos = (jax.lax.broadcasted_iota(I32, bits.shape, 0) * LANES
           + jax.lax.broadcasted_iota(I32, bits.shape, 1))
    order = ((bits ^ ((bits >> 31) & 0x7FFFFFFF)) >> 16) + 0x8000
    key = pltpu.bitcast((order << ibits) + (imask - pos) + 0x20000000, F32)
    sub = jax.lax.broadcasted_iota(I32, (TOPC, LANES), 0)
    lane = jax.lax.broadcasted_iota(I32, (TOPC, LANES), 1)
    idxs, blks = [], []
    keyv = jnp.zeros((TOPC, LANES), I32)
    xh_sel = jnp.zeros((TOPC, 2 * d), F32)
    for cidx in range(TOPC):
        top = jnp.max(jnp.max(key, axis=0, keepdims=True), axis=1, keepdims=True)
        key = jnp.where(key == top, 0.0, key)
        topi = pltpu.bitcast(jnp.broadcast_to(top, (TOPC, LANES)), I32)
        keyv = jnp.where(sub == cidx, topi, keyv)
        ixv = imask - (topi & imask)
        ix = ixv[0, 0]
        idxs.append(ix)
        blks.append(ix >> 7)
        cols = pl.ds(pl.multiple_of(blks[cidx] * LANES, LANES), LANES)
        oh1 = jnp.where((lane == (ixv & (LANES - 1))) & (sub == cidx), 1.0, 0.0).astype(BF16)
        xh_sel = xh_sel + jax.lax.dot_general(oh1, xh_scr[:, cols], NT, preferred_element_type=F32)

    for b in range(nblk):
        hit = blks[0] == b
        for bb in blks[1:]:
            hit = jnp.logical_or(hit, bb == b)

        @pl.when(jnp.logical_not(hit))
        def _(b=b):
            out_copy(b).start()

    uniq = []
    for cidx in range(TOPC):
        u = True
        for other in blks[cidx + 1:]:
            u = jnp.logical_and(u, other != blks[cidx])
        uniq.append(jnp.asarray(u))

    scope('r4_moe')
    x_sel = xh_sel[:, 0:d]
    x1_sel = xh_sel[:, d:2 * d]
    ob = (((keyv - 0x20000000) >> ibits) - 0x8000) << 16
    r_sel = pltpu.bitcast((ob ^ ((ob >> 31) & 0x7FFFFFFF)) & ~0xFFFF, F32)[:, 0:1]
    xs = x_sel.astype(BF16)
    gt = _rnd(jnp.dot(xs, wg_v[...], preferred_element_type=F32))
    gt = _rnd(gt * jax.nn.sigmoid(gt))
    up = _rnd(jnp.dot(xs, wu_v[...], preferred_element_type=F32))
    gu = (gt * up).astype(BF16)
    gate_r = _rnd(jax.nn.sigmoid(r_sel))
    out32 = out_v.bitcast(jnp.uint32)

    def down(fs):
        y = _rnd(jnp.dot(gu, pltpu.bitcast(wd_scr[:, fs], BF16), preferred_element_type=F32))
        y = _rnd(y * gate_r)
        return x1_sel[:, fs] + _rnd(row_scr[2, :, fs] * _rnd(x_sel[:, fs] + y))

    def patch(fs, new):
        n = fs.stop - fs.start
        newt = jnp.concatenate([new, jnp.zeros((LANES - TOPC, n), F32)], axis=0).astype(BF16).T
        newt32 = pltpu.bitcast(newt, jnp.uint32)
        lane_d = jax.lax.broadcasted_iota(I32, newt32.shape, 1)
        for cidx in range(TOPC):
            cols = pl.ds(pl.multiple_of(blks[cidx] * LANES, LANES), LANES)
            ln = idxs[cidx] & (LANES - 1)
            moved = pltpu.roll(newt32, (ln - cidx) & (LANES - 1), 1)
            pltpu.store(out32.at[fs.start // 2:fs.stop // 2, cols], moved, mask=lane_d == ln)

            @pl.when(uniq[cidx])
            def _(cols=cols):
                pltpu.make_async_copy(out_v.at[fs, cols], out_hbm.at[fs, cols], msem.at[1]).start()

    pch = [slice(a, b) for a, b in zip((0,) + cuts, cuts + (d,))]
    new_scr[:, pch[0]] = down(pch[0])
    scope('r5_patch')
    for j in range(len(pch)):
        @pl.when(z_scr[0, 0] == 0)
        def _(j=j):
            prev = new_scr[:, pch[j]]
            if j + 1 < len(pch):
                new_scr[:, pch[j + 1]] = down(pch[j + 1])
            patch(pch[j], prev)

    scope('r6_outwait')
    pltpu.make_async_copy(out_v, out_hbm, msem.at[1]).wait()
    es.close()


def build(ahead=384, qh=128, oh=144, lw=32, nf=3, prof=0, mid=1, dt1=48, dt2=80, dl=320, ra=96,
          ra2=64, rc2=32, marg=128, sub=64, spause=128, kcp=256, ahp=320, vmode=1, vch=256, l1mode=1, wpause=0, cuts=(256,), nochk=0,
          sched_f='|a Q0 Q1 |b K0 |c V Q2 P0 |d K1 K2 O0 P1 P2 O1 O2',
          sched_l='|a V L0 L1 K0 K1 P0 P1 O0 O1'):
    @jax.jit
    def fn(A_x, A_k_cache, A_v_cache, A_wq, A_wo, B_x, B_w_r, B_w_gate, B_w_up, B_w_down, c, w_mod):
        b, s_len, d = A_x.shape
        hkv, sk = A_k_cache.shape[1], A_k_cache.shape[2]
        rep = HQ // hkv
        f = B_w_gate.shape[1]
        xt = A_x.reshape(s_len, d).T
        k3 = A_k_cache.reshape(hkv, sk, DH)
        v3 = A_v_cache.reshape(hkv, sk, DH)
        nblk = s_len // LANES
        tg = GW // rep
        scratch = [
            pltpu.VMEM((1, d, s_len), BF16),
            pltpu.VMEM((2, sk, DH), BF16),
            pltpu.VMEM((2, sk, DH), BF16),
            pltpu.VMEM((2, d, rep * DH), BF16),
            pltpu.VMEM((2, d, rep * DH), BF16),
            pltpu.VMEM((d, rep * DH), BF16),
            pltpu.VMEM((s_len // tg, GW, DH), BF16),
            pltpu.VMEM((d,), BF16),
            pltpu.VMEM((1, d), BF16),
            pltpu.VMEM((d, 6 * d), BF16),
            pltpu.VMEM((d, f), BF16),
            pltpu.VMEM((d, f), BF16),
            pltpu.VMEM((d, f), BF16),
            pltpu.VMEM((f // 2, d), F32),
            pltpu.VMEM((d, s_len), BF16),
            pltpu.VMEM((1, s_len, d), BF16),
            pltpu.VMEM((d, s_len), F32),
            pltpu.VMEM((3, 8, d), F32),
            pltpu.VMEM((5, d, LANES), F32),
            pltpu.VMEM((1, DH // 2, sk), F32),
            pltpu.VMEM((2 * d, s_len), BF16),
            pltpu.VMEM((nblk, LANES), F32),
            pltpu.VMEM((2, 8, s_len), F32),
            pltpu.VMEM((1, sk, GW), F32),
            pltpu.VMEM((1, sk, GW), F32),
            pltpu.SMEM((8, LANES), I32),
            pltpu.VMEM((8, LANES), I32),
            pltpu.VMEM((TOPC, d), F32),
            pltpu.SemaphoreType.DMA((7,)),
        ]
        out = pl.pallas_call(
            functools.partial(_kernel, n_groups=hkv, rep=rep, ahead=ahead, qh=qh, oh=oh, lw=lw,
                              nf=nf, prof=prof, mid=mid, dt1=dt1, dt2=dt2, dl=dl, ra=ra, ra2=ra2, rc2=rc2,
                              marg=marg, sub=sub, spause=spause, sched_f=sched_f, sched_l=sched_l, kcp=kcp, ahp=ahp, vmode=vmode, vch=vch, l1mode=l1mode, wpause=wpause, cuts=cuts),
            in_specs=[pl.BlockSpec(memory_space=pl.ANY)] * 11,
            out_specs=pl.BlockSpec(memory_space=pl.ANY),
            out_shape=jax.ShapeDtypeStruct((d, s_len), BF16),
            scratch_shapes=scratch,
            compiler_params=pltpu.CompilerParams(vmem_limit_bytes=100 * 1024 * 1024,
                                                 disable_bounds_checks=bool(nochk)),
        )(xt, k3, v3, A_wq, A_wo.T, B_w_r, c, w_mod, B_w_gate, B_w_up, B_w_down.T)
        return out.T.reshape(b, s_len, d)
    return fn


pallas_adaLN_cond__gqa_block_cached__moe_arch_mod__prompt_kernel = build()
```

```python
import functools

import jax
import jax.numpy as jnp
import jax.experimental.pallas as pl
import jax.experimental.pallas.tpu as pltpu

HQ = 32
DH = 128
TOPC = 8
LN_EPS = 1.0013580322265625e-05
LOG2E = 1.4426950408889634
F32 = jnp.float32
BF16 = jnp.bfloat16
I32 = jnp.int32
NT = (((1,), (1,)), ((), ()))
LANES = 128
GW = 512
MXU_LAT = 128
NXC = 4


def _rnd(v):
    return v.astype(BF16).astype(F32)


def _by8(v):
    return v.reshape(v.shape[0] // 8, 8, v.shape[1])


class _Moments:
    def __init__(self):
        self.shift = self.s1 = self.s2 = None

    def add(self, v):
        if self.shift is None:
            self.shift = jnp.broadcast_to(v[0:1], (8, v.shape[1]))
        dv = _by8(v) - self.shift[None]
        a, b = jnp.sum(dv, axis=0), jnp.sum(dv * dv, axis=0)
        self.s1, self.s2 = (a, b) if self.s1 is None else (self.s1 + a, self.s2 + b)

    def stats(self, d):
        e1 = jnp.sum(self.s1, axis=0, keepdims=True) * (1.0 / d)
        e2 = jnp.sum(self.s2, axis=0, keepdims=True) * (1.0 / d)
        var = jnp.maximum(e2 - e1 * e1, 0.0)
        den = _rnd(jnp.sqrt(_rnd(_rnd(var) + LN_EPS)))
        return _rnd(self.shift + e1), jnp.broadcast_to(1.0 / den, self.shift.shape)


def _chain(*jobs):
    gate = yield
    for job in jobs:
        next(job)
        while True:
            try:
                v = job.send(gate)
            except StopIteration:
                break
            gate = yield v


def _mix(a, b, every):
    next(a)
    next(b)
    gate = yield
    n, live = 0, [a, b]
    while live:
        n += 1
        job = b if (b in live and (n % (every + 1) == 0 or a not in live)) else a
        try:
            v = job.send(gate)
        except StopIteration:
            live.remove(job)
            continue
        gate = yield v


def _finish(job):
    try:
        while True:
            job.send(lambda t: t)
    except StopIteration:
        pass


def _kernel(xt_hbm, k_hbm, v_hbm, wq_hbm, wot_hbm, wr_hbm, c_hbm, wmod_hbm,
            wg_hbm, wu_hbm, wdt_hbm,
            out_hbm,
            xt_v, kbuf, vbuf, wqbuf, wobuf, wql_v, q_scr,
            wr_v, c_v, wmod_v, wg_v, wu_v, wdt_v, wd_scr, out_v,
            h_scr, acc_scr, row_scr, col_scr, vt_scr, xh_scr, r_scr, st_scr, s0_scr, s1_scr,
            z_scr, zv_scr, new_scr, sem, *,
            n_groups, rep, ahead, ahp, kcp, oh, lw, dt, dl, rc2, marg, sub, cuts):
    _, d, s_len = xt_v.shape
    sk = kbuf.shape[1]
    gcols = rep * DH
    tg = GW // rep
    ng = s_len // tg
    nblk = s_len // LANES
    nlt = tg // LANES
    xw = s_len // NXC
    per = xw // tg
    lastg = n_groups - 1
    s_bufs = (s0_scr, s1_scr)
    qscale = (DH ** -0.5) * LOG2E

    def group_copies(g, slot):
        cols = pl.ds(pl.multiple_of(g * gcols, gcols), gcols)
        s = sem.at[NXC + 1 + slot]
        return (pltpu.make_async_copy(wq_hbm.at[:, cols], wqbuf.at[slot], s),
                pltpu.make_async_copy(k_hbm.at[g], kbuf.at[slot], s),
                pltpu.make_async_copy(v_hbm.at[g], vbuf.at[slot], s),
                pltpu.make_async_copy(wot_hbm.at[:, cols], wobuf.at[slot], s))

    def x_copy(j, s):
        cols = pl.ds(pl.multiple_of(j * xw, xw), xw)
        return pltpu.make_async_copy(xt_hbm.at[:, cols], xt_v.at[0, :, cols], sem.at[s])

    cp_z = pltpu.make_async_copy(zv_scr, z_scr, sem.at[0])
    cp_c = pltpu.make_async_copy(c_hbm, c_v, sem.at[1])
    cp_m0 = pltpu.make_async_copy(wmod_hbm.at[:, 0:2 * d], wmod_v.at[:, 0:2 * d], sem.at[1])
    cp_wql = pltpu.make_async_copy(wq_hbm.at[:, lastg * gcols:(lastg + 1) * gcols], wql_v,
                                   sem.at[2])
    cp_tail = (pltpu.make_async_copy(wmod_hbm.at[:, 2 * d:6 * d], wmod_v.at[:, 2 * d:6 * d],
                                     sem.at[0]),
               pltpu.make_async_copy(wr_hbm, wr_v, sem.at[0]),
               pltpu.make_async_copy(wg_hbm, wg_v, sem.at[0]),
               pltpu.make_async_copy(wu_hbm, wu_v, sem.at[0]),
               pltpu.make_async_copy(wdt_hbm, wdt_v, sem.at[0]))

    def out_start(rows, cols):
        pltpu.make_async_copy(out_v.at[rows, cols], out_hbm.at[rows, cols], sem.at[1]).start()

    def modulation(lo, hi):
        cf = c_v[...].astype(F32)
        sc = jnp.broadcast_to((cf * jax.nn.sigmoid(cf)).astype(BF16), (8, d))
        return _rnd(jnp.dot(sc, wmod_v[:, lo:hi], preferred_element_type=F32))

    def tspan(i, lo, n):
        if isinstance(i, int):
            return slice(i * tg + lo, i * tg + lo + n)
        return pl.ds(pl.multiple_of(i * tg + lo, n), n)

    def tcols(i):
        return tspan(i, 0, tg)

    def col(j, rows):
        return jnp.concatenate([col_scr[j, rows, :]] * nlt, axis=1)

    def ln1_norm(cols, n, rch):
        mo = _Moments()
        for r0 in range(0, d, rch):
            mo.add(xt_v[0, r0:r0 + rch, cols].astype(F32))
        mean, rinv = mo.stats(d)
        y = (_by8(xt_v[z_scr[0, 0], :, cols].astype(F32)) - mean[None]) * rinv[None]
        return y.reshape(d, n).astype(BF16).T

    def ln1_mod(rows, y):
        h = y.astype(F32) * row_scr[1, 0:1, :] + row_scr[0, 0:1, :]
        h_scr[rows, :] = h.astype(BF16)

    def project_q(tok, wq_ref, step=lambda *a: None):
        parts = []
        for lt in range(nlt):
            q = jnp.dot(h_scr[tspan(tok, lt * LANES, LANES), :], wq_ref[...],
                        preferred_element_type=F32)
            step(q, LANES * pl.cdiv(d, LANES) * rep // 4)
            parts.append((q * qscale).astype(BF16))
        return jnp.concatenate([p[:, r * DH:(r + 1) * DH] for r in range(rep) for p in parts],
                               axis=0)

    def ln2_job(i):
        gate = yield
        mean, rinv = st_scr[0, :, tcols(i)], st_scr[1, :, tcols(i)]
        racc = None
        for r0 in range(0, d, rc2):
            rows = slice(r0, r0 + rc2)
            x1 = xh_scr[d + r0:d + r0 + rc2, tcols(i)].astype(F32)
            xc = (_by8(x1) - gate(mean)[None]).reshape(x1.shape)
            y = _rnd((_by8(_rnd(xc)) * rinv[None]).reshape(x1.shape))
            h2b = (_rnd(y * col(2, rows)) + col(1, rows)).astype(BF16)
            h2 = h2b.astype(F32)
            xh_scr[rows, tcols(i)] = h2b
            out_v[rows, tcols(i)] = (x1 + col(3, rows) * h2).astype(BF16)
            part = jnp.sum(_by8(h2 * col(4, rows)), axis=0)
            racc = part if racc is None else racc + part
            if r0 + rc2 == d:
                r = jnp.sum(racc, axis=0, keepdims=True)
                for lt in range(nlt):
                    r_scr[pl.ds(i * nlt + lt, 1), :] = r[:, lt * LANES:(lt + 1) * LANES]
            gate = yield racc

    def wd_job(t, parts):
        gate = yield
        fw = wdt_v.shape[1] // parts
        for f0 in range(0, fw, LANES):
            lo = pl.multiple_of(t * fw + f0, LANES)
            w32 = pltpu.bitcast(wdt_v[:, pl.ds(lo, LANES)], I32)
            w32 = gate(_by8(w32)).reshape(w32.shape)
            wd = pltpu.bitcast(w32, BF16).T
            half = pl.multiple_of(t * (fw // 2) + f0 // 2, LANES // 2)
            wd_scr[pl.ds(half, LANES // 2), :] = pltpu.bitcast(wd, I32)
            gate = yield wd_scr[0:8, 0:LANES]

    def attention(slot, toks, sched, last=False, job=None, hook=None):
        wq_ref, k_ref, v_ref, wot_ref = (wqbuf.at[slot], kbuf.at[slot], vbuf.at[slot],
                                         wobuf.at[slot])
        zero = z_scr[0, 0]
        zvec = jnp.full((8, LANES), zero, I32)
        st = dict(clock=0, nxt=0, job=job)
        hist = []
        due = []
        if job is not None:
            next(job)

        def token(when):
            want = when - MXU_LAT
            for start, dur, res in reversed(hist):
                if start <= want:
                    row = min((want - start) * res.shape[0] // dur // 8 * 8, res.shape[0] - 8)
                    return pltpu.bitcast(res[row:row + 8, 0:LANES], I32) & zvec
            return None

        def tie(x, tok):
            if tok is None:
                return x
            if x.shape[-1] > LANES:
                tok = jnp.concatenate([tok] * (x.shape[-1] // LANES), axis=1)
            if x.ndim == 3:
                tok = tok[None]
            if x.dtype == I32:
                return x | tok
            return pltpu.bitcast(pltpu.bitcast(x, I32) | tok, x.dtype)

        def tie_due(x, now):
            while due and due[0][0] <= now:
                v = due.pop(0)[1]
                v = v if v.dtype == I32 else pltpu.bitcast(v, I32)
                bits = v[:, 0:LANES]
                for j in range(1, v.shape[1] // LANES):
                    bits = bits | v[:, j * LANES:(j + 1) * LANES]
                x = tie(x, bits & zvec)
            return x

        def side(upto):
            while st['job'] is not None and st['nxt'] <= upto:
                tok = token(st['nxt'] + MXU_LAT)
                try:
                    v = st['job'].send(lambda x, tok=tok: tie(x, tok))
                except StopIteration:
                    st['job'] = None
                    break
                due.append((st['nxt'] + dl, v))
                st['nxt'] += dt

        def step(result, dur, advance=None):
            hist.append((st['clock'], dur, result))
            st['clock'] += dur if advance is None else advance

        def scores(qg, buf, rows, cols, advance=None):
            s = jax.lax.dot_general(k_ref[rows, :], qg[cols], NT, preferred_element_type=F32)
            s_bufs[buf][zero, rows, cols] = s
            step(s, s.shape[0], advance)
            return s

        def max_fin(m):
            return jnp.broadcast_to(jnp.max(m, axis=0, keepdims=True), m.shape)

        def qk(qg, buf):
            m = None
            st['nxt'] = max(st['nxt'], st['clock'])
            stop = st['clock'] + sk - marg
            for j in range(4):
                t0 = st['clock']
                s = scores(qg, buf, slice(j * sk // 4, (j + 1) * sk // 4), slice(0, GW))
                blk = s.shape[0] if job is None else sub
                for r0 in range(0, s.shape[0], blk):
                    mj = jnp.max(_by8(s[r0:r0 + blk]), axis=0)
                    if m is not None:
                        m0 = tie_due(m[:, 0:LANES], t0 + r0)
                        mj = jnp.maximum(jnp.concatenate([m0, m[:, LANES:]], axis=1), mj)
                    m = mj
                    side(min(t0 + r0 + blk - 1, stop))
            return max_fin(m)

        def pv_unit(buf, m, u, kc, advance, lead):
            cs = slice(u * LANES, (u + 1) * LANES)
            o = l = None
            for j in range(sk // kc):
                when = st['clock'] - lead
                mu = tie_due(tie(m[:, cs], token(when)), when)
                p = jnp.exp2(_by8(s_bufs[buf][0, j * kc:(j + 1) * kc, cs]) - mu[None])
                lj = jnp.sum(p.reshape(kc // lw, lw, LANES), axis=0)
                oj = jnp.dot(pltpu.bitcast(vt_scr[0, :, j * kc:(j + 1) * kc], BF16),
                             p.reshape(kc, LANES).astype(BF16), preferred_element_type=F32)
                o = oj if o is None else o + oj
                l = lj if l is None else l + lj
                step(oj, DH, advance)
            return (o / jnp.sum(l, axis=0, keepdims=True)).astype(BF16)

        def heads_major(outs):
            return jnp.concatenate(
                [jnp.concatenate(outs[r * nlt:(r + 1) * nlt], axis=1) for r in range(rep)], axis=0)

        def pv(buf, m):
            return heads_major([pv_unit(buf, m, u, kcp, kcp // 4, ahp) for u in range(4)])

        def pv_qk(buf, m, qn, nbuf):
            outs, mns = [], []
            for half in range(2):
                s = scores(qn, nbuf, slice(0, sk), slice(half * GW // 2, (half + 1) * GW // 2), 0)
                mns.append(jnp.max(_by8(s), axis=0))
                outs += [pv_unit(buf, m, u, 2 * LANES, DH, ahead) for u in (2 * half, 2 * half + 1)]
            return heads_major(outs), max_fin(jnp.concatenate(mns, axis=1))

        def oproj(tok, ot):
            cols = tcols(tok)
            mo = _Moments()
            for r0 in range(0, d, oh):
                rows = slice(r0, r0 + oh)
                res = jnp.dot(wot_ref[rows, :], ot, preferred_element_type=F32)
                attn = res + acc_scr[rows, cols]
                if last:
                    x1b = (xt_v[0, rows, cols].astype(F32) + col(0, rows) * attn).astype(BF16)
                    xh_scr[d + r0:d + r0 + oh, cols] = x1b
                    mo.add(x1b.astype(F32))
                else:
                    acc_scr[rows, cols] = attn
                step(res, oh)
            if last:
                st_scr[0, :, cols], st_scr[1, :, cols] = mo.stats(d)

        qs, ots, ms, bufs, free = {}, {}, {}, {}, [0, 1]
        for item in sched.split():
            kind, i = item[0], int(item[1:] or 0)
            if kind == '!':
                hook()
            elif kind == 'V':
                vt_scr[zero] = pltpu.bitcast(v_ref[...].T, I32)
            elif kind == 'Q':
                qs[i] = project_q(toks[i], wq_ref, step)
            elif kind == 'L':
                qs[i] = q_scr[toks[i]]
            elif kind == 'K':
                bufs[i] = free.pop(0)
                ms[i] = qk(qs[i], bufs[i])
            elif kind == 'P':
                ots[i] = pv(bufs[i], ms[i])
                free.append(bufs[i])
            elif kind == 'S':
                bufs[i + 1] = free.pop(0)
                ots[i], ms[i + 1] = pv_qk(bufs[i], ms[i], qs[i + 1], bufs[i + 1])
                free.append(bufs[i])
            elif kind == 'O':
                oproj(toks[i], ots[i])
        if st['job'] is not None:
            _finish(st['job'])

    zv_scr[...] = jnp.zeros(zv_scr.shape, I32)
    for cp in ((cp_z, cp_c, x_copy(0, 0), cp_m0, cp_wql)
               + tuple(x_copy(j, j + 1) for j in range(1, NXC)) + group_copies(0, 0)):
        cp.start()

    def zero_body(j, carry):
        acc_scr[pl.ds(pl.multiple_of(j * 64, 64), 64), :] = jnp.zeros((64, s_len), F32)
        return carry

    jax.lax.fori_loop(0, d // 64, zero_body, 0)
    xh_scr[d:2 * d, s_len - 2 * tg:s_len] = jnp.zeros((d, 2 * tg), BF16)
    st_scr[...] = jnp.zeros(st_scr.shape, F32)
    cp_z.wait()
    x_copy(0, 0).wait()
    ys = [ln1_norm(tcols(i), tg, 64) for i in range(per)]
    cp_c.wait()
    cp_m0.wait()
    mod = modulation(0, 2 * d)
    row_scr[0] = mod[:, 0:d]
    row_scr[1] = _rnd(1.0 + mod[:, d:2 * d])
    for i in range(per):
        ln1_mod(tcols(i), ys[i])
    cp_wql.wait()

    def ln1_body(j, carry):
        x_copy(j + 1, j + 2).wait()
        for i in range(per):
            q_scr[j * per + i] = project_q(j * per + i, wql_v)
        cols = pl.ds(pl.multiple_of(j * xw + xw, xw), xw)
        ln1_mod(cols, ln1_norm(cols, xw, 32))
        return carry

    jax.lax.fori_loop(0, NXC - 1, ln1_body, 0)

    steady = 'V Q0 Q1 K0 ! ' + ' '.join(
        ('O%d ' % (i - 2) if i >= 2 else '') + ('Q%d ' % (i + 2) if i + 2 < ng else '')
        + ('S%d' % i if i + 1 < ng else 'P%d' % i) for i in range(ng)
    ) + ' O%d O%d' % (ng - 2, ng - 1)

    def group_body(g, carry):
        slot = g & 1
        for cp in group_copies(g, slot):
            cp.wait()

        def prefetch():
            for cp in group_copies(g + 1, 1 - slot):
                cp.start()
            for j, cp in enumerate(cp_tail):
                @pl.when(g == 1 + j)
                def _(cp=cp):
                    cp.start()

        attention(slot, list(range(ng)), steady, hook=prefetch)
        return carry
    jax.lax.fori_loop(0, lastg, group_body, 0)

    for cp in group_copies(lastg, lastg % 2) + cp_tail:
        cp.wait()
    mod = modulation(2 * d, 6 * d)
    piece = lambda j: mod[0:1, j * d:(j + 1) * d]
    for j, row in enumerate((piece(0), piece(1), _rnd(1.0 + piece(2)), piece(3),
                             wr_v[...].astype(F32).reshape(1, d))):
        col_scr[j] = jnp.broadcast_to(row, (LANES, d)).T
    row_scr[2] = mod[:, 3 * d:4 * d]
    for i in range(ng - per, ng):
        q_scr[i] = project_q(i, wql_v)
    npair = ng // 2

    def last_body(t, carry):
        prev = (t + npair - 1) % npair
        attention(lastg % 2, [2 * t, 2 * t + 1], 'V L0 L1 K0 K1 P0 P1 O0 O1', last=True,
                  job=_mix(_chain(ln2_job(2 * prev), ln2_job(2 * prev + 1)), wd_job(t, npair), 4))
        return carry
    jax.lax.fori_loop(0, npair, last_body, 0)
    rest = _chain(ln2_job(ng - 2), ln2_job(ng - 1))
    next(rest)
    _finish(rest)

    ibits = (s_len - 1).bit_length()
    imask = (1 << ibits) - 1
    bits = pltpu.bitcast(_rnd(r_scr[...]), I32)
    pos = (jax.lax.broadcasted_iota(I32, bits.shape, 0) * LANES
           + jax.lax.broadcasted_iota(I32, bits.shape, 1))
    order = ((bits ^ ((bits >> 31) & 0x7FFFFFFF)) >> 16) + 0x8000
    key = pltpu.bitcast((order << ibits) + (imask - pos) + 0x20000000, F32)
    subl = jax.lax.broadcasted_iota(I32, (TOPC, LANES), 0)
    lane = jax.lax.broadcasted_iota(I32, (TOPC, LANES), 1)
    idxs, blks, bcols = [], [], []
    keyv = jnp.zeros((TOPC, LANES), I32)
    xh_sel = jnp.zeros((TOPC, 2 * d), F32)
    for c in range(TOPC):
        top = jnp.max(jnp.max(key, axis=0, keepdims=True), axis=1, keepdims=True)
        key = jnp.where(key == top, 0.0, key)
        topi = pltpu.bitcast(jnp.broadcast_to(top, (TOPC, LANES)), I32)
        keyv = jnp.where(subl == c, topi, keyv)
        ixv = imask - (topi & imask)
        idxs.append(ixv[0, 0])
        blks.append(idxs[c] // LANES)
        bcols.append(pl.ds(pl.multiple_of(blks[c] * LANES, LANES), LANES))
        pick = jnp.where((lane == (ixv & (LANES - 1))) & (subl == c), 1.0, 0.0).astype(BF16)
        xh_sel = xh_sel + jax.lax.dot_general(pick, xh_scr[:, bcols[c]], NT,
                                              preferred_element_type=F32)

    for b in range(nblk):
        hit = blks[0] == b
        for bb in blks[1:]:
            hit = jnp.logical_or(hit, bb == b)

        @pl.when(jnp.logical_not(hit))
        def _(b=b):
            out_start(slice(0, d), slice(b * LANES, (b + 1) * LANES))

    final = []
    for c in range(TOPC):
        u = True
        for other in blks[c + 1:]:
            u = jnp.logical_and(u, other != blks[c])
        final.append(jnp.asarray(u))

    x_sel = xh_sel[:, 0:d]
    x1_sel = xh_sel[:, d:2 * d]
    ob = (((keyv - 0x20000000) >> ibits) - 0x8000) << 16
    r_sel = pltpu.bitcast((ob ^ ((ob >> 31) & 0x7FFFFFFF)) & ~0xFFFF, F32)[:, 0:1]
    xs = x_sel.astype(BF16)
    gt = _rnd(jnp.dot(xs, wg_v[...], preferred_element_type=F32))
    gt = _rnd(gt * jax.nn.sigmoid(gt))
    up = _rnd(jnp.dot(xs, wu_v[...], preferred_element_type=F32))
    gu = (gt * up).astype(BF16)
    gate_r = _rnd(jax.nn.sigmoid(r_sel))

    def down(fs):
        y = _rnd(jnp.dot(gu, pltpu.bitcast(wd_scr[:, fs], BF16), preferred_element_type=F32))
        y = _rnd(y * gate_r)
        return x1_sel[:, fs] + _rnd(row_scr[2, :, fs] * _rnd(x_sel[:, fs] + y))

    def patch(fs, new):
        n = fs.stop - fs.start
        newt = jnp.concatenate([new, jnp.zeros((LANES - TOPC, n), F32)], axis=0).astype(BF16).T
        newt32 = pltpu.bitcast(newt, I32)
        lane_d = jax.lax.broadcasted_iota(I32, newt32.shape, 1)
        for c in range(TOPC):
            ln = idxs[c] & (LANES - 1)
            moved = pltpu.roll(newt32, (ln - c) & (LANES - 1), 1)
            cur = pltpu.bitcast(out_v[fs, bcols[c]], I32)
            out_v[fs, bcols[c]] = pltpu.bitcast(jnp.where(lane_d == ln, moved, cur), BF16)

            @pl.when(final[c])
            def _(c=c):
                out_start(fs, bcols[c])

    pch = [slice(a, b) for a, b in zip((0,) + cuts, cuts + (d,))]
    new_scr[:, pch[0]] = down(pch[0])
    for j in range(len(pch)):
        @pl.when(z_scr[0, 0] == 0)
        def _(j=j):
            prev = new_scr[:, pch[j]]
            if j + 1 < len(pch):
                new_scr[:, pch[j + 1]] = down(pch[j + 1])
            patch(pch[j], prev)
    pltpu.make_async_copy(out_v, out_hbm, sem.at[1]).wait()


def _build(ahead=384, ahp=320, kcp=256, oh=144, lw=32, dt=80, dl=320, rc2=32,
          marg=128, sub=64, cuts=(384,)):
    @jax.jit
    def pallas_adaLN_cond__gqa_block_cached__moe_arch_mod__prompt_kernel(
            A_x, A_k_cache, A_v_cache, A_wq, A_wo, B_x, B_w_r, B_w_gate, B_w_up, B_w_down, c, w_mod):
        b, s_len, d = A_x.shape
        assert b == 1
        hkv, sk = A_k_cache.shape[1], A_k_cache.shape[2]
        rep = HQ // hkv
        f = B_w_gate.shape[1]
        tg = GW // rep
        scratch = [
            pltpu.VMEM((1, d, s_len), BF16),
            pltpu.VMEM((2, sk, DH), BF16),
            pltpu.VMEM((2, sk, DH), BF16),
            pltpu.VMEM((2, d, rep * DH), BF16),
            pltpu.VMEM((2, d, rep * DH), BF16),
            pltpu.VMEM((d, rep * DH), BF16),
            pltpu.VMEM((s_len // tg, GW, DH), BF16),
            pltpu.VMEM((d,), BF16),
            pltpu.VMEM((1, d), BF16),
            pltpu.VMEM((d, 6 * d), BF16),
            pltpu.VMEM((d, f), BF16),
            pltpu.VMEM((d, f), BF16),
            pltpu.VMEM((d, f), BF16),
            pltpu.VMEM((f // 2, d), I32),
            pltpu.VMEM((d, s_len), BF16),
            pltpu.VMEM((s_len, d), BF16),
            pltpu.VMEM((d, s_len), F32),
            pltpu.VMEM((3, 8, d), F32),
            pltpu.VMEM((5, d, LANES), F32),
            pltpu.VMEM((1, DH // 2, sk), I32),
            pltpu.VMEM((2 * d, s_len), BF16),
            pltpu.VMEM((s_len // LANES, LANES), F32),
            pltpu.VMEM((2, 8, s_len), F32),
            pltpu.VMEM((1, sk, GW), F32),
            pltpu.VMEM((1, sk, GW), F32),
            pltpu.SMEM((8, LANES), I32),
            pltpu.VMEM((8, LANES), I32),
            pltpu.VMEM((TOPC, d), F32),
            pltpu.SemaphoreType.DMA((NXC + 3,)),
        ]
        out = pl.pallas_call(
            functools.partial(_kernel, n_groups=hkv, rep=rep, ahead=ahead,
                              ahp=ahp, kcp=kcp, oh=oh, lw=lw, dt=dt, dl=dl, rc2=rc2, marg=marg,
                              sub=sub, cuts=cuts),
            in_specs=[pl.BlockSpec(memory_space=pl.ANY)] * 11,
            out_specs=pl.BlockSpec(memory_space=pl.ANY),
            out_shape=jax.ShapeDtypeStruct((d, s_len), BF16),
            scratch_shapes=scratch,
            compiler_params=pltpu.CompilerParams(vmem_limit_bytes=100 * 1024 * 1024),
        )(A_x.reshape(s_len, d).T, A_k_cache.reshape(hkv, sk, DH), A_v_cache.reshape(hkv, sk, DH),
          A_wq, A_wo.T, B_w_r, c, w_mod, B_w_gate, B_w_up, B_w_down.T)
        return out.T.reshape(b, s_len, d)
    return pallas_adaLN_cond__gqa_block_cached__moe_arch_mod__prompt_kernel


pallas_adaLN_cond__gqa_block_cached__moe_arch_mod__prompt_kernel = _build()
```

```python
import functools

import jax
import jax.numpy as jnp
import jax.experimental.pallas as pl
import jax.experimental.pallas.tpu as pltpu

HQ = 32
DH = 128
TOPC = 8
LN_EPS = 1.0013580322265625e-05
LOG2E = 1.4426950408889634
F32 = jnp.float32
BF16 = jnp.bfloat16
I32 = jnp.int32
NT = (((1,), (1,)), ((), ()))
LANES = 128
GW = 512
MXU_LAT = 128
NXC = 4


def _rnd(v):
    return v.astype(BF16).astype(F32)


def _by8(v):
    return v.reshape(v.shape[0] // 8, 8, v.shape[1])


class _Moments:
    def __init__(self):
        self.shift = self.s1 = self.s2 = None

    def add(self, v):
        if self.shift is None:
            self.shift = jnp.broadcast_to(v[0:1], (8, v.shape[1]))
        dv = _by8(v) - self.shift[None]
        a, b = jnp.sum(dv, axis=0), jnp.sum(dv * dv, axis=0)
        self.s1, self.s2 = (a, b) if self.s1 is None else (self.s1 + a, self.s2 + b)

    def stats(self, d):
        e1 = jnp.sum(self.s1, axis=0, keepdims=True) * (1.0 / d)
        e2 = jnp.sum(self.s2, axis=0, keepdims=True) * (1.0 / d)
        var = jnp.maximum(e2 - e1 * e1, 0.0)
        den = _rnd(jnp.sqrt(_rnd(_rnd(var) + LN_EPS)))
        return _rnd(self.shift + e1), jnp.broadcast_to(1.0 / den, self.shift.shape)


def _chain(*jobs):
    gate = yield
    for job in jobs:
        next(job)
        while True:
            try:
                v = job.send(gate)
            except StopIteration:
                break
            gate = yield v


def _mix(a, b, every):
    next(a)
    next(b)
    gate = yield
    n, live = 0, [a, b]
    while live:
        n += 1
        job = b if (b in live and (n % (every + 1) == 0 or a not in live)) else a
        try:
            v = job.send(gate)
        except StopIteration:
            live.remove(job)
            continue
        gate = yield v


def _finish(job):
    try:
        while True:
            job.send(lambda t: t)
    except StopIteration:
        pass


def _kernel(xt_hbm, k_hbm, v_hbm, wq_hbm, wot_hbm, wr_hbm, c_hbm, wmod_hbm,
            wg_hbm, wu_hbm, wdt_hbm,
            out_hbm,
            xt_v, kbuf, vbuf, wqbuf, wobuf, wql_v, q_scr,
            wr_v, c_v, wmod_v, wg_v, wu_v, wdt_v, wd_scr, out_v,
            h_scr, acc_scr, row_scr, col_scr, vt_scr, xh_scr, r_scr, st_scr, s0_scr, s1_scr,
            z_scr, zv_scr, new_scr, cc_scr, mod_scr, sem, *,
            n_groups, rep, ahead, ahp, kcp, oh, lw, dt, dl, rc2, marg, sub, cuts,
            mrows, dtm):
    _, d, s_len = xt_v.shape
    sk = kbuf.shape[1]
    gcols = rep * DH
    tg = GW // rep
    ng = s_len // tg
    nblk = s_len // LANES
    nlt = tg // LANES
    xw = s_len // NXC
    per = xw // tg
    lastg = n_groups - 1
    s_bufs = (s0_scr, s1_scr)
    qscale = (DH ** -0.5) * LOG2E

    def group_copies(g, slot):
        cols = pl.ds(pl.multiple_of(g * gcols, gcols), gcols)
        s = sem.at[NXC + 1 + slot]
        return (pltpu.make_async_copy(wq_hbm.at[:, cols], wqbuf.at[slot], s),
                pltpu.make_async_copy(k_hbm.at[g], kbuf.at[slot], s),
                pltpu.make_async_copy(v_hbm.at[g], vbuf.at[slot], s),
                pltpu.make_async_copy(wot_hbm.at[:, cols], wobuf.at[slot], s))

    def x_copy(j, s):
        cols = pl.ds(pl.multiple_of(j * xw, xw), xw)
        return pltpu.make_async_copy(xt_hbm.at[:, cols], xt_v.at[0, :, cols], sem.at[s])

    cp_z = pltpu.make_async_copy(zv_scr, z_scr, sem.at[0])
    cp_c = pltpu.make_async_copy(c_hbm, c_v, sem.at[0])
    cp_m0 = pltpu.make_async_copy(wmod_hbm.at[:, 0:2 * d], wmod_v.at[:, 0:2 * d], sem.at[1])
    cp_wql = pltpu.make_async_copy(wq_hbm.at[:, lastg * gcols:(lastg + 1) * gcols], wql_v,
                                   sem.at[2])
    cp_m1 = pltpu.make_async_copy(wmod_hbm.at[:, 2 * d:6 * d], wmod_v.at[:, 2 * d:6 * d], sem.at[2])
    cp_tail = (pltpu.make_async_copy(wr_hbm, wr_v, sem.at[0]),
               pltpu.make_async_copy(wg_hbm, wg_v, sem.at[0]),
               pltpu.make_async_copy(wu_hbm, wu_v, sem.at[0]),
               pltpu.make_async_copy(wdt_hbm, wdt_v, sem.at[0]))

    def out_start(rows, cols):
        pltpu.make_async_copy(out_v.at[rows, cols], out_hbm.at[rows, cols], sem.at[1]).start()

    def silu_c():
        cf = c_v[...].astype(F32)
        return (cf * jax.nn.sigmoid(cf)).astype(BF16)

    def mod_job(g):
        gate = yield
        mw = 2 * LANES
        lo = jnp.where(g < 2, 0, 2 * d + mw * jnp.minimum(g - 2, 4 * d // mw - 1))
        cols = pl.ds(pl.multiple_of(lo, LANES), mw)
        acc = jnp.zeros((8, mw), F32)
        for r0 in range(0, d, mrows):
            cc = jnp.concatenate([cc_scr[r0:r0 + mrows, :]] * 2, axis=1)
            prod = _by8(wmod_v[r0:r0 + mrows, cols].astype(F32) * cc)
            acc = gate(acc) + jnp.sum(prod, axis=0)
            if r0 + mrows == d:
                mod_scr[:, cols] = jnp.broadcast_to(jnp.sum(acc, axis=0, keepdims=True), (8, mw))
            gate = yield acc

    def tspan(i, lo, n):
        if isinstance(i, int):
            return slice(i * tg + lo, i * tg + lo + n)
        return pl.ds(pl.multiple_of(i * tg + lo, n), n)

    def tcols(i):
        return tspan(i, 0, tg)

    def col(j, rows):
        return jnp.concatenate([col_scr[j, rows, :]] * nlt, axis=1)

    def ln1_norm(cols, n, rch):
        mo = _Moments()
        for r0 in range(0, d, rch):
            mo.add(xt_v[0, r0:r0 + rch, cols].astype(F32))
        mean, rinv = mo.stats(d)
        y = (_by8(xt_v[z_scr[0, 0], :, cols].astype(F32)) - mean[None]) * rinv[None]
        return y.reshape(d, n).astype(BF16).T

    def ln1_mod(rows, y):
        h = y.astype(F32) * row_scr[1, 0:1, :] + row_scr[0, 0:1, :]
        h_scr[rows, :] = h.astype(BF16)

    def project_q(tok, wq_ref, step=lambda *a: None):
        parts = []
        for lt in range(nlt):
            q = jnp.dot(h_scr[tspan(tok, lt * LANES, LANES), :], wq_ref[...],
                        preferred_element_type=F32)
            step(q, LANES * pl.cdiv(d, LANES) * rep // 4)
            parts.append((q * qscale).astype(BF16))
        return jnp.concatenate([p[:, r * DH:(r + 1) * DH] for r in range(rep) for p in parts],
                               axis=0)

    def ln2_job(i):
        gate = yield
        mo = _Moments()
        mo.shift, mo.s1, mo.s2 = (st_scr[j, :, tcols(i)] for j in range(3))
        mean, rinv = mo.stats(d)
        racc = None
        for r0 in range(0, d, rc2):
            rows = slice(r0, r0 + rc2)
            x1 = xh_scr[d + r0:d + r0 + rc2, tcols(i)].astype(F32)
            xc = (_by8(x1) - gate(mean)[None]).reshape(x1.shape)
            y = _rnd((_by8(_rnd(xc)) * rinv[None]).reshape(x1.shape))
            h2b = (_rnd(y * col(2, rows)) + col(1, rows)).astype(BF16)
            h2 = h2b.astype(F32)
            xh_scr[rows, tcols(i)] = h2b
            out_v[rows, tcols(i)] = (x1 + col(3, rows) * h2).astype(BF16)
            part = jnp.sum(_by8(h2 * col(4, rows)), axis=0)
            racc = part if racc is None else racc + part
            if r0 + rc2 == d:
                r = jnp.sum(racc, axis=0, keepdims=True)
                for lt in range(nlt):
                    r_scr[pl.ds(i * nlt + lt, 1), :] = r[:, lt * LANES:(lt + 1) * LANES]
            gate = yield racc

    def wd_job(t, parts):
        gate = yield
        fw = wdt_v.shape[1] // parts
        for f0 in range(0, fw, LANES):
            lo = pl.multiple_of(t * fw + f0, LANES)
            w32 = pltpu.bitcast(wdt_v[:, pl.ds(lo, LANES)], I32)
            w32 = gate(_by8(w32)).reshape(w32.shape)
            wd = pltpu.bitcast(w32, BF16).T
            half = pl.multiple_of(t * (fw // 2) + f0 // 2, LANES // 2)
            wd_scr[pl.ds(half, LANES // 2), :] = pltpu.bitcast(wd, I32)
            gate = yield wd_scr[0:8, 0:LANES]

    def attention(slot, toks, sched, last=False, job=None, hook=None, dt=dt):
        wq_ref, k_ref, v_ref, wot_ref = (wqbuf.at[slot], kbuf.at[slot], vbuf.at[slot],
                                         wobuf.at[slot])
        zero = z_scr[0, 0]
        zvec = jnp.full((8, LANES), zero, I32)
        st = dict(clock=0, nxt=0, job=job)
        hist = []
        due = []
        if job is not None:
            next(job)

        def token(when):
            want = when - MXU_LAT
            for start, dur, res in reversed(hist):
                if start <= want:
                    row = min((want - start) * res.shape[0] // dur // 8 * 8, res.shape[0] - 8)
                    return pltpu.bitcast(res[row:row + 8, 0:LANES], I32) & zvec
            return None

        def tie(x, tok):
            if tok is None:
                return x
            if x.shape[-1] > LANES:
                tok = jnp.concatenate([tok] * (x.shape[-1] // LANES), axis=1)
            if x.ndim == 3:
                tok = tok[None]
            if x.dtype == I32:
                return x | tok
            return pltpu.bitcast(pltpu.bitcast(x, I32) | tok, x.dtype)

        def tie_due(x, now):
            while due and due[0][0] <= now:
                v = due.pop(0)[1]
                v = v if v.dtype == I32 else pltpu.bitcast(v, I32)
                bits = v[:, 0:LANES]
                for j in range(1, v.shape[1] // LANES):
                    bits = bits | v[:, j * LANES:(j + 1) * LANES]
                x = tie(x, bits & zvec)
            return x

        def side(upto):
            while st['job'] is not None and st['nxt'] <= upto:
                tok = token(st['nxt'] + MXU_LAT)
                try:
                    v = st['job'].send(lambda x, tok=tok: tie(x, tok))
                except StopIteration:
                    st['job'] = None
                    break
                due.append((st['nxt'] + dl, v))
                st['nxt'] += dt

        def step(result, dur, advance=None):
            hist.append((st['clock'], dur, result))
            st['clock'] += dur if advance is None else advance

        def scores(qg, buf, rows, cols, advance=None):
            s = jax.lax.dot_general(k_ref[rows, :], qg[cols], NT, preferred_element_type=F32)
            s_bufs[buf][zero, rows, cols] = s
            step(s, s.shape[0], advance)
            return s

        def max_fin(m):
            return jnp.broadcast_to(jnp.max(m, axis=0, keepdims=True), m.shape)

        def qk(qg, buf):
            m = None
            st['nxt'] = max(st['nxt'], st['clock'])
            stop = st['clock'] + sk - marg
            for j in range(4):
                t0 = st['clock']
                s = scores(qg, buf, slice(j * sk // 4, (j + 1) * sk // 4), slice(0, GW))
                blk = s.shape[0] if job is None else sub
                for r0 in range(0, s.shape[0], blk):
                    mj = jnp.max(_by8(s[r0:r0 + blk]), axis=0)
                    if m is not None:
                        m0 = tie_due(m[:, 0:LANES], t0 + r0)
                        mj = jnp.maximum(jnp.concatenate([m0, m[:, LANES:]], axis=1), mj)
                    m = mj
                    side(min(t0 + r0 + blk - 1, stop))
            return max_fin(m)

        def pv_unit(buf, m, u, kc, advance, lead):
            cs = slice(u * LANES, (u + 1) * LANES)
            o = l = None
            for j in range(sk // kc):
                when = st['clock'] - lead
                mu = tie_due(tie(m[:, cs], token(when)), when)
                p = jnp.exp2(_by8(s_bufs[buf][0, j * kc:(j + 1) * kc, cs]) - mu[None])
                lj = jnp.sum(p.reshape(kc // lw, lw, LANES), axis=0)
                oj = jnp.dot(pltpu.bitcast(vt_scr[0, :, j * kc:(j + 1) * kc], BF16),
                             p.reshape(kc, LANES).astype(BF16), preferred_element_type=F32)
                o = oj if o is None else o + oj
                l = lj if l is None else l + lj
                step(oj, DH, advance)
            return (o / jnp.sum(l, axis=0, keepdims=True)).astype(BF16)

        def heads_major(outs):
            return jnp.concatenate(
                [jnp.concatenate(outs[r * nlt:(r + 1) * nlt], axis=1) for r in range(rep)], axis=0)

        def pv(buf, m):
            return heads_major([pv_unit(buf, m, u, kcp, kcp // 4, ahp) for u in range(4)])

        def pv_qk(buf, m, qn, nbuf):
            outs, mns = [], []
            for half in range(2):
                s = scores(qn, nbuf, slice(0, sk), slice(half * GW // 2, (half + 1) * GW // 2), 0)
                mns.append(jnp.max(_by8(s), axis=0))
                outs += [pv_unit(buf, m, u, 2 * LANES, DH, ahead) for u in (2 * half, 2 * half + 1)]
            return heads_major(outs), max_fin(jnp.concatenate(mns, axis=1))

        def oproj(tok, ot):
            cols = tcols(tok)
            mo = _Moments()
            for r0 in range(0, d, oh):
                rows = slice(r0, r0 + oh)
                res = jnp.dot(wot_ref[rows, :], ot, preferred_element_type=F32)
                attn = res + acc_scr[rows, cols]
                if last:
                    x1b = (xt_v[0, rows, cols].astype(F32) + col(0, rows) * attn).astype(BF16)
                    xh_scr[d + r0:d + r0 + oh, cols] = x1b
                    mo.add(x1b.astype(F32))
                else:
                    acc_scr[rows, cols] = attn
                step(res, oh)
            if last:
                for j, v in enumerate((mo.shift, mo.s1, mo.s2)):
                    st_scr[j, :, cols] = v

        qs, ots, ms, bufs, free = {}, {}, {}, {}, [0, 1]
        for item in sched.split():
            kind, i = item[0], int(item[1:] or 0)
            if kind == '!':
                hook()
            elif kind == 'V':
                vt_scr[zero] = pltpu.bitcast(v_ref[...].T, I32)
            elif kind == 'Q':
                qs[i] = project_q(toks[i], wq_ref, step)
            elif kind == 'L':
                qs[i] = q_scr[toks[i]]
            elif kind == 'K':
                bufs[i] = free.pop(0)
                ms[i] = qk(qs[i], bufs[i])
            elif kind == 'P':
                ots[i] = pv(bufs[i], ms[i])
                free.append(bufs[i])
            elif kind == 'S':
                bufs[i + 1] = free.pop(0)
                ots[i], ms[i + 1] = pv_qk(bufs[i], ms[i], qs[i + 1], bufs[i + 1])
                free.append(bufs[i])
            elif kind == 'O':
                oproj(toks[i], ots[i])
        if st['job'] is not None:
            _finish(st['job'])

    zv_scr[...] = jnp.zeros(zv_scr.shape, I32)
    for cp in ((cp_z, cp_c, x_copy(0, 0), cp_m0, cp_wql)
               + tuple(x_copy(j, j + 1) for j in range(1, NXC)) + group_copies(0, 0)):
        cp.start()

    def zero_body(j, carry):
        rows = pl.ds(pl.multiple_of(j * 32, 32), 32)
        acc_scr[rows, :] = jnp.zeros((32, s_len), F32)
        xh_scr[pl.ds(pl.multiple_of(d + j * 32, 32), 32), s_len - 2 * tg:s_len] = (
            jnp.zeros((32, 2 * tg), BF16))
        return carry

    jax.lax.fori_loop(0, d // 32, zero_body, 0)
    st_scr[:, :, s_len - 2 * tg:s_len] = jnp.zeros((3, 8, 2 * tg), F32)
    cp_z.wait()
    cp_c.wait()
    x_copy(0, 0).wait()

    def norm_body(i, carry):
        h_scr[tcols(i), :] = ln1_norm(tcols(i), tg, 64)
        return carry

    jax.lax.fori_loop(0, per, norm_body, 0)
    cc_scr[...] = jnp.broadcast_to(silu_c(), (LANES, d)).T.astype(F32)
    cp_m0.wait()
    mod = _rnd(jnp.dot(jnp.broadcast_to(silu_c(), (8, d)), wmod_v[:, 0:2 * d],
                       preferred_element_type=F32))
    row_scr[0] = mod[:, 0:d]
    row_scr[1] = _rnd(1.0 + mod[:, d:2 * d])

    def mod_body(i, carry):
        rows = pl.ds(pl.multiple_of(i * LANES, LANES), LANES)
        ln1_mod(rows, h_scr[rows, :])
        return carry

    jax.lax.fori_loop(0, xw // LANES, mod_body, 0)
    cp_wql.wait()

    def ln1_body(j, carry):
        x_copy(j + 1, j + 2).wait()
        for i in range(per):
            q_scr[j * per + i] = project_q(j * per + i, wql_v)
        cols = pl.ds(pl.multiple_of(j * xw + xw, xw), xw)
        ln1_mod(cols, ln1_norm(cols, xw, 32))
        return carry

    jax.lax.fori_loop(0, NXC - 1, ln1_body, 0)

    steady = 'V Q0 Q1 K0 ! ' + ' '.join(
        ('O%d ' % (i - 2) if i >= 2 else '') + ('Q%d ' % (i + 2) if i + 2 < ng else '')
        + ('S%d' % i if i + 1 < ng else 'P%d' % i) for i in range(ng)
    ) + ' O%d O%d' % (ng - 2, ng - 1)

    def group_body(g, carry):
        slot = g & 1
        for cp in group_copies(g, slot):
            cp.wait()

        @pl.when(g == 2)
        def _():
            cp_m1.wait()

        def prefetch():
            for cp in group_copies(g + 1, 1 - slot):
                cp.start()
            for j, cp in enumerate((cp_m1,) + cp_tail):
                @pl.when(g == j)
                def _(cp=cp):
                    cp.start()

        attention(slot, list(range(ng)), steady, hook=prefetch, job=mod_job(g), dt=dtm)
        return carry
    jax.lax.fori_loop(0, lastg, group_body, 0)

    for cp in group_copies(lastg, lastg % 2) + cp_tail:
        cp.wait()
    mod = _rnd(mod_scr[:, 2 * d:6 * d])
    piece = lambda j: mod[0:1, j * d:(j + 1) * d]
    for j, row in enumerate((piece(0), piece(1), _rnd(1.0 + piece(2)), piece(3),
                             wr_v[...].astype(F32).reshape(1, d))):
        col_scr[j] = jnp.broadcast_to(row, (LANES, d)).T
    row_scr[2] = mod[:, 3 * d:4 * d]
    for i in range(ng - per, ng):
        q_scr[i] = project_q(i, wql_v)
    npair = ng // 2

    def last_body(t, carry):
        prev = (t + npair - 1) % npair
        attention(lastg % 2, [2 * t, 2 * t + 1], 'V L0 L1 K0 K1 P0 P1 O0 O1', last=True,
                  job=_mix(_chain(ln2_job(2 * prev), ln2_job(2 * prev + 1)), wd_job(t, npair), 4))
        return carry
    jax.lax.fori_loop(0, npair, last_body, 0)
    rest = _chain(ln2_job(ng - 2), ln2_job(ng - 1))
    next(rest)
    _finish(rest)

    ibits = (s_len - 1).bit_length()
    imask = (1 << ibits) - 1
    bits = pltpu.bitcast(_rnd(r_scr[...]), I32)
    pos = (jax.lax.broadcasted_iota(I32, bits.shape, 0) * LANES
           + jax.lax.broadcasted_iota(I32, bits.shape, 1))
    order = ((bits ^ ((bits >> 31) & 0x7FFFFFFF)) >> 16) + 0x8000
    key = pltpu.bitcast((order << ibits) + (imask - pos) + 0x20000000, F32)
    subl = jax.lax.broadcasted_iota(I32, (TOPC, LANES), 0)
    lane = jax.lax.broadcasted_iota(I32, (TOPC, LANES), 1)
    idxs, blks, bcols = [], [], []
    keyv = jnp.zeros((TOPC, LANES), I32)
    x_sel = jnp.zeros((TOPC, d), F32)
    x1_sel = jnp.zeros((TOPC, d), F32)
    for c in range(TOPC):
        top = jnp.max(jnp.max(key, axis=0, keepdims=True), axis=1, keepdims=True)
        key = jnp.where(key == top, 0.0, key)
        topi = pltpu.bitcast(jnp.broadcast_to(top, (TOPC, LANES)), I32)
        keyv = jnp.where(subl == c, topi, keyv)
        ixv = imask - (topi & imask)
        idxs.append(ixv[0, 0])
        blks.append(idxs[c] // LANES)
        bcols.append(pl.ds(pl.multiple_of(blks[c] * LANES, LANES), LANES))
        pick = jnp.where((lane == (ixv & (LANES - 1))) & (subl == c), 1.0, 0.0).astype(BF16)
        x_sel = x_sel + jax.lax.dot_general(pick, xh_scr[0:d, bcols[c]], NT,
                                            preferred_element_type=F32)
        x1_sel = x1_sel + jax.lax.dot_general(pick, xh_scr[d:2 * d, bcols[c]], NT,
                                              preferred_element_type=F32)

    for b in range(nblk):
        hit = blks[0] == b
        for bb in blks[1:]:
            hit = jnp.logical_or(hit, bb == b)

        @pl.when(jnp.logical_not(hit))
        def _(b=b):
            out_start(slice(0, d), slice(b * LANES, (b + 1) * LANES))

    final = []
    for c in range(TOPC):
        u = True
        for other in blks[c + 1:]:
            u = jnp.logical_and(u, other != blks[c])
        final.append(jnp.asarray(u))

    ob = (((keyv - 0x20000000) >> ibits) - 0x8000) << 16
    r_sel = pltpu.bitcast((ob ^ ((ob >> 31) & 0x7FFFFFFF)) & ~0xFFFF, F32)
    xs = x_sel.astype(BF16)
    gt = _rnd(jnp.dot(xs, wg_v[...], preferred_element_type=F32))
    gt = _rnd(gt * jax.nn.sigmoid(gt))
    up = _rnd(jnp.dot(xs, wu_v[...], preferred_element_type=F32))
    gu = (gt * up).astype(BF16)
    gate_r = jnp.concatenate([_rnd(jax.nn.sigmoid(r_sel))] * pl.cdiv(d, LANES), axis=1)

    def down(fs):
        y = _rnd(jnp.dot(gu, pltpu.bitcast(wd_scr[:, fs], BF16), preferred_element_type=F32))
        y = _rnd(y * gate_r[:, fs])
        return x1_sel[:, fs] + _rnd(row_scr[2, :, fs] * _rnd(x_sel[:, fs] + y))

    def patch(fs, new):
        n = fs.stop - fs.start
        lane_d = jax.lax.broadcasted_iota(I32, (n // 2, LANES), 1)
        for c in range(TOPC):
            ln = idxs[c] & (LANES - 1)
            wide = jnp.broadcast_to(new[c:c + 1], (LANES, n)).astype(BF16).T
            moved = pltpu.bitcast(wide, I32)
            cur = pltpu.bitcast(out_v[fs, bcols[c]], I32)
            out_v[fs, bcols[c]] = pltpu.bitcast(jnp.where(lane_d == ln, moved, cur), BF16)

            @pl.when(final[c])
            def _(c=c):
                out_start(fs, bcols[c])

    pch = [slice(a, b) for a, b in zip((0,) + cuts, cuts + (d,))]
    new_scr[:, pch[0]] = down(pch[0])
    for j in range(len(pch)):
        @pl.when(z_scr[0, 0] == 0)
        def _(j=j):
            prev = new_scr[:, pch[j]]
            if j + 1 < len(pch):
                new_scr[:, pch[j + 1]] = down(pch[j + 1])
            patch(pch[j], prev)
    pltpu.make_async_copy(out_v, out_hbm, sem.at[1]).wait()


def _build(ahead=384, ahp=320, kcp=256, oh=144, lw=32, dt=80, dl=320, rc2=32,
          marg=128, sub=64, cuts=(256, 512), mrows=64, dtm=160):
    @jax.jit
    def pallas_adaLN_cond__gqa_block_cached__moe_arch_mod__prompt_kernel(
            A_x, A_k_cache, A_v_cache, A_wq, A_wo, B_x, B_w_r, B_w_gate, B_w_up, B_w_down, c, w_mod):
        b, s_len, d = A_x.shape
        assert b == 1
        hkv, sk = A_k_cache.shape[1], A_k_cache.shape[2]
        rep = HQ // hkv
        f = B_w_gate.shape[1]
        tg = GW // rep
        scratch = [
            pltpu.VMEM((1, d, s_len), BF16),
            pltpu.VMEM((2, sk, DH), BF16),
            pltpu.VMEM((2, sk, DH), BF16),
            pltpu.VMEM((2, d, rep * DH), BF16),
            pltpu.VMEM((2, d, rep * DH), BF16),
            pltpu.VMEM((d, rep * DH), BF16),
            pltpu.VMEM((s_len // tg, GW, DH), BF16),
            pltpu.VMEM((d,), BF16),
            pltpu.VMEM((1, d), BF16),
            pltpu.VMEM((d, 6 * d), BF16),
            pltpu.VMEM((d, f), BF16),
            pltpu.VMEM((d, f), BF16),
            pltpu.VMEM((d, f), BF16),
            pltpu.VMEM((f // 2, d), I32),
            pltpu.VMEM((d, s_len), BF16),
            pltpu.VMEM((s_len, d), BF16),
            pltpu.VMEM((d, s_len), F32),
            pltpu.VMEM((3, 8, d), F32),
            pltpu.VMEM((5, d, LANES), F32),
            pltpu.VMEM((1, DH // 2, sk), I32),
            pltpu.VMEM((2 * d, s_len), BF16),
            pltpu.VMEM((s_len // LANES, LANES), F32),
            pltpu.VMEM((3, 8, s_len), F32),
            pltpu.VMEM((1, sk, GW), F32),
            pltpu.VMEM((1, sk, GW), F32),
            pltpu.SMEM((8, LANES), I32),
            pltpu.VMEM((8, LANES), I32),
            pltpu.VMEM((TOPC, d), F32),
            pltpu.VMEM((d, LANES), F32),
            pltpu.VMEM((8, 6 * d), F32),
            pltpu.SemaphoreType.DMA((NXC + 3,)),
        ]
        out = pl.pallas_call(
            functools.partial(_kernel, n_groups=hkv, rep=rep, ahead=ahead,
                              ahp=ahp, kcp=kcp, oh=oh, lw=lw, dt=dt, dl=dl, rc2=rc2, marg=marg,
                              sub=sub, cuts=cuts, mrows=mrows, dtm=dtm),
            in_specs=[pl.BlockSpec(memory_space=pl.ANY)] * 11,
            out_specs=pl.BlockSpec(memory_space=pl.ANY),
            out_shape=jax.ShapeDtypeStruct((d, s_len), BF16),
            scratch_shapes=scratch,
            compiler_params=pltpu.CompilerParams(vmem_limit_bytes=100 * 1024 * 1024),
        )(A_x.reshape(s_len, d).T, A_k_cache.reshape(hkv, sk, DH), A_v_cache.reshape(hkv, sk, DH),
          A_wq, A_wo.T, B_w_r, c, w_mod, B_w_gate, B_w_up, B_w_down.T)
        return out.T.reshape(b, s_len, d)
    return pallas_adaLN_cond__gqa_block_cached__moe_arch_mod__prompt_kernel


pallas_adaLN_cond__gqa_block_cached__moe_arch_mod__prompt_kernel = _build()
```

```python
import functools

import jax
import jax.numpy as jnp
import jax.experimental.pallas as pl
import jax.experimental.pallas.tpu as pltpu

HQ = 32
DH = 128
TOPC = 8
LN_EPS = 1.0013580322265625e-05
LOG2E = 1.4426950408889634
F32 = jnp.float32
BF16 = jnp.bfloat16
I32 = jnp.int32
NT = (((1,), (1,)), ((), ()))
LANES = 128
GW = 512
MXU_LAT = 128
NXC = 4


def _rnd(v):
    return v.astype(BF16).astype(F32)


def _by8(v):
    return v.reshape(v.shape[0] // 8, 8, v.shape[1])


class _Moments:
    def __init__(self):
        self.shift = self.s1 = self.s2 = None

    def add(self, v):
        if self.shift is None:
            self.shift = jnp.broadcast_to(v[0:1], (8, v.shape[1]))
        dv = _by8(v) - self.shift[None]
        a, b = jnp.sum(dv, axis=0), jnp.sum(dv * dv, axis=0)
        self.s1, self.s2 = (a, b) if self.s1 is None else (self.s1 + a, self.s2 + b)

    def stats(self, d):
        e1 = jnp.sum(self.s1, axis=0, keepdims=True) * (1.0 / d)
        e2 = jnp.sum(self.s2, axis=0, keepdims=True) * (1.0 / d)
        var = jnp.maximum(e2 - e1 * e1, 0.0)
        den = _rnd(jnp.sqrt(_rnd(_rnd(var) + LN_EPS)))
        return _rnd(self.shift + e1), jnp.broadcast_to(1.0 / den, self.shift.shape)


def _chain(*jobs):
    gate = yield
    for job in jobs:
        next(job)
        while True:
            try:
                v = job.send(gate)
            except StopIteration:
                break
            gate = yield v


def _mix(a, b, every):
    next(a)
    next(b)
    gate = yield
    n, live = 0, [a, b]
    while live:
        n += 1
        job = b if (b in live and (n % (every + 1) == 0 or a not in live)) else a
        try:
            v = job.send(gate)
        except StopIteration:
            live.remove(job)
            continue
        gate = yield v


def _finish(job):
    try:
        while True:
            job.send(lambda t: t)
    except StopIteration:
        pass


def _kernel(xt_hbm, k_hbm, v_hbm, wq_hbm, wot_hbm, wr_hbm, c_hbm, wmod_hbm,
            wg_hbm, wu_hbm, wdt_hbm,
            out_hbm,
            xt_v, kbuf, vbuf, wqbuf, wobuf, wql_v, q_scr,
            wr_v, c_v, wmod_v, wg_v, wu_v, wdt_v, wd_scr, out_v,
            h_scr, acc_scr, row_scr, col_scr, vt_scr, xh_scr, r_scr, st_scr, s0_scr, s1_scr,
            z_scr, zv_scr, new_scr, cc_scr, mod_scr, hn_scr, sem, *,
            n_groups, rep, ahead, ahp, kcp, oh, lw, dt, dl, rc2, marg, sub, cuts,
            mrows, dtm, cw, lt0, lsp, lst, lxp, lsc, cdl):
    _, d, s_len = xt_v.shape
    sk = kbuf.shape[1]
    gcols = rep * DH
    tg = GW // rep
    ng = s_len // tg
    nblk = s_len // LANES
    nlt = tg // LANES
    xw = s_len // NXC
    per = xw // tg
    lastg = n_groups - 1
    s_bufs = (s0_scr, s1_scr)
    cpad = (d // LANES + 1) * LANES
    assert d % LANES == LANES // 2 and n_groups >= 5 + 4 * d // (2 * LANES)
    qscale = (DH ** -0.5) * LOG2E

    def group_copies(g, slot):
        cols = pl.ds(pl.multiple_of(g * gcols, gcols), gcols)
        s = sem.at[NXC + 1 + slot]
        return (pltpu.make_async_copy(wq_hbm.at[:, cols], wqbuf.at[slot], s),
                pltpu.make_async_copy(k_hbm.at[g], kbuf.at[slot], s),
                pltpu.make_async_copy(v_hbm.at[g], vbuf.at[slot], s),
                pltpu.make_async_copy(wot_hbm.at[:, cols], wobuf.at[slot], s))

    def x_copy(j, s):
        cols = pl.ds(pl.multiple_of(j * xw, xw), xw)
        return pltpu.make_async_copy(xt_hbm.at[:, cols], xt_v.at[0, :, cols], sem.at[s])

    cp_z = pltpu.make_async_copy(zv_scr, z_scr, sem.at[0])
    cp_c = pltpu.make_async_copy(c_hbm, c_v, sem.at[0])
    cp_m0 = pltpu.make_async_copy(wmod_hbm.at[:, 0:2 * d], wmod_v.at[:, 0:2 * d], sem.at[1])
    cp_wql = pltpu.make_async_copy(wq_hbm.at[:, lastg * gcols:(lastg + 1) * gcols], wql_v,
                                   sem.at[2])
    cp_m1 = pltpu.make_async_copy(wmod_hbm.at[:, 2 * d:6 * d], wmod_v.at[:, 2 * d:6 * d], sem.at[2])
    cp_wr = pltpu.make_async_copy(wr_hbm, wr_v, sem.at[0])
    cp_tail = (pltpu.make_async_copy(wg_hbm, wg_v, sem.at[0]),
               pltpu.make_async_copy(wu_hbm, wu_v, sem.at[0]),
               pltpu.make_async_copy(wdt_hbm, wdt_v, sem.at[0]))

    def out_start(rows, cols):
        pltpu.make_async_copy(out_v.at[rows, cols], out_hbm.at[rows, cols], sem.at[1]).start()

    def silu_c():
        cf = c_v[...].astype(F32)
        return (cf * jax.nn.sigmoid(cf)).astype(BF16)

    def mod_job(g):
        gate = yield
        mw = 2 * LANES
        lo = jnp.where(g < 2, 0, 2 * d + mw * jnp.minimum(g - 2, 4 * d // mw - 1))
        cols = pl.ds(pl.multiple_of(lo, LANES), mw)
        acc = jnp.zeros((8, mw), F32)
        for r0 in range(0, d, mrows):
            cc = jnp.concatenate([cc_scr[r0:r0 + mrows, :]] * 2, axis=1)
            prod = _by8(wmod_v[r0:r0 + mrows, cols].astype(F32) * cc)
            acc = gate(acc) + jnp.sum(prod, axis=0)
            if r0 + mrows == d:
                mod_scr[:, cols] = jnp.broadcast_to(jnp.sum(acc, axis=0, keepdims=True), (8, mw))
            gate = yield acc

    def col_job(j):
        gate = yield
        lo = pl.multiple_of((2 + j) * d // LANES * LANES, LANES)
        w = _rnd(gate(mod_scr[:, pl.ds(lo, cpad)]))
        row = jnp.where((2 + j) * d == lo, w[:, 0:d], w[:, cpad - d:cpad])
        row = jnp.where(j == 2, _rnd(1.0 + row), row)
        row_scr[j] = row
        col_scr[j] = to_col(row[0:1])
        gate = yield col_scr[0, 0:8, :], cdl

    def tspan(i, lo, n):
        if isinstance(i, int):
            return slice(i * tg + lo, i * tg + lo + n)
        return pl.ds(pl.multiple_of(i * tg + lo, n), n)

    def tcols(i):
        return tspan(i, 0, tg)

    def col(j, rows):
        return jnp.concatenate([col_scr[j, rows, :]] * nlt, axis=1)

    fch = [slice(lo, min(lo + LANES, d)) for lo in range(0, d, LANES)]

    def ln1_chunk(cols_of, mark=lambda v: None, stats=None):
        if stats is None:
            mo = _Moments()
            for r0 in range(0, d, 32):
                mo.add(xt_v[0, r0:r0 + 32, cols_of(0, xw)].astype(F32))
                mark(mo.s2)
            stats = mo.stats(d)
            mark(stats[1])
        mean, rinv = stats
        for b in range(0, xw, cw):
            for rows in fch:
                wide = lambda j: jnp.concatenate([col_scr[j, rows, :]] * (cw // LANES), axis=1)
                x = _by8(xt_v[z_scr[0, 0], rows, cols_of(b, cw)].astype(F32))
                y = ((x - mean[None, :, b:b + cw]) * rinv[None, :, b:b + cw]).reshape(-1, cw)
                h32 = pltpu.bitcast((y * wide(1) + wide(0)).astype(BF16).T, I32)
                hn_scr[b // 2:(b + cw) // 2, rows] = h32
                mark(h32[cw // 2 - 8:cw // 2])

    def to_col(row):
        return jnp.broadcast_to(row, (LANES, d)).T

    def project_q(tok, wq_ref, step=lambda *a: None):
        parts = []
        for lt in range(nlt):
            lo = tok * (tg // 2) + lt * (LANES // 2)
            rows = (slice(lo, lo + LANES // 2) if isinstance(tok, int)
                    else pl.ds(pl.multiple_of(lo, LANES // 2), LANES // 2))
            q = jnp.dot(pltpu.bitcast(h_scr[rows, :], BF16), wq_ref[...],
                        preferred_element_type=F32)
            step(q, LANES * pl.cdiv(d, LANES) * rep // 4)
            parts.append((q * qscale).astype(BF16))
        return jnp.concatenate([p[:, r * DH:(r + 1) * DH] for r in range(rep) for p in parts],
                               axis=0)

    def ln2_job(i):
        gate = yield
        mo = _Moments()
        mo.shift, mo.s1, mo.s2 = (st_scr[j, :, tcols(i)] for j in range(3))
        mean, rinv = mo.stats(d)
        racc = None
        for r0 in range(0, d, rc2):
            rows = slice(r0, r0 + rc2)
            x1 = xh_scr[d + r0:d + r0 + rc2, tcols(i)].astype(F32)
            xc = (_by8(x1) - gate(mean)[None]).reshape(x1.shape)
            y = _rnd((_by8(_rnd(xc)) * rinv[None]).reshape(x1.shape))
            h2b = (_rnd(y * col(2, rows)) + col(1, rows)).astype(BF16)
            h2 = h2b.astype(F32)
            xh_scr[rows, tcols(i)] = h2b
            out_v[rows, tcols(i)] = (x1 + col(3, rows) * h2).astype(BF16)
            part = jnp.sum(_by8(h2 * col(4, rows)), axis=0)
            racc = part if racc is None else racc + part
            if r0 + rc2 == d:
                r = jnp.sum(racc, axis=0, keepdims=True)
                for lt in range(nlt):
                    r_scr[pl.ds(i * nlt + lt, 1), :] = r[:, lt * LANES:(lt + 1) * LANES]
            gate = yield racc

    def wd_job(t, parts):
        gate = yield
        fw = wdt_v.shape[1] // parts
        for f0 in range(0, fw, LANES):
            lo = pl.multiple_of(t * fw + f0, LANES)
            w32 = pltpu.bitcast(wdt_v[:, pl.ds(lo, LANES)], I32)
            w32 = gate(_by8(w32)).reshape(w32.shape)
            wd = pltpu.bitcast(w32, BF16).T
            half = pl.multiple_of(t * (fw // 2) + f0 // 2, LANES // 2)
            wd_scr[pl.ds(half, LANES // 2), :] = pltpu.bitcast(wd, I32)
            gate = yield wd_scr[0:8, 0:LANES]

    def attention(slot, toks, sched, last=False, job=None, hook=None, dt=dt):
        wq_ref, k_ref, v_ref, wot_ref = (wqbuf.at[slot], kbuf.at[slot], vbuf.at[slot],
                                         wobuf.at[slot])
        zero = z_scr[0, 0]
        zvec = jnp.full((8, LANES), zero, I32)
        st = dict(clock=0, nxt=0, job=job)
        hist = []
        due = []
        if job is not None:
            next(job)

        def token(when):
            want = when - MXU_LAT
            for start, dur, res in reversed(hist):
                if start <= want:
                    row = min((want - start) * res.shape[0] // dur // 8 * 8, res.shape[0] - 8)
                    return pltpu.bitcast(res[row:row + 8, 0:LANES], I32) & zvec
            return None

        def tie(x, tok):
            if tok is None:
                return x
            if x.shape[-1] > LANES:
                tok = jnp.concatenate([tok] * (x.shape[-1] // LANES), axis=1)
            if x.ndim == 3:
                tok = tok[None]
            if x.dtype == I32:
                return x | tok
            return pltpu.bitcast(pltpu.bitcast(x, I32) | tok, x.dtype)

        def tie_due(x, now):
            while due and due[0][0] <= now:
                v = due.pop(0)[1]
                v = v if v.dtype == I32 else pltpu.bitcast(v, I32)
                bits = v[:, 0:LANES]
                for j in range(1, v.shape[1] // LANES):
                    bits = bits | v[:, j * LANES:(j + 1) * LANES]
                x = tie(x, bits & zvec)
            return x

        def side(upto):
            while st['job'] is not None and st['nxt'] <= upto:
                tok = token(st['nxt'] + MXU_LAT)
                try:
                    v = st['job'].send(lambda x, tok=tok: tie(x, tok))
                except StopIteration:
                    st['job'] = None
                    break
                v, extra = v if isinstance(v, tuple) else (v, 0)
                due.append((st['nxt'] + dl + extra, v))
                due.sort(key=lambda e: e[0])
                st['nxt'] += dt

        def step(result, dur, advance=None):
            hist.append((st['clock'], dur, result))
            st['clock'] += dur if advance is None else advance

        def scores(qg, buf, rows, cols, advance=None):
            s = jax.lax.dot_general(k_ref[rows, :], qg[cols], NT, preferred_element_type=F32)
            s_bufs[buf][zero, rows, cols] = s
            step(s, s.shape[0], advance)
            return s

        def max_fin(m):
            return jnp.broadcast_to(jnp.max(m, axis=0, keepdims=True), m.shape)

        def qk(qg, buf):
            m = None
            st['nxt'] = max(st['nxt'], st['clock'])
            stop = st['clock'] + sk - marg
            for j in range(4):
                t0 = st['clock']
                s = scores(qg, buf, slice(j * sk // 4, (j + 1) * sk // 4), slice(0, GW))
                blk = s.shape[0] if job is None else sub
                for r0 in range(0, s.shape[0], blk):
                    mj = jnp.max(_by8(s[r0:r0 + blk]), axis=0)
                    if m is not None:
                        m0 = tie_due(m[:, 0:LANES], t0 + r0)
                        mj = jnp.maximum(jnp.concatenate([m0, m[:, LANES:]], axis=1), mj)
                    m = mj
                    side(min(t0 + r0 + blk - 1, stop))
            return max_fin(m)

        def pv_unit(buf, m, u, kc, advance, lead):
            cs = slice(u * LANES, (u + 1) * LANES)
            o = l = None
            for j in range(sk // kc):
                when = st['clock'] - lead
                mu = tie_due(tie(m[:, cs], token(when)), when)
                p = jnp.exp2(_by8(s_bufs[buf][0, j * kc:(j + 1) * kc, cs]) - mu[None])
                lj = jnp.sum(p.reshape(kc // lw, lw, LANES), axis=0)
                oj = jnp.dot(pltpu.bitcast(vt_scr[0, :, j * kc:(j + 1) * kc], BF16),
                             p.reshape(kc, LANES).astype(BF16), preferred_element_type=F32)
                o = oj if o is None else o + oj
                l = lj if l is None else l + lj
                step(oj, DH, advance)
            return (o / jnp.sum(l, axis=0, keepdims=True)).astype(BF16)

        def heads_major(outs):
            return jnp.concatenate(
                [jnp.concatenate(outs[r * nlt:(r + 1) * nlt], axis=1) for r in range(rep)], axis=0)

        def pv(buf, m):
            return heads_major([pv_unit(buf, m, u, kcp, kcp // 4, ahp) for u in range(4)])

        def pv_qk(buf, m, qn, nbuf):
            outs, mns = [], []
            for half in range(2):
                s = scores(qn, nbuf, slice(0, sk), slice(half * GW // 2, (half + 1) * GW // 2), 0)
                mns.append(jnp.max(_by8(s), axis=0))
                outs += [pv_unit(buf, m, u, 2 * LANES, DH, ahead) for u in (2 * half, 2 * half + 1)]
            return heads_major(outs), max_fin(jnp.concatenate(mns, axis=1))

        def oproj(tok, ot):
            cols = tcols(tok)
            mo = _Moments()
            for r0 in range(0, d, oh):
                rows = slice(r0, r0 + oh)
                res = jnp.dot(wot_ref[rows, :], ot, preferred_element_type=F32)
                attn = res + acc_scr[rows, cols]
                if last:
                    x1b = (xt_v[0, rows, cols].astype(F32) + col(0, rows) * attn).astype(BF16)
                    xh_scr[d + r0:d + r0 + oh, cols] = x1b
                    mo.add(x1b.astype(F32))
                else:
                    acc_scr[rows, cols] = attn
                step(res, oh)
            if last:
                for j, v in enumerate((mo.shift, mo.s1, mo.s2)):
                    st_scr[j, :, cols] = v

        qs, ots, ms, bufs, free = {}, {}, {}, {}, [0, 1]
        for item in sched.split():
            kind, i = item[0], int(item[1:] or 0)
            if kind == '!':
                hook()
            elif kind == 'V':
                vt_scr[zero] = pltpu.bitcast(v_ref[...].T, I32)
            elif kind == 'Q':
                qs[i] = project_q(toks[i], wq_ref, step)
            elif kind == 'L':
                qs[i] = q_scr[toks[i]]
            elif kind == 'K':
                bufs[i] = free.pop(0)
                ms[i] = qk(qs[i], bufs[i])
            elif kind == 'P':
                ots[i] = pv(bufs[i], ms[i])
                free.append(bufs[i])
            elif kind == 'S':
                bufs[i + 1] = free.pop(0)
                ots[i], ms[i + 1] = pv_qk(bufs[i], ms[i], qs[i + 1], bufs[i + 1])
                free.append(bufs[i])
            elif kind == 'O':
                oproj(toks[i], ots[i])
        if st['job'] is not None:
            _finish(st['job'])

    zv_scr[...] = jnp.zeros(zv_scr.shape, I32)
    for cp in ((cp_z, cp_c, cp_wr, x_copy(0, 0), cp_m0, cp_wql)
               + tuple(x_copy(j, j + 1) for j in range(1, NXC)) + group_copies(0, 0)):
        cp.start()

    def zero_body(j, carry):
        rows = pl.ds(pl.multiple_of(j * 32, 32), 32)
        acc_scr[rows, :] = jnp.zeros((32, s_len), F32)
        xh_scr[pl.ds(pl.multiple_of(d + j * 32, 32), 32), s_len - 2 * tg:s_len] = (
            jnp.zeros((32, 2 * tg), BF16))
        return carry

    jax.lax.fori_loop(0, d // 32, zero_body, 0)
    st_scr[:, :, s_len - 2 * tg:s_len] = jnp.zeros((3, 8, 2 * tg), F32)
    mod_scr[...] = jnp.zeros(mod_scr.shape, F32)
    cp_z.wait()
    cp_c.wait()
    cp_wr.wait()
    x_copy(0, 0).wait()

    mo0 = _Moments()
    for r0 in range(0, d, 32):
        mo0.add(xt_v[0, r0:r0 + 32, 0:xw].astype(F32))
    stats0 = mo0.stats(d)
    cc_scr[...] = to_col(silu_c()).astype(F32)
    mod_scr[:, 6 * d:7 * d] = jnp.broadcast_to(wr_v[...].astype(F32).reshape(1, d), (8, d))
    cp_m0.wait()
    mod = _rnd(jnp.dot(jnp.broadcast_to(silu_c(), (8, d)), wmod_v[:, 0:2 * d],
                       preferred_element_type=F32))
    col_scr[z_scr[0, 0]] = to_col(mod[0:1, 0:d])
    col_scr[z_scr[0, 0] + 1] = to_col(_rnd(1.0 + mod[0:1, d:2 * d]))
    ln1_chunk(lambda lo, n: slice(lo, lo + n), stats=stats0)
    cp_wql.wait()

    def ln1_body(j, carry):
        src = jnp.minimum(j + 1, NXC - 1)

        @pl.when(j + 1 < NXC)
        def _():
            x_copy(src, src + 1).wait()

        zvec = jnp.full((8, LANES), z_scr[0, 0], I32)
        nb = xw // LANES
        half = LANES // 2
        lhs = [hn_scr[b * half:(b + 1) * half, :] for b in range(nb)]
        for b in range(nb):
            h_scr[pl.ds(pl.multiple_of(j * (xw // 2) + b * half, half), half), :] = lhs[b]
        marks = []
        ln1_chunk(lambda lo, n: pl.ds(pl.multiple_of(src * xw + lo, n), n), marks.append)
        na = d // 32
        times = ([lt0 + lsp * i for i in range(na)] + [lt0 + lsp * na + lst]
                 + [lt0 + lsp * na + lst + lxp + lsc * i for i in range(len(marks) - na - 1)])
        dur = LANES * len(fch) * rep // 4
        ties = {}
        for t, v in zip(times, marks):
            b, off = t // dur, t % dur
            if off >= 2 * LANES:
                b, off = b + 1, 0
            if b < nb:
                v = v if v.dtype == I32 else pltpu.bitcast(v, I32)
                bits = v[:, 0:LANES] if v.shape[1] >= LANES else jnp.concatenate([v, v], axis=1)
                for c0 in range(LANES, v.shape[1], LANES):
                    bits = bits | v[:, c0:c0 + LANES]
                where = (b, off % LANES // 16, 0 if off < LANES else len(fch) - 1)
                ties[where] = bits if where not in ties else ties[where] | bits
        for b in range(nb):
            grid = [[lhs[b][r * 8:(r + 1) * 8, fs] for fs in fch] for r in range(half // 8)]
            for (bb, r, k), bits in ties.items():
                if bb == b:
                    grid[r][k] = grid[r][k] | (bits & zvec)[:, 0:grid[r][k].shape[1]]
            hb = jnp.concatenate([jnp.concatenate(row, axis=1) for row in grid], axis=0)
            q = jnp.dot(pltpu.bitcast(hb, BF16), wql_v[...], preferred_element_type=F32)
            q = (q * qscale).astype(BF16)
            for r in range(rep):
                lo = r * tg + (b % nlt) * LANES
                q_scr[j * per + b // nlt, lo:lo + LANES, :] = q[:, r * DH:(r + 1) * DH]
        return carry

    jax.lax.fori_loop(0, NXC, ln1_body, 0)

    steady = 'V Q0 Q1 K0 ! ' + ' '.join(
        ('O%d ' % (i - 2) if i >= 2 else '') + ('Q%d ' % (i + 2) if i + 2 < ng else '')
        + ('S%d' % i if i + 1 < ng else 'P%d' % i) for i in range(ng)
    ) + ' O%d O%d' % (ng - 2, ng - 1)

    def group_body(g, carry):
        slot = g & 1
        for cp in group_copies(g, slot):
            cp.wait()

        @pl.when(g == 2)
        def _():
            cp_m1.wait()

        def prefetch():
            for cp in group_copies(g + 1, 1 - slot):
                cp.start()
            for j, cp in enumerate((cp_m1,) + cp_tail):
                @pl.when(g == j)
                def _(cp=cp):
                    cp.start()

        attention(slot, list(range(ng)), steady, hook=prefetch, dt=dtm,
                  job=_chain(col_job(jnp.clip(g - (lastg - 5), 0, 4)), mod_job(g)))
        return carry
    jax.lax.fori_loop(0, lastg, group_body, 0)

    for cp in group_copies(lastg, lastg % 2) + cp_tail:
        cp.wait()
    npair = ng // 2

    def last_body(t, carry):
        prev = (t + npair - 1) % npair
        attention(lastg % 2, [2 * t, 2 * t + 1], 'V L0 L1 K0 K1 P0 P1 O0 O1', last=True,
                  job=_mix(_chain(ln2_job(2 * prev), ln2_job(2 * prev + 1)), wd_job(t, npair), 4))
        return carry
    jax.lax.fori_loop(0, npair, last_body, 0)
    rest = _chain(ln2_job(ng - 2), ln2_job(ng - 1))
    next(rest)
    _finish(rest)

    ibits = (s_len - 1).bit_length()
    imask = (1 << ibits) - 1
    bits = pltpu.bitcast(_rnd(r_scr[...]), I32)
    pos = (jax.lax.broadcasted_iota(I32, bits.shape, 0) * LANES
           + jax.lax.broadcasted_iota(I32, bits.shape, 1))
    order = ((bits ^ ((bits >> 31) & 0x7FFFFFFF)) >> 16) + 0x8000
    key = pltpu.bitcast((order << ibits) + (imask - pos) + 0x20000000, F32)
    subl = jax.lax.broadcasted_iota(I32, (TOPC, LANES), 0)
    lane = jax.lax.broadcasted_iota(I32, (TOPC, LANES), 1)
    idxs, blks, bcols = [], [], []
    keyv = jnp.zeros((TOPC, LANES), I32)
    x_sel = jnp.zeros((TOPC, d), F32)
    x1_sel = jnp.zeros((TOPC, d), F32)
    for c in range(TOPC):
        top = jnp.max(jnp.max(key, axis=0, keepdims=True), axis=1, keepdims=True)
        key = jnp.where(key == top, 0.0, key)
        topi = pltpu.bitcast(jnp.broadcast_to(top, (TOPC, LANES)), I32)
        keyv = jnp.where(subl == c, topi, keyv)
        ixv = imask - (topi & imask)
        idxs.append(ixv[0, 0])
        blks.append(idxs[c] // LANES)
        bcols.append(pl.ds(pl.multiple_of(blks[c] * LANES, LANES), LANES))
        pick = jnp.where((lane == (ixv & (LANES - 1))) & (subl == c), 1.0, 0.0).astype(BF16)
        x_sel = x_sel + jax.lax.dot_general(pick, xh_scr[0:d, bcols[c]], NT,
                                            preferred_element_type=F32)
        x1_sel = x1_sel + jax.lax.dot_general(pick, xh_scr[d:2 * d, bcols[c]], NT,
                                              preferred_element_type=F32)

    for b in range(nblk):
        hit = blks[0] == b
        for bb in blks[1:]:
            hit = jnp.logical_or(hit, bb == b)

        @pl.when(jnp.logical_not(hit))
        def _(b=b):
            out_start(slice(0, d), slice(b * LANES, (b + 1) * LANES))

    final = []
    for c in range(TOPC):
        u = True
        for other in blks[c + 1:]:
            u = jnp.logical_and(u, other != blks[c])
        final.append(jnp.asarray(u))

    ob = (((keyv - 0x20000000) >> ibits) - 0x8000) << 16
    r_sel = pltpu.bitcast((ob ^ ((ob >> 31) & 0x7FFFFFFF)) & ~0xFFFF, F32)
    xs = x_sel.astype(BF16)
    gt = _rnd(jnp.dot(xs, wg_v[...], preferred_element_type=F32))
    gt = _rnd(gt * jax.nn.sigmoid(gt))
    up = _rnd(jnp.dot(xs, wu_v[...], preferred_element_type=F32))
    gu = (gt * up).astype(BF16)
    gate_r = jnp.concatenate([_rnd(jax.nn.sigmoid(r_sel))] * pl.cdiv(d, LANES), axis=1)

    def down(fs):
        y = _rnd(jnp.dot(gu, pltpu.bitcast(wd_scr[:, fs], BF16), preferred_element_type=F32))
        y = _rnd(y * gate_r[:, fs])
        return x1_sel[:, fs] + _rnd(row_scr[3, :, fs] * _rnd(x_sel[:, fs] + y))

    def patch(fs, new):
        n = fs.stop - fs.start
        lane_d = jax.lax.broadcasted_iota(I32, (n // 2, LANES), 1)
        for c in range(TOPC):
            ln = idxs[c] & (LANES - 1)
            wide = jnp.broadcast_to(new[c:c + 1], (LANES, n)).astype(BF16).T
            moved = pltpu.bitcast(wide, I32)
            cur = pltpu.bitcast(out_v[fs, bcols[c]], I32)
            out_v[fs, bcols[c]] = pltpu.bitcast(jnp.where(lane_d == ln, moved, cur), BF16)

            @pl.when(final[c])
            def _(c=c):
                out_start(fs, bcols[c])

    pch = [slice(a, b) for a, b in zip((0,) + cuts, cuts + (d,))]
    new_scr[:, pch[0]] = down(pch[0])
    for j in range(len(pch)):
        @pl.when(z_scr[0, 0] == 0)
        def _(j=j):
            prev = new_scr[:, pch[j]]
            if j + 1 < len(pch):
                new_scr[:, pch[j + 1]] = down(pch[j + 1])
            patch(pch[j], prev)
    pltpu.make_async_copy(out_v, out_hbm, sem.at[1]).wait()


def _build(ahead=384, ahp=320, kcp=256, oh=144, lw=32, dt=80, dl=320, rc2=32,
          marg=128, sub=64, cuts=(256, 512), mrows=64, dtm=150, cw=256, lt0=40, lsp=28, lst=150, lxp=230, lsc=56, cdl=600):
    @jax.jit
    def pallas_adaLN_cond__gqa_block_cached__moe_arch_mod__prompt_kernel(
            A_x, A_k_cache, A_v_cache, A_wq, A_wo, B_x, B_w_r, B_w_gate, B_w_up, B_w_down, c, w_mod):
        b, s_len, d = A_x.shape
        assert b == 1
        hkv, sk = A_k_cache.shape[1], A_k_cache.shape[2]
        rep = HQ // hkv
        f = B_w_gate.shape[1]
        tg = GW // rep
        scratch = [
            pltpu.VMEM((1, d, s_len), BF16),
            pltpu.VMEM((2, sk, DH), BF16),
            pltpu.VMEM((2, sk, DH), BF16),
            pltpu.VMEM((2, d, rep * DH), BF16),
            pltpu.VMEM((2, d, rep * DH), BF16),
            pltpu.VMEM((d, rep * DH), BF16),
            pltpu.VMEM((s_len // tg, GW, DH), BF16),
            pltpu.VMEM((d,), BF16),
            pltpu.VMEM((1, d), BF16),
            pltpu.VMEM((d, 6 * d), BF16),
            pltpu.VMEM((d, f), BF16),
            pltpu.VMEM((d, f), BF16),
            pltpu.VMEM((d, f), BF16),
            pltpu.VMEM((f // 2, d), I32),
            pltpu.VMEM((d, s_len), BF16),
            pltpu.VMEM((s_len // 2, d), I32),
            pltpu.VMEM((d, s_len), F32),
            pltpu.VMEM((5, 8, d), F32),
            pltpu.VMEM((5, d, LANES), F32),
            pltpu.VMEM((1, DH // 2, sk), I32),
            pltpu.VMEM((2 * d, s_len), BF16),
            pltpu.VMEM((s_len // LANES, LANES), F32),
            pltpu.VMEM((3, 8, s_len), F32),
            pltpu.VMEM((1, sk, GW), F32),
            pltpu.VMEM((1, sk, GW), F32),
            pltpu.SMEM((8, LANES), I32),
            pltpu.VMEM((8, LANES), I32),
            pltpu.VMEM((TOPC, d), F32),
            pltpu.VMEM((d, LANES), F32),
            pltpu.VMEM((8, 6 * d + (d // LANES + 1) * LANES), F32),
            pltpu.VMEM((s_len // NXC // 2, d), I32),
            pltpu.SemaphoreType.DMA((NXC + 3,)),
        ]
        out = pl.pallas_call(
            functools.partial(_kernel, n_groups=hkv, rep=rep, ahead=ahead,
                              ahp=ahp, kcp=kcp, oh=oh, lw=lw, dt=dt, dl=dl, rc2=rc2, marg=marg,
                              sub=sub, cuts=cuts, mrows=mrows, dtm=dtm, cw=cw, lt0=lt0, lsp=lsp,
                              lst=lst, lxp=lxp, lsc=lsc, cdl=cdl),
            in_specs=[pl.BlockSpec(memory_space=pl.ANY)] * 11,
            out_specs=pl.BlockSpec(memory_space=pl.ANY),
            out_shape=jax.ShapeDtypeStruct((d, s_len), BF16),
            scratch_shapes=scratch,
            compiler_params=pltpu.CompilerParams(vmem_limit_bytes=100 * 1024 * 1024),
        )(A_x.reshape(s_len, d).T, A_k_cache.reshape(hkv, sk, DH), A_v_cache.reshape(hkv, sk, DH),
          A_wq, A_wo.T, B_w_r, c, w_mod, B_w_gate, B_w_up, B_w_down.T)
        return out.T.reshape(b, s_len, d)
    return pallas_adaLN_cond__gqa_block_cached__moe_arch_mod__prompt_kernel


pallas_adaLN_cond__gqa_block_cached__moe_arch_mod__prompt_kernel = _build()
```

```python
import functools

import jax
import jax.numpy as jnp
import jax.experimental.pallas as pl
import jax.experimental.pallas.tpu as pltpu

HQ = 32
DH = 128
TOPC = 8
LN_EPS = 1.0013580322265625e-05
LOG2E = 1.4426950408889634
F32 = jnp.float32
BF16 = jnp.bfloat16
I32 = jnp.int32
NT = (((1,), (1,)), ((), ()))
LANES = 128
GW = 512
MXU_LAT = 128
NXC = 4


def _rnd(v):
    return v.astype(BF16).astype(F32)


def _by8(v):
    return v.reshape(v.shape[0] // 8, 8, v.shape[1])


class _Moments:
    def __init__(self):
        self.shift = self.s1 = self.s2 = None

    def add(self, v):
        if self.shift is None:
            self.shift = jnp.broadcast_to(v[0:1], (8, v.shape[1]))
        dv = _by8(v) - self.shift[None]
        a, b = jnp.sum(dv, axis=0), jnp.sum(dv * dv, axis=0)
        self.s1, self.s2 = (a, b) if self.s1 is None else (self.s1 + a, self.s2 + b)

    def stats(self, d):
        e1 = jnp.sum(self.s1, axis=0, keepdims=True) * (1.0 / d)
        e2 = jnp.sum(self.s2, axis=0, keepdims=True) * (1.0 / d)
        var = jnp.maximum(e2 - e1 * e1, 0.0)
        den = _rnd(jnp.sqrt(_rnd(_rnd(var) + LN_EPS)))
        return _rnd(self.shift + e1), jnp.broadcast_to(1.0 / den, self.shift.shape)


def _chain(*jobs):
    gate = yield
    for job in jobs:
        next(job)
        while True:
            try:
                v = job.send(gate)
            except StopIteration:
                break
            gate = yield v


def _mix(a, b, every):
    next(a)
    next(b)
    gate = yield
    n, live = 0, [a, b]
    while live:
        n += 1
        job = b if (b in live and (n % (every + 1) == 0 or a not in live)) else a
        try:
            v = job.send(gate)
        except StopIteration:
            live.remove(job)
            continue
        gate = yield v


def _finish(job):
    try:
        while True:
            job.send(lambda t: t)
    except StopIteration:
        pass


def _kernel(xt_hbm, k_hbm, v_hbm, wq_hbm, wot_hbm, wr_hbm, c_hbm, wmod_hbm,
            wg_hbm, wu_hbm, wdt_hbm,
            out_hbm,
            xt_v, kbuf, vbuf, wqbuf, wobuf, wql_v, q_scr,
            wr_v, c_v, wmod_v, wg_v, wu_v, wdt_v, wd_scr, out_v,
            h_scr, acc_scr, row_scr, col_scr, vt_scr, xh_scr, r_scr, st_scr, s0_scr, s1_scr,
            z_scr, zv_scr, new_scr, cc_scr, mod_scr, hn_scr, sem, *,
            n_groups, rep, ahead, ahp, kcp, oh, lw, dt, dl, rc2, marg, sub, cuts,
            mrows, dtm, cw, lt0, lsp, lst, lxp, lsc, cdl):
    _, d, s_len = xt_v.shape
    sk = kbuf.shape[1]
    gcols = rep * DH
    tg = GW // rep
    ng = s_len // tg
    nblk = s_len // LANES
    nlt = tg // LANES
    xw = s_len // NXC
    per = xw // tg
    lastg = n_groups - 1
    s_bufs = (s0_scr, s1_scr)
    cpad = (d // LANES + 1) * LANES
    assert d % LANES == LANES // 2 and n_groups >= 5 + 4 * d // (2 * LANES)
    qscale = (DH ** -0.5) * LOG2E

    def group_copies(g, slot):
        cols = pl.ds(pl.multiple_of(g * gcols, gcols), gcols)
        s = sem.at[NXC + 2 + slot]
        return (pltpu.make_async_copy(wq_hbm.at[:, cols], wqbuf.at[slot], s),
                pltpu.make_async_copy(k_hbm.at[g], kbuf.at[slot], s),
                pltpu.make_async_copy(v_hbm.at[g], vbuf.at[slot], s),
                pltpu.make_async_copy(wot_hbm.at[:, cols], wobuf.at[slot], s))

    def x_copy(j, s):
        cols = pl.ds(pl.multiple_of(j * xw, xw), xw)
        return pltpu.make_async_copy(xt_hbm.at[:, cols], xt_v.at[0, :, cols], sem.at[s])

    cp_z = pltpu.make_async_copy(zv_scr, z_scr, sem.at[0])
    cp_c = pltpu.make_async_copy(c_hbm, c_v, sem.at[0])
    cp_m0 = pltpu.make_async_copy(wmod_hbm.at[:, 0:2 * d], wmod_v.at[:, 0:2 * d], sem.at[1])
    cp_wql = pltpu.make_async_copy(wq_hbm.at[:, lastg * gcols:(lastg + 1) * gcols], wql_v,
                                   sem.at[2])
    cp_m1 = pltpu.make_async_copy(wmod_hbm.at[:, 2 * d:6 * d], wmod_v.at[:, 2 * d:6 * d], sem.at[2])
    cp_wr = pltpu.make_async_copy(wr_hbm, wr_v, sem.at[0])
    cp_tail = (pltpu.make_async_copy(wg_hbm, wg_v, sem.at[0]),
               pltpu.make_async_copy(wu_hbm, wu_v, sem.at[0]),
               pltpu.make_async_copy(wdt_hbm, wdt_v, sem.at[0]))

    def out_start(rows, cols):
        pltpu.make_async_copy(out_v.at[rows, cols], out_hbm.at[rows, cols], sem.at[1]).start()

    def silu_c():
        cf = c_v[...].astype(F32)
        return (cf * jax.nn.sigmoid(cf)).astype(BF16)

    def mod_job(g):
        gate = yield
        mw = 2 * LANES
        lo = jnp.where(g < 2, 0, 2 * d + mw * jnp.minimum(g - 2, 4 * d // mw - 1))
        cols = pl.ds(pl.multiple_of(lo, LANES), mw)
        acc = jnp.zeros((8, mw), F32)
        for r0 in range(0, d, mrows):
            cc = jnp.concatenate([cc_scr[r0:r0 + mrows, :]] * 2, axis=1)
            prod = _by8(wmod_v[r0:r0 + mrows, cols].astype(F32) * cc)
            acc = gate(acc) + jnp.sum(prod, axis=0)
            if r0 + mrows == d:
                mod_scr[:, cols] = jnp.broadcast_to(jnp.sum(acc, axis=0, keepdims=True), (8, mw))
            gate = yield acc

    def col_job(j):
        gate = yield
        lo = pl.multiple_of((2 + j) * d // LANES * LANES, LANES)
        w = _rnd(gate(mod_scr[:, pl.ds(lo, cpad)]))
        row = jnp.where((2 + j) * d == lo, w[:, 0:d], w[:, cpad - d:cpad])
        row = jnp.where(j == 2, _rnd(1.0 + row), row)
        row_scr[j] = row
        col_scr[j] = to_col(row[0:1])
        gate = yield col_scr[0, 0:8, :], cdl

    def tspan(i, lo, n):
        if isinstance(i, int):
            return slice(i * tg + lo, i * tg + lo + n)
        return pl.ds(pl.multiple_of(i * tg + lo, n), n)

    def tcols(i):
        return tspan(i, 0, tg)

    def col(j, rows):
        return jnp.concatenate([col_scr[j, rows, :]] * nlt, axis=1)

    fch = [slice(lo, min(lo + LANES, d)) for lo in range(0, d, LANES)]

    def ln1_chunk(cols_of, mark=lambda v: None, stats=None):
        if stats is None:
            mo = _Moments()
            for r0 in range(0, d, 32):
                mo.add(xt_v[0, r0:r0 + 32, cols_of(0, xw)].astype(F32))
                mark(mo.s2)
            stats = mo.stats(d)
            mark(stats[1])
        mean, rinv = stats
        for b in range(0, xw, cw):
            for rows in fch:
                wide = lambda j: jnp.concatenate([col_scr[j, rows, :]] * (cw // LANES), axis=1)
                x = _by8(xt_v[z_scr[0, 0], rows, cols_of(b, cw)].astype(F32))
                y = ((x - mean[None, :, b:b + cw]) * rinv[None, :, b:b + cw]).reshape(-1, cw)
                h32 = pltpu.bitcast((y * wide(1) + wide(0)).astype(BF16).T, I32)
                hn_scr[b // 2:(b + cw) // 2, rows] = h32
                mark(h32[cw // 2 - 8:cw // 2])

    def to_col(row):
        return jnp.broadcast_to(row, (LANES, d)).T

    def project_q(tok, wq_ref, step=lambda *a: None):
        parts = []
        for lt in range(nlt):
            lo = tok * (tg // 2) + lt * (LANES // 2)
            rows = (slice(lo, lo + LANES // 2) if isinstance(tok, int)
                    else pl.ds(pl.multiple_of(lo, LANES // 2), LANES // 2))
            q = jnp.dot(pltpu.bitcast(h_scr[rows, :], BF16), wq_ref[...],
                        preferred_element_type=F32)
            step(q, LANES * pl.cdiv(d, LANES) * rep // 4)
            parts.append((q * qscale).astype(BF16))
        return jnp.concatenate([p[:, r * DH:(r + 1) * DH] for r in range(rep) for p in parts],
                               axis=0)

    def ln2_job(i):
        gate = yield
        mo = _Moments()
        mo.shift, mo.s1, mo.s2 = (st_scr[j, :, tcols(i)] for j in range(3))
        mean, rinv = mo.stats(d)
        racc = None
        for r0 in range(0, d, rc2):
            rows = slice(r0, r0 + rc2)
            x1 = xh_scr[d + r0:d + r0 + rc2, tcols(i)].astype(F32)
            xc = (_by8(x1) - gate(mean)[None]).reshape(x1.shape)
            y = _rnd((_by8(_rnd(xc)) * rinv[None]).reshape(x1.shape))
            h2b = (_rnd(y * col(2, rows)) + col(1, rows)).astype(BF16)
            h2 = h2b.astype(F32)
            xh_scr[rows, tcols(i)] = h2b
            out_v[rows, tcols(i)] = (x1 + col(3, rows) * h2).astype(BF16)
            part = jnp.sum(_by8(h2 * col(4, rows)), axis=0)
            racc = part if racc is None else racc + part
            if r0 + rc2 == d:
                r = jnp.sum(racc, axis=0, keepdims=True)
                for lt in range(nlt):
                    r_scr[pl.ds(i * nlt + lt, 1), :] = r[:, lt * LANES:(lt + 1) * LANES]
            gate = yield racc

    def wd_job(t, parts):
        gate = yield
        fw = wdt_v.shape[1] // parts
        for f0 in range(0, fw, LANES):
            lo = pl.multiple_of(t * fw + f0, LANES)
            w32 = pltpu.bitcast(wdt_v[:, pl.ds(lo, LANES)], I32)
            w32 = gate(_by8(w32)).reshape(w32.shape)
            wd = pltpu.bitcast(w32, BF16).T
            half = pl.multiple_of(t * (fw // 2) + f0 // 2, LANES // 2)
            wd_scr[pl.ds(half, LANES // 2), :] = pltpu.bitcast(wd, I32)
            gate = yield wd_scr[0:8, 0:LANES]

    def attention(slot, toks, sched, last=False, job=None, hook=None, dt=dt):
        wq_ref, k_ref, v_ref, wot_ref = (wqbuf.at[slot], kbuf.at[slot], vbuf.at[slot],
                                         wobuf.at[slot])
        zero = z_scr[0, 0]
        zvec = jnp.full((8, LANES), zero, I32)
        st = dict(clock=0, nxt=0, job=job)
        hist = []
        due = []
        if job is not None:
            next(job)

        def token(when):
            want = when - MXU_LAT
            for start, dur, res in reversed(hist):
                if start <= want:
                    row = min((want - start) * res.shape[0] // dur // 8 * 8, res.shape[0] - 8)
                    return pltpu.bitcast(res[row:row + 8, 0:LANES], I32) & zvec
            return None

        def tie(x, tok):
            if tok is None:
                return x
            if x.shape[-1] > LANES:
                tok = jnp.concatenate([tok] * (x.shape[-1] // LANES), axis=1)
            if x.ndim == 3:
                tok = tok[None]
            if x.dtype == I32:
                return x | tok
            return pltpu.bitcast(pltpu.bitcast(x, I32) | tok, x.dtype)

        def tie_due(x, now):
            while due and due[0][0] <= now:
                v = due.pop(0)[1]
                v = v if v.dtype == I32 else pltpu.bitcast(v, I32)
                bits = v[:, 0:LANES]
                for j in range(1, v.shape[1] // LANES):
                    bits = bits | v[:, j * LANES:(j + 1) * LANES]
                x = tie(x, bits & zvec)
            return x

        def side(upto):
            while st['job'] is not None and st['nxt'] <= upto:
                tok = token(st['nxt'] + MXU_LAT)
                try:
                    v = st['job'].send(lambda x, tok=tok: tie(x, tok))
                except StopIteration:
                    st['job'] = None
                    break
                v, extra = v if isinstance(v, tuple) else (v, 0)
                due.append((st['nxt'] + dl + extra, v))
                due.sort(key=lambda e: e[0])
                st['nxt'] += dt

        def step(result, dur, advance=None):
            hist.append((st['clock'], dur, result))
            st['clock'] += dur if advance is None else advance

        def scores(qg, buf, rows, cols, advance=None):
            s = jax.lax.dot_general(k_ref[rows, :], qg[cols], NT, preferred_element_type=F32)
            s_bufs[buf][zero, rows, cols] = s
            step(s, s.shape[0], advance)
            return s

        def max_fin(m):
            return jnp.broadcast_to(jnp.max(m, axis=0, keepdims=True), m.shape)

        def qk(qg, buf):
            m = None
            st['nxt'] = max(st['nxt'], st['clock'])
            stop = st['clock'] + sk - marg
            for j in range(4):
                t0 = st['clock']
                s = scores(qg, buf, slice(j * sk // 4, (j + 1) * sk // 4), slice(0, GW))
                blk = s.shape[0] if job is None else sub
                for r0 in range(0, s.shape[0], blk):
                    mj = jnp.max(_by8(s[r0:r0 + blk]), axis=0)
                    if m is not None:
                        m0 = tie_due(m[:, 0:LANES], t0 + r0)
                        mj = jnp.maximum(jnp.concatenate([m0, m[:, LANES:]], axis=1), mj)
                    m = mj
                    side(min(t0 + r0 + blk - 1, stop))
            return max_fin(m)

        def pv_unit(buf, m, u, kc, advance, lead):
            cs = slice(u * LANES, (u + 1) * LANES)
            o = l = None
            for j in range(sk // kc):
                when = st['clock'] - lead
                mu = tie_due(tie(m[:, cs], token(when)), when)
                p = jnp.exp2(_by8(s_bufs[buf][0, j * kc:(j + 1) * kc, cs]) - mu[None])
                lj = jnp.sum(p.reshape(kc // lw, lw, LANES), axis=0)
                oj = jnp.dot(pltpu.bitcast(vt_scr[0, :, j * kc:(j + 1) * kc], BF16),
                             p.reshape(kc, LANES).astype(BF16), preferred_element_type=F32)
                o = oj if o is None else o + oj
                l = lj if l is None else l + lj
                step(oj, DH, advance)
            return (o / jnp.sum(l, axis=0, keepdims=True)).astype(BF16)

        def heads_major(outs):
            return jnp.concatenate(
                [jnp.concatenate(outs[r * nlt:(r + 1) * nlt], axis=1) for r in range(rep)], axis=0)

        def pv(buf, m):
            return heads_major([pv_unit(buf, m, u, kcp, kcp // 4, ahp) for u in range(4)])

        def pv_qk(buf, m, qn, nbuf):
            outs, mns = [], []
            for half in range(2):
                s = scores(qn, nbuf, slice(0, sk), slice(half * GW // 2, (half + 1) * GW // 2), 0)
                mns.append(jnp.max(_by8(s), axis=0))
                outs += [pv_unit(buf, m, u, 2 * LANES, DH, ahead) for u in (2 * half, 2 * half + 1)]
            return heads_major(outs), max_fin(jnp.concatenate(mns, axis=1))

        def oproj(tok, ot):
            cols = tcols(tok)
            mo = _Moments()
            for r0 in range(0, d, oh):
                rows = slice(r0, r0 + oh)
                res = jnp.dot(wot_ref[rows, :], ot, preferred_element_type=F32)
                attn = res + acc_scr[rows, cols]
                if last:
                    x1b = (xt_v[0, rows, cols].astype(F32) + col(0, rows) * attn).astype(BF16)
                    xh_scr[d + r0:d + r0 + oh, cols] = x1b
                    mo.add(x1b.astype(F32))
                else:
                    acc_scr[rows, cols] = attn
                step(res, oh)
            if last:
                for j, v in enumerate((mo.shift, mo.s1, mo.s2)):
                    st_scr[j, :, cols] = v

        qs, ots, ms, bufs, free = {}, {}, {}, {}, [0, 1]
        for item in sched.split():
            kind, i = item[0], int(item[1:] or 0)
            if kind == '!':
                hook()
            elif kind == 'V':
                vt_scr[zero] = pltpu.bitcast(v_ref[...].T, I32)
            elif kind == 'Q':
                qs[i] = project_q(toks[i], wq_ref, step)
            elif kind == 'L':
                qs[i] = q_scr[toks[i]]
            elif kind == 'K':
                bufs[i] = free.pop(0)
                ms[i] = qk(qs[i], bufs[i])
            elif kind == 'P':
                ots[i] = pv(bufs[i], ms[i])
                free.append(bufs[i])
            elif kind == 'S':
                bufs[i + 1] = free.pop(0)
                ots[i], ms[i + 1] = pv_qk(bufs[i], ms[i], qs[i + 1], bufs[i + 1])
                free.append(bufs[i])
            elif kind == 'O':
                oproj(toks[i], ots[i])
        if st['job'] is not None:
            _finish(st['job'])

    zv_scr[...] = jnp.zeros(zv_scr.shape, I32)
    for cp in ((cp_z, cp_c, cp_wr, x_copy(0, 0), cp_m0, cp_wql)
               + tuple(x_copy(j, j + 2) for j in range(1, NXC)) + group_copies(0, 0)):
        cp.start()

    def zero_body(j, carry):
        rows = pl.ds(pl.multiple_of(j * 32, 32), 32)
        acc_scr[rows, :] = jnp.zeros((32, s_len), F32)
        xh_scr[pl.ds(pl.multiple_of(d + j * 32, 32), 32), s_len - 2 * tg:s_len] = (
            jnp.zeros((32, 2 * tg), BF16))
        return carry

    jax.lax.fori_loop(0, d // 32, zero_body, 0)
    st_scr[:, :, s_len - 2 * tg:s_len] = jnp.zeros((3, 8, 2 * tg), F32)
    mod_scr[...] = jnp.zeros(mod_scr.shape, F32)
    cp_z.wait()
    cp_c.wait()
    cp_wr.wait()
    x_copy(0, 0).wait()

    mo0 = _Moments()
    for r0 in range(0, d, 32):
        mo0.add(xt_v[0, r0:r0 + 32, 0:xw].astype(F32))
    stats0 = mo0.stats(d)
    cc_scr[...] = to_col(silu_c()).astype(F32)
    mod_scr[:, 6 * d:7 * d] = jnp.broadcast_to(wr_v[...].astype(F32).reshape(1, d), (8, d))
    cp_m0.wait()
    mod = _rnd(jnp.dot(jnp.broadcast_to(silu_c(), (8, d)), wmod_v[:, 0:2 * d],
                       preferred_element_type=F32))
    col_scr[z_scr[0, 0]] = to_col(mod[0:1, 0:d])
    col_scr[z_scr[0, 0] + 1] = to_col(_rnd(1.0 + mod[0:1, d:2 * d]))
    ln1_chunk(lambda lo, n: slice(lo, lo + n), stats=stats0)
    cp_wql.wait()

    def ln1_body(j, carry):
        src = jnp.minimum(j + 1, NXC - 1)

        @pl.when(j + 1 < NXC)
        def _():
            x_copy(src, src + 2).wait()

        zvec = jnp.full((8, LANES), z_scr[0, 0], I32)
        nb = xw // LANES
        half = LANES // 2
        lhs = [hn_scr[b * half:(b + 1) * half, :] for b in range(nb)]
        for b in range(nb):
            h_scr[pl.ds(pl.multiple_of(j * (xw // 2) + b * half, half), half), :] = lhs[b]
        marks = []
        ln1_chunk(lambda lo, n: pl.ds(pl.multiple_of(src * xw + lo, n), n), marks.append)
        na = d // 32
        times = ([lt0 + lsp * i for i in range(na)] + [lt0 + lsp * na + lst]
                 + [lt0 + lsp * na + lst + lxp + lsc * i for i in range(len(marks) - na - 1)])
        dur = LANES * len(fch) * rep // 4
        ties = {}
        for t, v in zip(times, marks):
            b, off = t // dur, t % dur
            if off >= 2 * LANES:
                b, off = b + 1, 0
            if b < nb:
                v = v if v.dtype == I32 else pltpu.bitcast(v, I32)
                bits = v[:, 0:LANES] if v.shape[1] >= LANES else jnp.concatenate([v, v], axis=1)
                for c0 in range(LANES, v.shape[1], LANES):
                    bits = bits | v[:, c0:c0 + LANES]
                where = (b, off % LANES // 16, 0 if off < LANES else len(fch) - 1)
                ties[where] = bits if where not in ties else ties[where] | bits
        for b in range(nb):
            grid = [[lhs[b][r * 8:(r + 1) * 8, fs] for fs in fch] for r in range(half // 8)]
            for (bb, r, k), bits in ties.items():
                if bb == b:
                    grid[r][k] = grid[r][k] | (bits & zvec)[:, 0:grid[r][k].shape[1]]
            hb = jnp.concatenate([jnp.concatenate(row, axis=1) for row in grid], axis=0)
            q = jnp.dot(pltpu.bitcast(hb, BF16), wql_v[...], preferred_element_type=F32)
            q = (q * qscale).astype(BF16)
            for r in range(rep):
                lo = r * tg + (b % nlt) * LANES
                q_scr[j * per + b // nlt, lo:lo + LANES, :] = q[:, r * DH:(r + 1) * DH]
        return carry

    jax.lax.fori_loop(0, NXC, ln1_body, 0)

    steady = 'V Q0 Q1 K0 ! ' + ' '.join(
        ('O%d ' % (i - 2) if i >= 2 else '') + ('Q%d ' % (i + 2) if i + 2 < ng else '')
        + ('S%d' % i if i + 1 < ng else 'P%d' % i) for i in range(ng)
    ) + ' O%d O%d' % (ng - 2, ng - 1)

    def group_body(g, carry):
        slot = g & 1
        for cp in group_copies(g, slot):
            cp.wait()

        @pl.when(g == 2)
        def _():
            cp_m1.wait()

        def prefetch():
            for cp in group_copies(g + 1, 1 - slot):
                cp.start()
            for j, cp in enumerate((cp_m1,) + cp_tail):
                @pl.when(g == j)
                def _(cp=cp):
                    cp.start()

        attention(slot, list(range(ng)), steady, hook=prefetch, dt=dtm,
                  job=_chain(col_job(jnp.clip(g - (lastg - 5), 0, 4)), mod_job(g)))
        return carry
    jax.lax.fori_loop(0, lastg, group_body, 0)

    for cp in group_copies(lastg, lastg % 2) + cp_tail:
        cp.wait()
    npair = ng // 2

    def last_body(t, carry):
        prev = (t + npair - 1) % npair
        attention(lastg % 2, [2 * t, 2 * t + 1], 'V L0 L1 K0 K1 P0 P1 O0 O1', last=True,
                  job=_mix(_chain(ln2_job(2 * prev), ln2_job(2 * prev + 1)), wd_job(t, npair), 4))
        return carry
    jax.lax.fori_loop(0, npair, last_body, 0)
    rest = _chain(ln2_job(ng - 2), ln2_job(ng - 1))
    next(rest)
    _finish(rest)

    ibits = (s_len - 1).bit_length()
    imask = (1 << ibits) - 1
    bits = pltpu.bitcast(_rnd(r_scr[...]), I32)
    pos = (jax.lax.broadcasted_iota(I32, bits.shape, 0) * LANES
           + jax.lax.broadcasted_iota(I32, bits.shape, 1))
    order = ((bits ^ ((bits >> 31) & 0x7FFFFFFF)) >> 16) + 0x8000
    key = pltpu.bitcast((order << ibits) + (imask - pos) + 0x20000000, F32)
    subl = jax.lax.broadcasted_iota(I32, (TOPC, LANES), 0)
    lane = jax.lax.broadcasted_iota(I32, (TOPC, LANES), 1)
    idxs, blks, bcols = [], [], []
    keyv = jnp.zeros((TOPC, LANES), I32)
    x_sel = jnp.zeros((TOPC, d), F32)
    x1_sel = jnp.zeros((TOPC, d), F32)
    for c in range(TOPC):
        top = jnp.max(jnp.max(key, axis=0, keepdims=True), axis=1, keepdims=True)
        key = jnp.where(key == top, 0.0, key)
        topi = pltpu.bitcast(jnp.broadcast_to(top, (TOPC, LANES)), I32)
        keyv = jnp.where(subl == c, topi, keyv)
        ixv = imask - (topi & imask)
        idxs.append(ixv[0, 0])
        blks.append(idxs[c] // LANES)
        bcols.append(pl.ds(pl.multiple_of(blks[c] * LANES, LANES), LANES))
        pick = jnp.where((lane == (ixv & (LANES - 1))) & (subl == c), 1.0, 0.0).astype(BF16)
        x_sel = x_sel + jax.lax.dot_general(pick, xh_scr[0:d, bcols[c]], NT,
                                            preferred_element_type=F32)
        x1_sel = x1_sel + jax.lax.dot_general(pick, xh_scr[d:2 * d, bcols[c]], NT,
                                              preferred_element_type=F32)

    for b in range(nblk):
        hit = blks[0] == b
        for bb in blks[1:]:
            hit = jnp.logical_or(hit, bb == b)

        @pl.when(jnp.logical_not(hit))
        def _(b=b):
            out_start(slice(0, d), slice(b * LANES, (b + 1) * LANES))

    final = []
    for c in range(TOPC):
        u = True
        for other in blks[c + 1:]:
            u = jnp.logical_and(u, other != blks[c])
        final.append(jnp.asarray(u))

    ob = (((keyv - 0x20000000) >> ibits) - 0x8000) << 16
    r_sel = pltpu.bitcast((ob ^ ((ob >> 31) & 0x7FFFFFFF)) & ~0xFFFF, F32)
    xs = x_sel.astype(BF16)
    gt = _rnd(jnp.dot(xs, wg_v[...], preferred_element_type=F32))
    gt = _rnd(gt * jax.nn.sigmoid(gt))
    up = _rnd(jnp.dot(xs, wu_v[...], preferred_element_type=F32))
    gu = (gt * up).astype(BF16)
    gate_r = jnp.concatenate([_rnd(jax.nn.sigmoid(r_sel))] * pl.cdiv(d, LANES), axis=1)

    def down(fs):
        y = _rnd(jnp.dot(gu, pltpu.bitcast(wd_scr[:, fs], BF16), preferred_element_type=F32))
        y = _rnd(y * gate_r[:, fs])
        return x1_sel[:, fs] + _rnd(row_scr[3, :, fs] * _rnd(x_sel[:, fs] + y))

    def patch(fs, new):
        n = fs.stop - fs.start
        lane_d = jax.lax.broadcasted_iota(I32, (n // 2, LANES), 1)
        for c in range(TOPC):
            ln = idxs[c] & (LANES - 1)
            wide = jnp.broadcast_to(new[c:c + 1], (LANES, n)).astype(BF16).T
            moved = pltpu.bitcast(wide, I32)
            cur = pltpu.bitcast(out_v[fs, bcols[c]], I32)
            out_v[fs, bcols[c]] = pltpu.bitcast(jnp.where(lane_d == ln, moved, cur), BF16)

            @pl.when(final[c])
            def _(c=c):
                out_start(fs, bcols[c])

    pch = [slice(a, b) for a, b in zip((0,) + cuts, cuts + (d,))]
    new_scr[:, pch[0]] = down(pch[0])
    for j in range(len(pch)):
        @pl.when(z_scr[0, 0] == 0)
        def _(j=j):
            prev = new_scr[:, pch[j]]
            if j + 1 < len(pch):
                new_scr[:, pch[j + 1]] = down(pch[j + 1])
            patch(pch[j], prev)
    pltpu.make_async_copy(out_v, out_hbm, sem.at[1]).wait()


def _build(ahead=384, ahp=320, kcp=256, oh=144, lw=32, dt=80, dl=320, rc2=32,
          marg=128, sub=64, cuts=(256, 512), mrows=64, dtm=150, cw=256, lt0=40, lsp=28, lst=150, lxp=230, lsc=56, cdl=600):
    @jax.jit
    def pallas_adaLN_cond__gqa_block_cached__moe_arch_mod__prompt_kernel(
            A_x, A_k_cache, A_v_cache, A_wq, A_wo, B_x, B_w_r, B_w_gate, B_w_up, B_w_down, c, w_mod):
        b, s_len, d = A_x.shape
        assert b == 1
        hkv, sk = A_k_cache.shape[1], A_k_cache.shape[2]
        rep = HQ // hkv
        f = B_w_gate.shape[1]
        tg = GW // rep
        scratch = [
            pltpu.VMEM((1, d, s_len), BF16),
            pltpu.VMEM((2, sk, DH), BF16),
            pltpu.VMEM((2, sk, DH), BF16),
            pltpu.VMEM((2, d, rep * DH), BF16),
            pltpu.VMEM((2, d, rep * DH), BF16),
            pltpu.VMEM((d, rep * DH), BF16),
            pltpu.VMEM((s_len // tg, GW, DH), BF16),
            pltpu.VMEM((d,), BF16),
            pltpu.VMEM((1, d), BF16),
            pltpu.VMEM((d, 6 * d), BF16),
            pltpu.VMEM((d, f), BF16),
            pltpu.VMEM((d, f), BF16),
            pltpu.VMEM((d, f), BF16),
            pltpu.VMEM((f // 2, d), I32),
            pltpu.VMEM((d, s_len), BF16),
            pltpu.VMEM((s_len // 2, d), I32),
            pltpu.VMEM((d, s_len), F32),
            pltpu.VMEM((5, 8, d), F32),
            pltpu.VMEM((5, d, LANES), F32),
            pltpu.VMEM((1, DH // 2, sk), I32),
            pltpu.VMEM((2 * d, s_len), BF16),
            pltpu.VMEM((s_len // LANES, LANES), F32),
            pltpu.VMEM((3, 8, s_len), F32),
            pltpu.VMEM((1, sk, GW), F32),
            pltpu.VMEM((1, sk, GW), F32),
            pltpu.SMEM((8, LANES), I32),
            pltpu.VMEM((8, LANES), I32),
            pltpu.VMEM((TOPC, d), F32),
            pltpu.VMEM((d, LANES), F32),
            pltpu.VMEM((8, 6 * d + (d // LANES + 1) * LANES), F32),
            pltpu.VMEM((s_len // NXC // 2, d), I32),
            pltpu.SemaphoreType.DMA((NXC + 4,)),
        ]
        out = pl.pallas_call(
            functools.partial(_kernel, n_groups=hkv, rep=rep, ahead=ahead,
                              ahp=ahp, kcp=kcp, oh=oh, lw=lw, dt=dt, dl=dl, rc2=rc2, marg=marg,
                              sub=sub, cuts=cuts, mrows=mrows, dtm=dtm, cw=cw, lt0=lt0, lsp=lsp,
                              lst=lst, lxp=lxp, lsc=lsc, cdl=cdl),
            in_specs=[pl.BlockSpec(memory_space=pl.ANY)] * 11,
            out_specs=pl.BlockSpec(memory_space=pl.ANY),
            out_shape=jax.ShapeDtypeStruct((d, s_len), BF16),
            scratch_shapes=scratch,
            compiler_params=pltpu.CompilerParams(vmem_limit_bytes=100 * 1024 * 1024),
        )(A_x.reshape(s_len, d).T, A_k_cache.reshape(hkv, sk, DH), A_v_cache.reshape(hkv, sk, DH),
          A_wq, A_wo.T, B_w_r, c, w_mod, B_w_gate, B_w_up, B_w_down.T)
        return out.T.reshape(b, s_len, d)
    return pallas_adaLN_cond__gqa_block_cached__moe_arch_mod__prompt_kernel


pallas_adaLN_cond__gqa_block_cached__moe_arch_mod__prompt_kernel = _build()
```

```python
import functools

import jax
import jax.numpy as jnp
import jax.experimental.pallas as pl
import jax.experimental.pallas.tpu as pltpu

HQ = 32
DH = 128
TOPC = 8
LN_EPS = 1.0013580322265625e-05
LOG2E = 1.4426950408889634
F32 = jnp.float32
BF16 = jnp.bfloat16
I32 = jnp.int32
NT = (((1,), (1,)), ((), ()))
LANES = 128
GW = 512
MXU_LAT = 128
NXC = 4


def _rnd(v):
    return v.astype(BF16).astype(F32)


def _by8(v):
    return v.reshape(v.shape[0] // 8, 8, v.shape[1])


class _Moments:
    def __init__(self):
        self.shift = self.s1 = self.s2 = None

    def add(self, v):
        if self.shift is None:
            self.shift = jnp.broadcast_to(v[0:1], (8, v.shape[1]))
        dv = _by8(v) - self.shift[None]
        a, b = jnp.sum(dv, axis=0), jnp.sum(dv * dv, axis=0)
        self.s1, self.s2 = (a, b) if self.s1 is None else (self.s1 + a, self.s2 + b)

    def stats(self, d):
        e1 = jnp.sum(self.s1, axis=0, keepdims=True) * (1.0 / d)
        e2 = jnp.sum(self.s2, axis=0, keepdims=True) * (1.0 / d)
        var = jnp.maximum(e2 - e1 * e1, 0.0)
        den = _rnd(jnp.sqrt(_rnd(_rnd(var) + LN_EPS)))
        return _rnd(self.shift + e1), jnp.broadcast_to(1.0 / den, self.shift.shape)


def _chain(*jobs):
    gate = yield
    for job in jobs:
        next(job)
        while True:
            try:
                v = job.send(gate)
            except StopIteration:
                break
            gate = yield v


def _mix(a, b, every):
    next(a)
    next(b)
    gate = yield
    n, live = 0, [a, b]
    while live:
        n += 1
        job = b if (b in live and (n % (every + 1) == 0 or a not in live)) else a
        try:
            v = job.send(gate)
        except StopIteration:
            live.remove(job)
            continue
        gate = yield v


def _finish(job):
    try:
        while True:
            job.send(lambda t: t)
    except StopIteration:
        pass


def _kernel(xt_hbm, k_hbm, v_hbm, wq_hbm, wot_hbm, wr_hbm, c_hbm, wmod_hbm,
            wg_hbm, wu_hbm, wdt_hbm,
            out_hbm,
            xt_v, kbuf, vbuf, wqbuf, wobuf, wql_v, q_scr,
            wr_v, c_v, wmod_v, wg_v, wu_v, wdt_v, wd_scr, out_v,
            h_scr, acc_scr, row_scr, col_scr, vt_scr, xh_scr, r_scr, st_scr, s0_scr, s1_scr,
            z_scr, zv_scr, new_scr, cc_scr, mod_scr, hn_scr, sem, *,
            n_groups, rep, ahead, ahp, kcp, oh, lw, dt, dl, rc2, marg, sub, cuts,
            mrows, dtm, cw, lt0, lsp, lst, lxp, lsc, cdl):
    _, d, s_len = xt_v.shape
    sk = kbuf.shape[1]
    gcols = rep * DH
    tg = GW // rep
    ng = s_len // tg
    nblk = s_len // LANES
    nlt = tg // LANES
    xw = s_len // NXC
    per = xw // tg
    lastg = n_groups - 1
    s_bufs = (s0_scr, s1_scr)
    cpad = (d // LANES + 1) * LANES
    assert d % LANES == LANES // 2 and n_groups >= 5 + 4 * d // (2 * LANES)
    qscale = (DH ** -0.5) * LOG2E

    def group_copies(g, slot):
        cols = pl.ds(pl.multiple_of(g * gcols, gcols), gcols)
        s = sem.at[NXC + 2 + slot]
        return (pltpu.make_async_copy(wq_hbm.at[:, cols], wqbuf.at[slot], s),
                pltpu.make_async_copy(k_hbm.at[g], kbuf.at[slot], s),
                pltpu.make_async_copy(v_hbm.at[g], vbuf.at[slot], s),
                pltpu.make_async_copy(wot_hbm.at[:, cols], wobuf.at[slot], s))

    def x_copy(j, s):
        cols = pl.ds(pl.multiple_of(j * xw, xw), xw)
        return pltpu.make_async_copy(xt_hbm.at[:, cols], xt_v.at[0, :, cols], sem.at[s])

    cp_z = pltpu.make_async_copy(zv_scr, z_scr, sem.at[0])
    cp_c = pltpu.make_async_copy(c_hbm, c_v, sem.at[0])
    cp_m0 = pltpu.make_async_copy(wmod_hbm.at[:, 0:2 * d], wmod_v.at[:, 0:2 * d], sem.at[1])
    cp_wql = pltpu.make_async_copy(wq_hbm.at[:, lastg * gcols:(lastg + 1) * gcols], wql_v,
                                   sem.at[2])
    cp_m1 = pltpu.make_async_copy(wmod_hbm.at[:, 2 * d:6 * d], wmod_v.at[:, 2 * d:6 * d], sem.at[2])
    cp_wr = pltpu.make_async_copy(wr_hbm, wr_v, sem.at[0])
    cp_tail = (pltpu.make_async_copy(wg_hbm, wg_v, sem.at[0]),
               pltpu.make_async_copy(wu_hbm, wu_v, sem.at[0]),
               pltpu.make_async_copy(wdt_hbm, wdt_v, sem.at[0]))

    def out_start(rows, cols):
        pltpu.make_async_copy(out_v.at[rows, cols], out_hbm.at[rows, cols], sem.at[1]).start()

    def silu_c():
        cf = c_v[...].astype(F32)
        return (cf * jax.nn.sigmoid(cf)).astype(BF16)

    def mod_job(g):
        gate = yield
        mw = 2 * LANES
        lo = jnp.where(g < 2, 0, 2 * d + mw * jnp.minimum(g - 2, 4 * d // mw - 1))
        cols = pl.ds(pl.multiple_of(lo, LANES), mw)
        acc = jnp.zeros((8, mw), F32)
        for r0 in range(0, d, mrows):
            cc = jnp.concatenate([cc_scr[r0:r0 + mrows, :]] * 2, axis=1)
            prod = _by8(wmod_v[r0:r0 + mrows, cols].astype(F32) * cc)
            acc = gate(acc) + jnp.sum(prod, axis=0)
            if r0 + mrows == d:
                mod_scr[:, cols] = jnp.broadcast_to(jnp.sum(acc, axis=0, keepdims=True), (8, mw))
            gate = yield acc

    def col_job(j):
        gate = yield
        lo = pl.multiple_of((2 + j) * d // LANES * LANES, LANES)
        w = _rnd(gate(mod_scr[:, pl.ds(lo, cpad)]))
        row = jnp.where((2 + j) * d == lo, w[:, 0:d], w[:, cpad - d:cpad])
        row = jnp.where(j == 2, _rnd(1.0 + row), row)
        row_scr[j] = row
        col_scr[j] = to_col(row[0:1])
        gate = yield col_scr[0, 0:8, :], cdl

    def tspan(i, lo, n):
        if isinstance(i, int):
            return slice(i * tg + lo, i * tg + lo + n)
        return pl.ds(pl.multiple_of(i * tg + lo, n), n)

    def tcols(i):
        return tspan(i, 0, tg)

    def col(j, rows, tiles=nlt):
        return jnp.concatenate([col_scr[j, rows, :]] * tiles, axis=1)

    fch = [slice(lo, min(lo + LANES, d)) for lo in range(0, d, LANES)]

    def ln1_chunk(cols_of, mark=lambda v: None, stats=None):
        if stats is None:
            mo = _Moments()
            for r0 in range(0, d, 32):
                mo.add(xt_v[0, r0:r0 + 32, cols_of(0, xw)].astype(F32))
                mark(mo.s2)
            stats = mo.stats(d)
            mark(stats[1])
        mean, rinv = stats
        for b in range(0, xw, cw):
            for rows in fch:
                wide = lambda j: jnp.concatenate([col_scr[j, rows, :]] * (cw // LANES), axis=1)
                x = _by8(xt_v[z_scr[0, 0], rows, cols_of(b, cw)].astype(F32))
                y = ((x - mean[None, :, b:b + cw]) * rinv[None, :, b:b + cw]).reshape(-1, cw)
                h32 = pltpu.bitcast((y * wide(1) + wide(0)).astype(BF16).T, I32)
                hn_scr[b // 2:(b + cw) // 2, rows] = h32
                mark(h32[cw // 2 - 8:cw // 2])

    def to_col(row):
        return jnp.broadcast_to(row, (LANES, d)).T

    def project_q(tok, wq_ref, step=lambda *a: None):
        parts = []
        for lt in range(nlt):
            lo = tok * (tg // 2) + lt * (LANES // 2)
            rows = (slice(lo, lo + LANES // 2) if isinstance(tok, int)
                    else pl.ds(pl.multiple_of(lo, LANES // 2), LANES // 2))
            q = jnp.dot(pltpu.bitcast(h_scr[rows, :], BF16), wq_ref[...],
                        preferred_element_type=F32)
            step(q, LANES * pl.cdiv(d, LANES) * rep // 4)
            parts.append((q * qscale).astype(BF16))
        return jnp.concatenate([p[:, r * DH:(r + 1) * DH] for r in range(rep) for p in parts],
                               axis=0)

    def ln2_job(i, n=2, rc=rc2):
        gate = yield
        cols, tiles = tspan(i, 0, n * tg), n * nlt
        mo = _Moments()
        mo.shift, mo.s1, mo.s2 = (st_scr[j, :, cols] for j in range(3))
        mean, rinv = mo.stats(d)
        racc = None
        for r0 in range(0, d, rc):
            rows = slice(r0, r0 + rc)
            x1 = xh_scr[d + r0:d + r0 + rc, cols].astype(F32)
            xc = (_by8(x1) - gate(mean)[None]).reshape(x1.shape)
            y = _rnd((_by8(_rnd(xc)) * rinv[None]).reshape(x1.shape))
            h2b = (_rnd(y * col(2, rows, tiles)) + col(1, rows, tiles)).astype(BF16)
            h2 = h2b.astype(F32)
            xh_scr[rows, cols] = h2b
            out_v[rows, cols] = (x1 + col(3, rows, tiles) * h2).astype(BF16)
            part = jnp.sum(_by8(h2 * col(4, rows, tiles)), axis=0)
            racc = part if racc is None else racc + part
            if r0 + rc == d:
                r = jnp.sum(racc, axis=0, keepdims=True)
                for lt in range(tiles):
                    r_scr[pl.ds(i * nlt + lt, 1), :] = r[:, lt * LANES:(lt + 1) * LANES]
            gate = yield racc

    def wd_job(t, parts):
        gate = yield
        fw = wdt_v.shape[1] // parts
        for f0 in range(0, fw, LANES):
            lo = pl.multiple_of(t * fw + f0, LANES)
            w32 = pltpu.bitcast(wdt_v[:, pl.ds(lo, LANES)], I32)
            w32 = gate(_by8(w32)).reshape(w32.shape)
            wd = pltpu.bitcast(w32, BF16).T
            half = pl.multiple_of(t * (fw // 2) + f0 // 2, LANES // 2)
            wd_scr[pl.ds(half, LANES // 2), :] = pltpu.bitcast(wd, I32)
            gate = yield wd_scr[0:8, 0:LANES]

    def attention(slot, toks, sched, last=False, job=None, hook=None, dt=dt):
        wq_ref, k_ref, v_ref, wot_ref = (wqbuf.at[slot], kbuf.at[slot], vbuf.at[slot],
                                         wobuf.at[slot])
        zero = z_scr[0, 0]
        zvec = jnp.full((8, LANES), zero, I32)
        st = dict(clock=0, nxt=0, job=job)
        hist = []
        due = []
        if job is not None:
            next(job)

        def token(when):
            want = when - MXU_LAT
            for start, dur, res in reversed(hist):
                if start <= want:
                    row = min((want - start) * res.shape[0] // dur // 8 * 8, res.shape[0] - 8)
                    return pltpu.bitcast(res[row:row + 8, 0:LANES], I32) & zvec
            return None

        def tie(x, tok):
            if tok is None:
                return x
            if x.shape[-1] > LANES:
                tok = jnp.concatenate([tok] * (x.shape[-1] // LANES), axis=1)
            if x.ndim == 3:
                tok = tok[None]
            if x.dtype == I32:
                return x | tok
            return pltpu.bitcast(pltpu.bitcast(x, I32) | tok, x.dtype)

        def tie_due(x, now):
            while due and due[0][0] <= now:
                v = due.pop(0)[1]
                v = v if v.dtype == I32 else pltpu.bitcast(v, I32)
                bits = v[:, 0:LANES]
                for j in range(1, v.shape[1] // LANES):
                    bits = bits | v[:, j * LANES:(j + 1) * LANES]
                x = tie(x, bits & zvec)
            return x

        def side(upto):
            while st['job'] is not None and st['nxt'] <= upto:
                tok = token(st['nxt'] + MXU_LAT)
                try:
                    v = st['job'].send(lambda x, tok=tok: tie(x, tok))
                except StopIteration:
                    st['job'] = None
                    break
                v, extra = v if isinstance(v, tuple) else (v, 0)
                due.append((st['nxt'] + dl + extra, v))
                due.sort(key=lambda e: e[0])
                st['nxt'] += dt

        def step(result, dur, advance=None):
            hist.append((st['clock'], dur, result))
            st['clock'] += dur if advance is None else advance

        def scores(qg, buf, rows, cols, advance=None):
            s = jax.lax.dot_general(k_ref[rows, :], qg[cols], NT, preferred_element_type=F32)
            s_bufs[buf][zero, rows, cols] = s
            step(s, s.shape[0], advance)
            return s

        def max_fin(m):
            return jnp.broadcast_to(jnp.max(m, axis=0, keepdims=True), m.shape)

        def qk(qg, buf):
            m = None
            st['nxt'] = max(st['nxt'], st['clock'])
            stop = st['clock'] + sk - marg
            for j in range(4):
                t0 = st['clock']
                s = scores(qg, buf, slice(j * sk // 4, (j + 1) * sk // 4), slice(0, GW))
                blk = s.shape[0] if job is None else sub
                for r0 in range(0, s.shape[0], blk):
                    mj = jnp.max(_by8(s[r0:r0 + blk]), axis=0)
                    if m is not None:
                        m0 = tie_due(m[:, 0:LANES], t0 + r0)
                        mj = jnp.maximum(jnp.concatenate([m0, m[:, LANES:]], axis=1), mj)
                    m = mj
                    side(min(t0 + r0 + blk - 1, stop))
            return max_fin(m)

        def pv_unit(buf, m, u, kc, advance, lead):
            cs = slice(u * LANES, (u + 1) * LANES)
            o = l = None
            for j in range(sk // kc):
                when = st['clock'] - lead
                mu = tie_due(tie(m[:, cs], token(when)), when)
                p = jnp.exp2(_by8(s_bufs[buf][0, j * kc:(j + 1) * kc, cs]) - mu[None])
                lj = jnp.sum(p.reshape(kc // lw, lw, LANES), axis=0)
                oj = jnp.dot(pltpu.bitcast(vt_scr[0, :, j * kc:(j + 1) * kc], BF16),
                             p.reshape(kc, LANES).astype(BF16), preferred_element_type=F32)
                o = oj if o is None else o + oj
                l = lj if l is None else l + lj
                step(oj, DH, advance)
            return (o / jnp.sum(l, axis=0, keepdims=True)).astype(BF16)

        def heads_major(outs):
            return jnp.concatenate(
                [jnp.concatenate(outs[r * nlt:(r + 1) * nlt], axis=1) for r in range(rep)], axis=0)

        def pv(buf, m):
            return heads_major([pv_unit(buf, m, u, kcp, kcp // 4, ahp) for u in range(4)])

        def pv_qk(buf, m, qn, nbuf):
            outs, mns = [], []
            for half in range(2):
                s = scores(qn, nbuf, slice(0, sk), slice(half * GW // 2, (half + 1) * GW // 2), 0)
                mns.append(jnp.max(_by8(s), axis=0))
                outs += [pv_unit(buf, m, u, 2 * LANES, DH, ahead) for u in (2 * half, 2 * half + 1)]
            return heads_major(outs), max_fin(jnp.concatenate(mns, axis=1))

        def oproj(tok, ot):
            cols = tcols(tok)
            mo = _Moments()
            for r0 in range(0, d, oh):
                rows = slice(r0, r0 + oh)
                res = jnp.dot(wot_ref[rows, :], ot, preferred_element_type=F32)
                attn = res + acc_scr[rows, cols]
                if last:
                    x1b = (xt_v[0, rows, cols].astype(F32) + col(0, rows) * attn).astype(BF16)
                    xh_scr[d + r0:d + r0 + oh, cols] = x1b
                    mo.add(x1b.astype(F32))
                else:
                    acc_scr[rows, cols] = attn
                step(res, oh)
            if last:
                for j, v in enumerate((mo.shift, mo.s1, mo.s2)):
                    st_scr[j, :, cols] = v

        qs, ots, ms, bufs, free = {}, {}, {}, {}, [0, 1]
        for item in sched.split():
            kind, i = item[0], int(item[1:] or 0)
            if kind == '!':
                hook()
            elif kind == 'V':
                vt_scr[zero] = pltpu.bitcast(v_ref[...].T, I32)
            elif kind == 'Q':
                qs[i] = project_q(toks[i], wq_ref, step)
            elif kind == 'L':
                qs[i] = q_scr[toks[i]]
            elif kind == 'K':
                bufs[i] = free.pop(0)
                ms[i] = qk(qs[i], bufs[i])
            elif kind == 'P':
                ots[i] = pv(bufs[i], ms[i])
                free.append(bufs[i])
            elif kind == 'S':
                bufs[i + 1] = free.pop(0)
                ots[i], ms[i + 1] = pv_qk(bufs[i], ms[i], qs[i + 1], bufs[i + 1])
                free.append(bufs[i])
            elif kind == 'O':
                oproj(toks[i], ots[i])
        if st['job'] is not None:
            _finish(st['job'])

    zv_scr[...] = jnp.zeros(zv_scr.shape, I32)
    for cp in ((cp_z, cp_c, cp_wr, x_copy(0, 0), cp_m0, cp_wql)
               + tuple(x_copy(j, j + 2) for j in range(1, NXC)) + group_copies(0, 0)):
        cp.start()

    def zero_body(j, carry):
        rows = pl.ds(pl.multiple_of(j * 32, 32), 32)
        acc_scr[rows, :] = jnp.zeros((32, s_len), F32)
        xh_scr[pl.ds(pl.multiple_of(d + j * 32, 32), 32), s_len - 2 * tg:s_len] = (
            jnp.zeros((32, 2 * tg), BF16))
        return carry

    jax.lax.fori_loop(0, d // 32, zero_body, 0)
    st_scr[:, :, s_len - 2 * tg:s_len] = jnp.zeros((3, 8, 2 * tg), F32)
    mod_scr[...] = jnp.zeros(mod_scr.shape, F32)
    cp_z.wait()
    cp_c.wait()
    cp_wr.wait()
    x_copy(0, 0).wait()

    mo0 = _Moments()
    for r0 in range(0, d, 32):
        mo0.add(xt_v[0, r0:r0 + 32, 0:xw].astype(F32))
    stats0 = mo0.stats(d)
    cc_scr[...] = to_col(silu_c()).astype(F32)
    mod_scr[:, 6 * d:7 * d] = jnp.broadcast_to(wr_v[...].astype(F32).reshape(1, d), (8, d))
    cp_m0.wait()
    mod = _rnd(jnp.dot(jnp.broadcast_to(silu_c(), (8, d)), wmod_v[:, 0:2 * d],
                       preferred_element_type=F32))
    col_scr[z_scr[0, 0]] = to_col(mod[0:1, 0:d])
    col_scr[z_scr[0, 0] + 1] = to_col(_rnd(1.0 + mod[0:1, d:2 * d]))
    ln1_chunk(lambda lo, n: slice(lo, lo + n), stats=stats0)
    cp_wql.wait()

    def ln1_body(j, carry):
        src = jnp.minimum(j + 1, NXC - 1)

        @pl.when(j + 1 < NXC)
        def _():
            x_copy(src, src + 2).wait()

        zvec = jnp.full((8, LANES), z_scr[0, 0], I32)
        nb = xw // LANES
        half = LANES // 2
        lhs = [hn_scr[b * half:(b + 1) * half, :] for b in range(nb)]
        for b in range(nb):
            h_scr[pl.ds(pl.multiple_of(j * (xw // 2) + b * half, half), half), :] = lhs[b]
        marks = []
        ln1_chunk(lambda lo, n: pl.ds(pl.multiple_of(src * xw + lo, n), n), marks.append)
        na = d // 32
        times = ([lt0 + lsp * i for i in range(na)] + [lt0 + lsp * na + lst]
                 + [lt0 + lsp * na + lst + lxp + lsc * i for i in range(len(marks) - na - 1)])
        dur = LANES * len(fch) * rep // 4
        ties = {}
        for t, v in zip(times, marks):
            b, off = t // dur, t % dur
            if off >= 2 * LANES:
                b, off = b + 1, 0
            if b < nb:
                v = v if v.dtype == I32 else pltpu.bitcast(v, I32)
                bits = v[:, 0:LANES] if v.shape[1] >= LANES else jnp.concatenate([v, v], axis=1)
                for c0 in range(LANES, v.shape[1], LANES):
                    bits = bits | v[:, c0:c0 + LANES]
                where = (b, off % LANES // 16, 0 if off < LANES else len(fch) - 1)
                ties[where] = bits if where not in ties else ties[where] | bits
        for b in range(nb):
            grid = [[lhs[b][r * 8:(r + 1) * 8, fs] for fs in fch] for r in range(half // 8)]
            for (bb, r, k), bits in ties.items():
                if bb == b:
                    grid[r][k] = grid[r][k] | (bits & zvec)[:, 0:grid[r][k].shape[1]]
            hb = jnp.concatenate([jnp.concatenate(row, axis=1) for row in grid], axis=0)
            q = jnp.dot(pltpu.bitcast(hb, BF16), wql_v[...], preferred_element_type=F32)
            q = (q * qscale).astype(BF16)
            for r in range(rep):
                lo = r * tg + (b % nlt) * LANES
                q_scr[j * per + b // nlt, lo:lo + LANES, :] = q[:, r * DH:(r + 1) * DH]
        return carry

    jax.lax.fori_loop(0, NXC, ln1_body, 0)

    steady = 'V Q0 Q1 K0 ! ' + ' '.join(
        ('O%d ' % (i - 2) if i >= 2 else '') + ('Q%d ' % (i + 2) if i + 2 < ng else '')
        + ('S%d' % i if i + 1 < ng else 'P%d' % i) for i in range(ng)
    ) + ' O%d O%d' % (ng - 2, ng - 1)

    def group_body(g, carry):
        slot = g & 1
        for cp in group_copies(g, slot):
            cp.wait()

        @pl.when(g == 2)
        def _():
            cp_m1.wait()

        def prefetch():
            for cp in group_copies(g + 1, 1 - slot):
                cp.start()
            for j, cp in enumerate((cp_m1,) + cp_tail):
                @pl.when(g == j)
                def _(cp=cp):
                    cp.start()

        attention(slot, list(range(ng)), steady, hook=prefetch, dt=dtm,
                  job=_chain(col_job(jnp.clip(g - (lastg - 5), 0, 4)), mod_job(g)))
        return carry

    jax.lax.fori_loop(0, lastg, group_body, 0)

    for cp in group_copies(lastg, lastg % 2) + cp_tail:
        cp.wait()
    npair = ng // 2

    def last_body(t, carry):
        prev = (t + npair - 1) % npair
        attention(lastg % 2, [2 * t, 2 * t + 1], 'V L0 L1 K0 K1 P0 P1 O0 O1', last=True,
                  job=_mix(ln2_job(2 * prev), wd_job(t, npair), 4))
        return carry

    jax.lax.fori_loop(0, npair, last_body, 0)
    rest = ln2_job(ng - 2)
    next(rest)
    _finish(rest)

    ibits = (s_len - 1).bit_length()
    imask = (1 << ibits) - 1
    bits = pltpu.bitcast(_rnd(r_scr[...]), I32)
    pos = (jax.lax.broadcasted_iota(I32, bits.shape, 0) * LANES
           + jax.lax.broadcasted_iota(I32, bits.shape, 1))
    order = ((bits ^ ((bits >> 31) & 0x7FFFFFFF)) >> 16) + 0x8000
    key = pltpu.bitcast((order << ibits) + (imask - pos) + 0x20000000, F32)
    subl = jax.lax.broadcasted_iota(I32, (TOPC, LANES), 0)
    lane = jax.lax.broadcasted_iota(I32, (TOPC, LANES), 1)
    subd = jax.lax.broadcasted_iota(I32, (TOPC, d), 0)
    idxs, blks, bcols = [], [], []
    keyv = jnp.zeros((TOPC, LANES), I32)
    x_sel = jnp.zeros((TOPC, d), F32)
    x1_sel = jnp.zeros((TOPC, d), F32)
    for c in range(TOPC):
        top = jnp.max(jnp.max(key, axis=0, keepdims=True), axis=1, keepdims=True)
        key = jnp.where(key == top, 0.0, key)
        topi = pltpu.bitcast(jnp.broadcast_to(top, (TOPC, LANES)), I32)
        keyv = jnp.where(subl == c, topi, keyv)
        ixv = imask - (topi & imask)
        idxs.append(ixv[0, 0])
        blks.append(jnp.clip(idxs[c] >> (LANES.bit_length() - 1), 0, nblk - 1))
        bcols.append(pl.ds(pl.multiple_of(blks[c] * LANES, LANES), LANES))
        pick = jnp.where(lane == (ixv & (LANES - 1)), 1.0, 0.0).astype(BF16)
        take = lambda rows: jax.lax.dot_general(pick, xh_scr[rows, bcols[c]], NT,
                                                preferred_element_type=F32)
        x_sel = jnp.where(subd == c, take(slice(0, d)), x_sel)
        x1_sel = jnp.where(subd == c, take(slice(d, 2 * d)), x1_sel)

    for b in range(nblk):
        hit = blks[0] == b
        for bb in blks[1:]:
            hit = jnp.logical_or(hit, bb == b)

        @pl.when(jnp.logical_not(hit))
        def _(b=b):
            out_start(slice(0, d), slice(b * LANES, (b + 1) * LANES))

    final = []
    for c in range(TOPC):
        u = True
        for other in blks[c + 1:]:
            u = jnp.logical_and(u, other != blks[c])
        final.append(jnp.asarray(u))

    ob = (((keyv - 0x20000000) >> ibits) - 0x8000) << 16
    r_sel = pltpu.bitcast((ob ^ ((ob >> 31) & 0x7FFFFFFF)) & ~0xFFFF, F32)
    xs = x_sel.astype(BF16)
    gt = _rnd(jnp.dot(xs, wg_v[...], preferred_element_type=F32))
    gt = _rnd(gt * jax.nn.sigmoid(gt))
    up = _rnd(jnp.dot(xs, wu_v[...], preferred_element_type=F32))
    gu = (gt * up).astype(BF16)
    gate_r = jnp.concatenate([_rnd(jax.nn.sigmoid(r_sel))] * pl.cdiv(d, LANES), axis=1)

    def down(fs):
        y = _rnd(jnp.dot(gu, pltpu.bitcast(wd_scr[:, fs], BF16), preferred_element_type=F32))
        y = _rnd(y * gate_r[:, fs])
        return x1_sel[:, fs] + _rnd(row_scr[3, :, fs] * _rnd(x_sel[:, fs] + y))

    def patch(fs, new):
        n = fs.stop - fs.start
        lane_d = jax.lax.broadcasted_iota(I32, (n // 2, LANES), 1)
        for c in range(TOPC):
            ln = idxs[c] & (LANES - 1)
            wide = jnp.broadcast_to(new[c:c + 1], (LANES, n)).astype(BF16).T
            moved = pltpu.bitcast(wide, I32)
            cur = pltpu.bitcast(out_v[fs, bcols[c]], I32)
            out_v[fs, bcols[c]] = pltpu.bitcast(jnp.where(lane_d == ln, moved, cur), BF16)

            @pl.when(final[c])
            def _(c=c):
                out_start(fs, bcols[c])

    pch = [slice(a, b) for a, b in zip((0,) + cuts, cuts + (d,))]
    new_scr[:, pch[0]] = down(pch[0])
    for j in range(len(pch)):
        @pl.when(z_scr[0, 0] == 0)
        def _(j=j):
            prev = new_scr[:, pch[j]]
            if j + 1 < len(pch):
                new_scr[:, pch[j + 1]] = down(pch[j + 1])
            patch(pch[j], prev)

    pltpu.make_async_copy(out_v, out_hbm, sem.at[1]).wait()


def _build(ahead=384, ahp=320, kcp=256, oh=144, lw=32, dt=80, dl=320, rc2=16,
          marg=128, sub=64, cuts=(256, 512), mrows=64, dtm=150, cw=256, lt0=40, lsp=28,
          lst=150, lxp=230, lsc=56, cdl=600):
    @jax.jit
    def pallas_adaLN_cond__gqa_block_cached__moe_arch_mod__prompt_kernel(
            A_x, A_k_cache, A_v_cache, A_wq, A_wo, B_x, B_w_r, B_w_gate, B_w_up, B_w_down, c, w_mod):
        b, s_len, d = A_x.shape
        assert b == 1
        hkv, sk = A_k_cache.shape[1], A_k_cache.shape[2]
        rep = HQ // hkv
        f = B_w_gate.shape[1]
        tg = GW // rep
        scratch = [
            pltpu.VMEM((1, d, s_len), BF16),
            pltpu.VMEM((2, sk, DH), BF16),
            pltpu.VMEM((2, sk, DH), BF16),
            pltpu.VMEM((2, d, rep * DH), BF16),
            pltpu.VMEM((2, d, rep * DH), BF16),
            pltpu.VMEM((d, rep * DH), BF16),
            pltpu.VMEM((s_len // tg, GW, DH), BF16),
            pltpu.VMEM((d,), BF16),
            pltpu.VMEM((1, d), BF16),
            pltpu.VMEM((d, 6 * d), BF16),
            pltpu.VMEM((d, f), BF16),
            pltpu.VMEM((d, f), BF16),
            pltpu.VMEM((d, f), BF16),
            pltpu.VMEM((f // 2, d), I32),
            pltpu.VMEM((d, s_len), BF16),
            pltpu.VMEM((s_len // 2, d), I32),
            pltpu.VMEM((d, s_len), F32),
            pltpu.VMEM((5, 8, d), F32),
            pltpu.VMEM((5, d, LANES), F32),
            pltpu.VMEM((1, DH // 2, sk), I32),
            pltpu.VMEM((2 * d, s_len), BF16),
            pltpu.VMEM((s_len // LANES, LANES), F32),
            pltpu.VMEM((3, 8, s_len), F32),
            pltpu.VMEM((1, sk, GW), F32),
            pltpu.VMEM((1, sk, GW), F32),
            pltpu.SMEM((8, LANES), I32),
            pltpu.VMEM((8, LANES), I32),
            pltpu.VMEM((TOPC, d), F32),
            pltpu.VMEM((d, LANES), F32),
            pltpu.VMEM((8, 6 * d + (d // LANES + 1) * LANES), F32),
            pltpu.VMEM((s_len // NXC // 2, d), I32),
            pltpu.SemaphoreType.DMA((NXC + 4,)),
        ]
        out = pl.pallas_call(
            functools.partial(_kernel, n_groups=hkv, rep=rep, ahead=ahead,
                              ahp=ahp, kcp=kcp, oh=oh, lw=lw, dt=dt, dl=dl, rc2=rc2, marg=marg,
                              sub=sub, cuts=cuts, mrows=mrows, dtm=dtm, cw=cw, lt0=lt0, lsp=lsp,
                              lst=lst, lxp=lxp, lsc=lsc, cdl=cdl),
            in_specs=[pl.BlockSpec(memory_space=pl.ANY)] * 11,
            out_specs=pl.BlockSpec(memory_space=pl.ANY),
            out_shape=jax.ShapeDtypeStruct((d, s_len), BF16),
            scratch_shapes=scratch,
            compiler_params=pltpu.CompilerParams(vmem_limit_bytes=100 * 1024 * 1024),
        )(A_x.reshape(s_len, d).T, A_k_cache.reshape(hkv, sk, DH), A_v_cache.reshape(hkv, sk, DH),
          A_wq, A_wo.T, B_w_r, c, w_mod, B_w_gate, B_w_up, B_w_down.T)
        return out.T.reshape(b, s_len, d)
    return pallas_adaLN_cond__gqa_block_cached__moe_arch_mod__prompt_kernel


pallas_adaLN_cond__gqa_block_cached__moe_arch_mod__prompt_kernel = _build()
```

```python
import functools

import jax
import jax.numpy as jnp
import jax.experimental.pallas as pl
import jax.experimental.pallas.tpu as pltpu

HQ = 32
DH = 128
TOPC = 8
LN_EPS = 1.0013580322265625e-05
LOG2E = 1.4426950408889634
F32 = jnp.float32
BF16 = jnp.bfloat16
I32 = jnp.int32
NT = (((1,), (1,)), ((), ()))
LANES = 128
GW = 512
MXU_LAT = 128
NXC = 4


def _rnd(v):
    return v.astype(BF16).astype(F32)


def _by8(v):
    return v.reshape(v.shape[0] // 8, 8, v.shape[1])


class _Moments:
    def __init__(self):
        self.shift = self.s1 = self.s2 = None

    def add(self, v):
        if self.shift is None:
            self.shift = jnp.broadcast_to(v[0:1], (8, v.shape[1]))
        dv = _by8(v) - self.shift[None]
        a, b = jnp.sum(dv, axis=0), jnp.sum(dv * dv, axis=0)
        self.s1, self.s2 = (a, b) if self.s1 is None else (self.s1 + a, self.s2 + b)

    def stats(self, d):
        e1 = jnp.sum(self.s1, axis=0, keepdims=True) * (1.0 / d)
        e2 = jnp.sum(self.s2, axis=0, keepdims=True) * (1.0 / d)
        var = jnp.maximum(e2 - e1 * e1, 0.0)
        den = _rnd(jnp.sqrt(_rnd(_rnd(var) + LN_EPS)))
        return _rnd(self.shift + e1), jnp.broadcast_to(1.0 / den, self.shift.shape)


def _chain(*jobs):
    gate = yield
    for job in jobs:
        next(job)
        while True:
            try:
                v = job.send(gate)
            except StopIteration:
                break
            gate = yield v


def _mix(a, b, every):
    next(a)
    next(b)
    gate = yield
    n, live = 0, [a, b]
    while live:
        n += 1
        job = b if (b in live and (n % (every + 1) == 0 or a not in live)) else a
        try:
            v = job.send(gate)
        except StopIteration:
            live.remove(job)
            continue
        gate = yield v


def _finish(job):
    try:
        while True:
            job.send(lambda t: t)
    except StopIteration:
        pass


def _kernel(xt_hbm, k_hbm, v_hbm, wq_hbm, wot_hbm, wr_hbm, c_hbm, wmod_hbm,
            wg_hbm, wu_hbm, wdt_hbm,
            out_hbm,
            xt_v, kbuf, vbuf, wqbuf, wobuf, wql_v, q_scr,
            wr_v, c_v, wmod_v, wg_v, wu_v, wdt_v, wd_scr, out_v,
            h_scr, acc_scr, row_scr, col_scr, vt_scr, xh_scr, r_scr, st_scr, s0_scr, s1_scr,
            z_scr, zv_scr, new_scr, cc_scr, mod_scr, hn_scr, sem, *,
            n_groups, rep, ahead, ahp, kcp, oh, lw, dt, dl, rc2, marg, sub, cuts,
            mrows, dtm, cw, lt0, lsp, lst, lxp, lsc, cdl):
    _, d, s_len = xt_v.shape
    sk = kbuf.shape[1]
    gcols = rep * DH
    tg = GW // rep
    ng = s_len // tg
    nblk = s_len // LANES
    nlt = tg // LANES
    xw = s_len // NXC
    per = xw // tg
    lastg = n_groups - 1
    s_bufs = (s0_scr, s1_scr)
    cpad = (d // LANES + 1) * LANES
    assert d % LANES == LANES // 2 and n_groups >= 5 + 4 * d // (2 * LANES)
    qscale = (DH ** -0.5) * LOG2E

    def group_copies(g, slot):
        cols = pl.ds(pl.multiple_of(g * gcols, gcols), gcols)
        s = sem.at[NXC + 2 + slot]
        return (pltpu.make_async_copy(wq_hbm.at[:, cols], wqbuf.at[slot], s),
                pltpu.make_async_copy(k_hbm.at[g], kbuf.at[slot], s),
                pltpu.make_async_copy(v_hbm.at[g], vbuf.at[slot], s),
                pltpu.make_async_copy(wot_hbm.at[:, cols], wobuf.at[slot], s))

    def x_copy(j, s):
        cols = pl.ds(pl.multiple_of(j * xw, xw), xw)
        return pltpu.make_async_copy(xt_hbm.at[:, cols], xt_v.at[0, :, cols], sem.at[s])

    cp_z = pltpu.make_async_copy(zv_scr, z_scr, sem.at[0])
    cp_c = pltpu.make_async_copy(c_hbm, c_v, sem.at[0])
    cp_m0 = pltpu.make_async_copy(wmod_hbm.at[:, 0:2 * d], wmod_v.at[:, 0:2 * d], sem.at[1])
    cp_wql = pltpu.make_async_copy(wq_hbm.at[:, lastg * gcols:(lastg + 1) * gcols], wql_v,
                                   sem.at[2])
    cp_m1 = pltpu.make_async_copy(wmod_hbm.at[:, 2 * d:6 * d], wmod_v.at[:, 2 * d:6 * d], sem.at[2])
    cp_wr = pltpu.make_async_copy(wr_hbm, wr_v, sem.at[0])
    cp_tail = (pltpu.make_async_copy(wg_hbm, wg_v, sem.at[0]),
               pltpu.make_async_copy(wu_hbm, wu_v, sem.at[0]),
               pltpu.make_async_copy(wdt_hbm, wdt_v, sem.at[0]))

    def out_start(rows, cols):
        pltpu.make_async_copy(out_v.at[rows, cols], out_hbm.at[rows, cols], sem.at[1]).start()

    def silu_c():
        cf = c_v[...].astype(F32)
        return (cf * jax.nn.sigmoid(cf)).astype(BF16)

    def mod_job(g):
        gate = yield
        mw = 2 * LANES
        lo = jnp.where(g < 2, 0, 2 * d + mw * jnp.minimum(g - 2, 4 * d // mw - 1))
        cols = pl.ds(pl.multiple_of(lo, LANES), mw)
        acc = jnp.zeros((8, mw), F32)
        for r0 in range(0, d, mrows):
            cc = jnp.concatenate([cc_scr[r0:r0 + mrows, :]] * 2, axis=1)
            prod = _by8(wmod_v[r0:r0 + mrows, cols].astype(F32) * cc)
            acc = gate(acc) + jnp.sum(prod, axis=0)
            if r0 + mrows == d:
                mod_scr[:, cols] = jnp.broadcast_to(jnp.sum(acc, axis=0, keepdims=True), (8, mw))
            gate = yield acc

    def col_job(j):
        gate = yield
        lo = pl.multiple_of((2 + j) * d // LANES * LANES, LANES)
        w = _rnd(gate(mod_scr[:, pl.ds(lo, cpad)]))
        row = jnp.where((2 + j) * d == lo, w[:, 0:d], w[:, cpad - d:cpad])
        row = jnp.where(j == 2, _rnd(1.0 + row), row)
        row_scr[j] = row
        col_scr[j] = to_col(row[0:1])
        gate = yield col_scr[0, 0:8, :], cdl

    def tspan(i, lo, n):
        if isinstance(i, int):
            return slice(i * tg + lo, i * tg + lo + n)
        return pl.ds(pl.multiple_of(i * tg + lo, n), n)

    def tcols(i):
        return tspan(i, 0, tg)

    def col(j, rows, tiles=nlt):
        return jnp.concatenate([col_scr[j, rows, :]] * tiles, axis=1)

    fch = [slice(lo, min(lo + LANES, d)) for lo in range(0, d, LANES)]

    def ln1_chunk(cols_of, mark=lambda v: None, stats=None):
        if stats is None:
            mo = _Moments()
            for r0 in range(0, d, 32):
                mo.add(xt_v[0, r0:r0 + 32, cols_of(0, xw)].astype(F32))
                mark(mo.s2)
            stats = mo.stats(d)
            mark(stats[1])
        mean, rinv = stats
        for b in range(0, xw, cw):
            for rows in fch:
                wide = lambda j: jnp.concatenate([col_scr[j, rows, :]] * (cw // LANES), axis=1)
                x = _by8(xt_v[z_scr[0, 0], rows, cols_of(b, cw)].astype(F32))
                y = ((x - mean[None, :, b:b + cw]) * rinv[None, :, b:b + cw]).reshape(-1, cw)
                h32 = pltpu.bitcast((y * wide(1) + wide(0)).astype(BF16).T, I32)
                hn_scr[b // 2:(b + cw) // 2, rows] = h32
                mark(h32[cw // 2 - 8:cw // 2])

    def to_col(row):
        return jnp.broadcast_to(row, (LANES, d)).T

    def project_q(tok, wq_ref, step, tail_first):
        half, full = LANES // 2, d // LANES * LANES
        hs = [pltpu.bitcast(h_scr[(tok * nlt + lt) * half:(tok * nlt + lt + 1) * half, :], BF16)
              for lt in range(nlt)]
        if tail_first:
            tails = [jnp.dot(h[:, full:], wq_ref[full:, :], preferred_element_type=F32) for h in hs]
            step(tails[0], LANES)
        parts = []
        for lt, h in enumerate(hs):
            if tail_first:
                q = jnp.dot(h[:, :full], wq_ref[:full, :], preferred_element_type=F32) + tails[lt]
                step(q, full * rep // 4)
            else:
                q = jnp.dot(h, wq_ref[...], preferred_element_type=F32)
                step(q, LANES * pl.cdiv(d, LANES) * rep // 4)
            parts.append((q * qscale).astype(BF16))
        return jnp.concatenate([p[:, r * DH:(r + 1) * DH] for r in range(rep) for p in parts],
                               axis=0)

    def ln2_job(i, n=2, rc=rc2):
        gate = yield
        cols, tiles = tspan(i, 0, n * tg), n * nlt
        mo = _Moments()
        mo.shift, mo.s1, mo.s2 = (st_scr[j, :, cols] for j in range(3))
        mean, rinv = mo.stats(d)
        racc = None
        for r0 in range(0, d, rc):
            rows = slice(r0, r0 + rc)
            x1 = xh_scr[d + r0:d + r0 + rc, cols].astype(F32)
            xc = (_by8(x1) - gate(mean)[None]).reshape(x1.shape)
            y = _rnd((_by8(_rnd(xc)) * rinv[None]).reshape(x1.shape))
            h2b = (_rnd(y * col(2, rows, tiles)) + col(1, rows, tiles)).astype(BF16)
            h2 = h2b.astype(F32)
            xh_scr[rows, cols] = h2b
            out_v[rows, cols] = (x1 + col(3, rows, tiles) * h2).astype(BF16)
            part = jnp.sum(_by8(h2 * col(4, rows, tiles)), axis=0)
            racc = part if racc is None else racc + part
            if r0 + rc == d:
                r = jnp.sum(racc, axis=0, keepdims=True)
                for lt in range(tiles):
                    r_scr[pl.ds(i * nlt + lt, 1), :] = r[:, lt * LANES:(lt + 1) * LANES]
            gate = yield racc

    def wd_job(t, parts):
        gate = yield
        fw = wdt_v.shape[1] // parts
        for f0 in range(0, fw, LANES):
            lo = pl.multiple_of(t * fw + f0, LANES)
            w32 = pltpu.bitcast(wdt_v[:, pl.ds(lo, LANES)], I32)
            w32 = gate(_by8(w32)).reshape(w32.shape)
            wd = pltpu.bitcast(w32, BF16).T
            half = pl.multiple_of(t * (fw // 2) + f0 // 2, LANES // 2)
            wd_scr[pl.ds(half, LANES // 2), :] = pltpu.bitcast(wd, I32)
            gate = yield wd_scr[0:8, 0:LANES]

    def attention(slot, toks, sched, last=False, job=None, hook=None, dt=dt):
        wq_ref, k_ref, v_ref, wot_ref = (wqbuf.at[slot], kbuf.at[slot], vbuf.at[slot],
                                         wobuf.at[slot])
        zero = z_scr[0, 0]
        zvec = jnp.full((8, LANES), zero, I32)
        st = dict(clock=0, nxt=0, job=job)
        hist = []
        due = []
        if job is not None:
            next(job)

        def token(when):
            want = when - MXU_LAT
            for start, dur, res in reversed(hist):
                if start <= want:
                    row = min((want - start) * res.shape[0] // dur // 8 * 8, res.shape[0] - 8)
                    return pltpu.bitcast(res[row:row + 8, 0:LANES], I32) & zvec
            return None

        def tie(x, tok):
            if tok is None:
                return x
            if x.shape[-1] > LANES:
                tok = jnp.concatenate([tok] * (x.shape[-1] // LANES), axis=1)
            if x.ndim == 3:
                tok = tok[None]
            if x.dtype == I32:
                return x | tok
            return pltpu.bitcast(pltpu.bitcast(x, I32) | tok, x.dtype)

        def tie_due(x, now):
            while due and due[0][0] <= now:
                v = due.pop(0)[1]
                v = v if v.dtype == I32 else pltpu.bitcast(v, I32)
                bits = v[:, 0:LANES]
                for j in range(1, v.shape[1] // LANES):
                    bits = bits | v[:, j * LANES:(j + 1) * LANES]
                x = tie(x, bits & zvec)
            return x

        def side(upto):
            while st['job'] is not None and st['nxt'] <= upto:
                tok = token(st['nxt'] + MXU_LAT)
                try:
                    v = st['job'].send(lambda x, tok=tok: tie(x, tok))
                except StopIteration:
                    st['job'] = None
                    break
                v, extra = v if isinstance(v, tuple) else (v, 0)
                due.append((st['nxt'] + dl + extra, v))
                due.sort(key=lambda e: e[0])
                st['nxt'] += dt

        def step(result, dur, advance=None):
            hist.append((st['clock'], dur, result))
            st['clock'] += dur if advance is None else advance

        def scores(qg, buf, rows, cols, advance=None):
            s = jax.lax.dot_general(k_ref[rows, :], qg[cols], NT, preferred_element_type=F32)
            s_bufs[buf][zero, rows, cols] = s
            step(s, s.shape[0], advance)
            return s

        def max_fin(m):
            return jnp.broadcast_to(jnp.max(m, axis=0, keepdims=True), m.shape)

        def qk(qg, buf):
            m = None
            st['nxt'] = max(st['nxt'], st['clock'])
            stop = st['clock'] + sk - marg
            for j in range(4):
                t0 = st['clock']
                s = scores(qg, buf, slice(j * sk // 4, (j + 1) * sk // 4), slice(0, GW))
                blk = s.shape[0] if job is None else sub
                for r0 in range(0, s.shape[0], blk):
                    mj = jnp.max(_by8(s[r0:r0 + blk]), axis=0)
                    if m is not None:
                        m0 = tie_due(m[:, 0:LANES], t0 + r0)
                        mj = jnp.maximum(jnp.concatenate([m0, m[:, LANES:]], axis=1), mj)
                    m = mj
                    side(min(t0 + r0 + blk - 1, stop))
            return max_fin(m)

        def pv_unit(buf, m, u, kc, advance, lead):
            cs = slice(u * LANES, (u + 1) * LANES)
            o = l = None
            for j in range(sk // kc):
                when = st['clock'] - lead
                mu = tie_due(tie(m[:, cs], token(when)), when)
                p = jnp.exp2(_by8(s_bufs[buf][0, j * kc:(j + 1) * kc, cs]) - mu[None])
                lj = jnp.sum(p.reshape(kc // lw, lw, LANES), axis=0)
                oj = jnp.dot(pltpu.bitcast(vt_scr[0, :, j * kc:(j + 1) * kc], BF16),
                             p.reshape(kc, LANES).astype(BF16), preferred_element_type=F32)
                o = oj if o is None else o + oj
                l = lj if l is None else l + lj
                step(oj, DH, advance)
            return (o / jnp.sum(l, axis=0, keepdims=True)).astype(BF16)

        def heads_major(outs):
            return jnp.concatenate(
                [jnp.concatenate(outs[r * nlt:(r + 1) * nlt], axis=1) for r in range(rep)], axis=0)

        def pv(buf, m):
            return heads_major([pv_unit(buf, m, u, kcp, kcp // 4, ahp) for u in range(4)])

        def pv_qk(buf, m, qn, nbuf):
            outs, mns = [], []
            for half in range(2):
                s = scores(qn, nbuf, slice(0, sk), slice(half * GW // 2, (half + 1) * GW // 2), 0)
                mns.append(jnp.max(_by8(s), axis=0))
                outs += [pv_unit(buf, m, u, 2 * LANES, DH, ahead) for u in (2 * half, 2 * half + 1)]
            return heads_major(outs), max_fin(jnp.concatenate(mns, axis=1))

        def oproj(tok, ot):
            cols = tcols(tok)
            mo = _Moments()
            for r0 in range(0, d, oh):
                rows = slice(r0, r0 + oh)
                res = jnp.dot(wot_ref[rows, :], ot, preferred_element_type=F32)
                attn = res + acc_scr[rows, cols]
                if last:
                    x1b = (xt_v[0, rows, cols].astype(F32) + col(0, rows) * attn).astype(BF16)
                    xh_scr[d + r0:d + r0 + oh, cols] = x1b
                    mo.add(x1b.astype(F32))
                else:
                    acc_scr[rows, cols] = attn
                step(res, oh)
            if last:
                for j, v in enumerate((mo.shift, mo.s1, mo.s2)):
                    st_scr[j, :, cols] = v

        qs, ots, ms, bufs, free = {}, {}, {}, {}, [0, 1]
        for item in sched.split():
            kind, i = item[0], int(item[1:] or 0)
            if kind == '!':
                hook()
            elif kind == 'V':
                vt_scr[zero] = pltpu.bitcast(v_ref[...].T, I32)
            elif kind == 'Q':
                qs[i] = project_q(toks[i], wq_ref, step, i == 0)
            elif kind == 'L':
                qs[i] = q_scr[toks[i]]
            elif kind == 'K':
                bufs[i] = free.pop(0)
                ms[i] = qk(qs[i], bufs[i])
            elif kind == 'P':
                ots[i] = pv(bufs[i], ms[i])
                free.append(bufs[i])
            elif kind == 'S':
                bufs[i + 1] = free.pop(0)
                ots[i], ms[i + 1] = pv_qk(bufs[i], ms[i], qs[i + 1], bufs[i + 1])
                free.append(bufs[i])
            elif kind == 'O':
                oproj(toks[i], ots[i])
        if st['job'] is not None:
            _finish(st['job'])

    zv_scr[...] = jnp.zeros(zv_scr.shape, I32)
    for cp in ((cp_z, cp_c, cp_wr, x_copy(0, 0), cp_m0, cp_wql)
               + tuple(x_copy(j, j + 2) for j in range(1, NXC)) + group_copies(0, 0)):
        cp.start()

    def zero_body(j, carry):
        rows = pl.ds(pl.multiple_of(j * 32, 32), 32)
        acc_scr[rows, :] = jnp.zeros((32, s_len), F32)
        xh_scr[pl.ds(pl.multiple_of(d + j * 32, 32), 32), s_len - 2 * tg:s_len] = (
            jnp.zeros((32, 2 * tg), BF16))
        return carry

    jax.lax.fori_loop(0, d // 32, zero_body, 0)
    st_scr[:, :, s_len - 2 * tg:s_len] = jnp.zeros((3, 8, 2 * tg), F32)
    mod_scr[...] = jnp.zeros(mod_scr.shape, F32)
    cp_z.wait()
    cp_c.wait()
    cp_wr.wait()
    x_copy(0, 0).wait()

    mo0 = _Moments()
    for r0 in range(0, d, 32):
        mo0.add(xt_v[0, r0:r0 + 32, 0:xw].astype(F32))
    stats0 = mo0.stats(d)
    cc_scr[...] = to_col(silu_c()).astype(F32)
    mod_scr[:, 6 * d:7 * d] = jnp.broadcast_to(wr_v[...].astype(F32).reshape(1, d), (8, d))
    cp_m0.wait()
    mod = _rnd(jnp.dot(jnp.broadcast_to(silu_c(), (8, d)), wmod_v[:, 0:2 * d],
                       preferred_element_type=F32))
    col_scr[z_scr[0, 0]] = to_col(mod[0:1, 0:d])
    col_scr[z_scr[0, 0] + 1] = to_col(_rnd(1.0 + mod[0:1, d:2 * d]))
    ln1_chunk(lambda lo, n: slice(lo, lo + n), stats=stats0)
    cp_wql.wait()

    def ln1_body(j, carry):
        src = jnp.minimum(j + 1, NXC - 1)

        @pl.when(j + 1 < NXC)
        def _():
            x_copy(src, src + 2).wait()

        zvec = jnp.full((8, LANES), z_scr[0, 0], I32)
        nb = xw // LANES
        half = LANES // 2
        lhs = [hn_scr[b * half:(b + 1) * half, :] for b in range(nb)]
        for b in range(nb):
            h_scr[pl.ds(pl.multiple_of(j * (xw // 2) + b * half, half), half), :] = lhs[b]
        marks = []
        ln1_chunk(lambda lo, n: pl.ds(pl.multiple_of(src * xw + lo, n), n), marks.append)
        na = d // 32
        times = ([lt0 + lsp * i for i in range(na)] + [lt0 + lsp * na + lst]
                 + [lt0 + lsp * na + lst + lxp + lsc * i for i in range(len(marks) - na - 1)])
        dur = LANES * len(fch) * rep // 4
        ties = {}
        for t, v in zip(times, marks):
            b, off = t // dur, t % dur
            if off >= 2 * LANES:
                b, off = b + 1, 0
            if b < nb:
                v = v if v.dtype == I32 else pltpu.bitcast(v, I32)
                bits = v[:, 0:LANES] if v.shape[1] >= LANES else jnp.concatenate([v, v], axis=1)
                for c0 in range(LANES, v.shape[1], LANES):
                    bits = bits | v[:, c0:c0 + LANES]
                where = (b, off % LANES // 16, 0 if off < LANES else len(fch) - 1)
                ties[where] = bits if where not in ties else ties[where] | bits
        for b in range(nb):
            grid = [[lhs[b][r * 8:(r + 1) * 8, fs] for fs in fch] for r in range(half // 8)]
            for (bb, r, k), bits in ties.items():
                if bb == b:
                    grid[r][k] = grid[r][k] | (bits & zvec)[:, 0:grid[r][k].shape[1]]
            hb = jnp.concatenate([jnp.concatenate(row, axis=1) for row in grid], axis=0)
            q = jnp.dot(pltpu.bitcast(hb, BF16), wql_v[...], preferred_element_type=F32)
            q = (q * qscale).astype(BF16)
            for r in range(rep):
                lo = r * tg + (b % nlt) * LANES
                q_scr[j * per + b // nlt, lo:lo + LANES, :] = q[:, r * DH:(r + 1) * DH]
        return carry

    jax.lax.fori_loop(0, NXC, ln1_body, 0)

    steady = 'V Q0 Q1 K0 ! ' + ' '.join(
        ('O%d ' % (i - 2) if i >= 2 else '') + ('Q%d ' % (i + 2) if i + 2 < ng else '')
        + ('S%d' % i if i + 1 < ng else 'P%d' % i) for i in range(ng)
    ) + ' O%d O%d' % (ng - 2, ng - 1)

    def group_body(g, carry):
        slot = g & 1
        for cp in group_copies(g, slot):
            cp.wait()

        @pl.when(g == 2)
        def _():
            cp_m1.wait()

        def prefetch():
            for cp in group_copies(g + 1, 1 - slot):
                cp.start()
            for j, cp in enumerate((cp_m1,) + cp_tail):
                @pl.when(g == j)
                def _(cp=cp):
                    cp.start()

        attention(slot, list(range(ng)), steady, hook=prefetch, dt=dtm,
                  job=_chain(col_job(jnp.clip(g - (lastg - 5), 0, 4)), mod_job(g)))
        return carry

    jax.lax.fori_loop(0, lastg, group_body, 0)

    for cp in group_copies(lastg, lastg % 2) + cp_tail:
        cp.wait()
    npair = ng // 2

    def last_body(t, carry):
        prev = (t + npair - 1) % npair
        attention(lastg % 2, [2 * t, 2 * t + 1], 'V L0 L1 K0 K1 P0 P1 O0 O1', last=True,
                  job=_mix(ln2_job(2 * prev), wd_job(t, npair), 4))
        return carry

    jax.lax.fori_loop(0, npair, last_body, 0)
    rest = ln2_job(ng - 2)
    next(rest)
    _finish(rest)

    ibits = (s_len - 1).bit_length()
    imask = (1 << ibits) - 1
    bits = pltpu.bitcast(_rnd(r_scr[...]), I32)
    pos = (jax.lax.broadcasted_iota(I32, bits.shape, 0) * LANES
           + jax.lax.broadcasted_iota(I32, bits.shape, 1))
    order = ((bits ^ ((bits >> 31) & 0x7FFFFFFF)) >> 16) + 0x8000
    key = pltpu.bitcast((order << ibits) + (imask - pos) + 0x20000000, F32)
    subl = jax.lax.broadcasted_iota(I32, (TOPC, LANES), 0)
    lane = jax.lax.broadcasted_iota(I32, (TOPC, LANES), 1)
    subd = jax.lax.broadcasted_iota(I32, (TOPC, d), 0)
    idxs, blks, bcols = [], [], []
    keyv = jnp.zeros((TOPC, LANES), I32)
    x_sel = jnp.zeros((TOPC, d), F32)
    x1_sel = jnp.zeros((TOPC, d), F32)
    for c in range(TOPC):
        top = jnp.max(jnp.max(key, axis=0, keepdims=True), axis=1, keepdims=True)
        key = jnp.where(key == top, 0.0, key)
        topi = pltpu.bitcast(jnp.broadcast_to(top, (TOPC, LANES)), I32)
        keyv = jnp.where(subl == c, topi, keyv)
        ixv = imask - (topi & imask)
        idxs.append(ixv[0, 0])
        blks.append(jnp.clip(idxs[c] >> (LANES.bit_length() - 1), 0, nblk - 1))
        bcols.append(pl.ds(pl.multiple_of(blks[c] * LANES, LANES), LANES))
        pick = jnp.where(lane == (ixv & (LANES - 1)), 1.0, 0.0).astype(BF16)
        take = lambda rows: jax.lax.dot_general(pick, xh_scr[rows, bcols[c]], NT,
                                                preferred_element_type=F32)
        x_sel = jnp.where(subd == c, take(slice(0, d)), x_sel)
        x1_sel = jnp.where(subd == c, take(slice(d, 2 * d)), x1_sel)

    for b in range(nblk):
        hit = blks[0] == b
        for bb in blks[1:]:
            hit = jnp.logical_or(hit, bb == b)

        @pl.when(jnp.logical_not(hit))
        def _(b=b):
            out_start(slice(0, d), slice(b * LANES, (b + 1) * LANES))

    final = []
    for c in range(TOPC):
        u = True
        for other in blks[c + 1:]:
            u = jnp.logical_and(u, other != blks[c])
        final.append(jnp.asarray(u))

    ob = (((keyv - 0x20000000) >> ibits) - 0x8000) << 16
    r_sel = pltpu.bitcast((ob ^ ((ob >> 31) & 0x7FFFFFFF)) & ~0xFFFF, F32)
    xs = x_sel.astype(BF16)
    gt = _rnd(jnp.dot(xs, wg_v[...], preferred_element_type=F32))
    gt = _rnd(gt * jax.nn.sigmoid(gt))
    up = _rnd(jnp.dot(xs, wu_v[...], preferred_element_type=F32))
    gu = (gt * up).astype(BF16)
    gate_r = jnp.concatenate([_rnd(jax.nn.sigmoid(r_sel))] * pl.cdiv(d, LANES), axis=1)

    def down(fs):
        y = _rnd(jnp.dot(gu, pltpu.bitcast(wd_scr[:, fs], BF16), preferred_element_type=F32))
        y = _rnd(y * gate_r[:, fs])
        return x1_sel[:, fs] + _rnd(row_scr[3, :, fs] * _rnd(x_sel[:, fs] + y))

    def patch(fs, new):
        n = fs.stop - fs.start
        lane_d = jax.lax.broadcasted_iota(I32, (n // 2, LANES), 1)
        for c in range(TOPC):
            ln = idxs[c] & (LANES - 1)
            wide = jnp.broadcast_to(new[c:c + 1], (LANES, n)).astype(BF16).T
            moved = pltpu.bitcast(wide, I32)
            cur = pltpu.bitcast(out_v[fs, bcols[c]], I32)
            out_v[fs, bcols[c]] = pltpu.bitcast(jnp.where(lane_d == ln, moved, cur), BF16)

            @pl.when(final[c])
            def _(c=c):
                out_start(fs, bcols[c])

    pch = [slice(a, b) for a, b in zip((0,) + cuts, cuts + (d,))]
    new_scr[:, pch[0]] = down(pch[0])
    for j in range(len(pch)):
        @pl.when(z_scr[0, 0] == 0)
        def _(j=j):
            prev = new_scr[:, pch[j]]
            if j + 1 < len(pch):
                new_scr[:, pch[j + 1]] = down(pch[j + 1])
            patch(pch[j], prev)

    pltpu.make_async_copy(out_v, out_hbm, sem.at[1]).wait()


def _build(ahead=384, ahp=280, kcp=256, oh=144, lw=32, dt=80, dl=320, rc2=16,
          marg=128, sub=64, cuts=(256, 512), mrows=64, dtm=150, cw=256, lt0=40, lsp=28,
          lst=150, lxp=230, lsc=56, cdl=600):
    @jax.jit
    def pallas_adaLN_cond__gqa_block_cached__moe_arch_mod__prompt_kernel(
            A_x, A_k_cache, A_v_cache, A_wq, A_wo, B_x, B_w_r, B_w_gate, B_w_up, B_w_down, c, w_mod):
        b, s_len, d = A_x.shape
        assert b == 1
        hkv, sk = A_k_cache.shape[1], A_k_cache.shape[2]
        rep = HQ // hkv
        f = B_w_gate.shape[1]
        tg = GW // rep
        scratch = [
            pltpu.VMEM((1, d, s_len), BF16),
            pltpu.VMEM((2, sk, DH), BF16),
            pltpu.VMEM((2, sk, DH), BF16),
            pltpu.VMEM((2, d, rep * DH), BF16),
            pltpu.VMEM((2, d, rep * DH), BF16),
            pltpu.VMEM((d, rep * DH), BF16),
            pltpu.VMEM((s_len // tg, GW, DH), BF16),
            pltpu.VMEM((d,), BF16),
            pltpu.VMEM((1, d), BF16),
            pltpu.VMEM((d, 6 * d), BF16),
            pltpu.VMEM((d, f), BF16),
            pltpu.VMEM((d, f), BF16),
            pltpu.VMEM((d, f), BF16),
            pltpu.VMEM((f // 2, d), I32),
            pltpu.VMEM((d, s_len), BF16),
            pltpu.VMEM((s_len // 2, d), I32),
            pltpu.VMEM((d, s_len), F32),
            pltpu.VMEM((5, 8, d), F32),
            pltpu.VMEM((5, d, LANES), F32),
            pltpu.VMEM((1, DH // 2, sk), I32),
            pltpu.VMEM((2 * d, s_len), BF16),
            pltpu.VMEM((s_len // LANES, LANES), F32),
            pltpu.VMEM((3, 8, s_len), F32),
            pltpu.VMEM((1, sk, GW), F32),
            pltpu.VMEM((1, sk, GW), F32),
            pltpu.SMEM((8, LANES), I32),
            pltpu.VMEM((8, LANES), I32),
            pltpu.VMEM((TOPC, d), F32),
            pltpu.VMEM((d, LANES), F32),
            pltpu.VMEM((8, 6 * d + (d // LANES + 1) * LANES), F32),
            pltpu.VMEM((s_len // NXC // 2, d), I32),
            pltpu.SemaphoreType.DMA((NXC + 4,)),
        ]
        out = pl.pallas_call(
            functools.partial(_kernel, n_groups=hkv, rep=rep, ahead=ahead,
                              ahp=ahp, kcp=kcp, oh=oh, lw=lw, dt=dt, dl=dl, rc2=rc2, marg=marg,
                              sub=sub, cuts=cuts, mrows=mrows, dtm=dtm, cw=cw, lt0=lt0, lsp=lsp,
                              lst=lst, lxp=lxp, lsc=lsc, cdl=cdl),
            in_specs=[pl.BlockSpec(memory_space=pl.ANY)] * 11,
            out_specs=pl.BlockSpec(memory_space=pl.ANY),
            out_shape=jax.ShapeDtypeStruct((d, s_len), BF16),
            scratch_shapes=scratch,
            compiler_params=pltpu.CompilerParams(vmem_limit_bytes=100 * 1024 * 1024),
        )(A_x.reshape(s_len, d).T, A_k_cache.reshape(hkv, sk, DH), A_v_cache.reshape(hkv, sk, DH),
          A_wq, A_wo.T, B_w_r, c, w_mod, B_w_gate, B_w_up, B_w_down.T)
        return out.T.reshape(b, s_len, d)
    return pallas_adaLN_cond__gqa_block_cached__moe_arch_mod__prompt_kernel


pallas_adaLN_cond__gqa_block_cached__moe_arch_mod__prompt_kernel = _build()
```

```python
import functools

import jax
import jax.numpy as jnp
import jax.experimental.pallas as pl
import jax.experimental.pallas.tpu as pltpu

HQ = 32
DH = 128
TOPC = 8
LN_EPS = 1.0013580322265625e-05
LOG2E = 1.4426950408889634
F32 = jnp.float32
BF16 = jnp.bfloat16
I32 = jnp.int32
NT = (((1,), (1,)), ((), ()))
LANES = 128
GW = 512
MXU_LAT = 128
NXC = 4


def _rnd(v):
    return v.astype(BF16).astype(F32)


def _by8(v):
    return v.reshape(v.shape[0] // 8, 8, v.shape[1])


class _Moments:
    def __init__(self):
        self.shift = self.s1 = self.s2 = None

    def add(self, v):
        if self.shift is None:
            self.shift = jnp.broadcast_to(v[0:1], (8, v.shape[1]))
        dv = _by8(v) - self.shift[None]
        a, b = jnp.sum(dv, axis=0), jnp.sum(dv * dv, axis=0)
        self.s1, self.s2 = (a, b) if self.s1 is None else (self.s1 + a, self.s2 + b)

    def stats(self, d):
        e1 = jnp.sum(self.s1, axis=0, keepdims=True) * (1.0 / d)
        e2 = jnp.sum(self.s2, axis=0, keepdims=True) * (1.0 / d)
        var = jnp.maximum(e2 - e1 * e1, 0.0)
        den = _rnd(jnp.sqrt(_rnd(_rnd(var) + LN_EPS)))
        return _rnd(self.shift + e1), jnp.broadcast_to(1.0 / den, self.shift.shape)


def _chain(*jobs):
    gate = yield
    for job in jobs:
        next(job)
        while True:
            try:
                v = job.send(gate)
            except StopIteration:
                break
            gate = yield v


def _mix(a, b, every):
    next(a)
    next(b)
    gate = yield
    n, live = 0, [a, b]
    while live:
        n += 1
        job = b if (b in live and (n % (every + 1) == 0 or a not in live)) else a
        try:
            v = job.send(gate)
        except StopIteration:
            live.remove(job)
            continue
        gate = yield v


def _finish(job):
    try:
        while True:
            job.send(lambda t: t)
    except StopIteration:
        pass


def _kernel(xt_hbm, k_hbm, v_hbm, wq_hbm, wot_hbm, wr_hbm, c_hbm, wmod_hbm,
            wg_hbm, wu_hbm, wdt_hbm,
            out_hbm,
            xt_v, kbuf, vbuf, wqbuf, wobuf, wql_v, q_scr,
            wr_v, c_v, wmod_v, wg_v, wu_v, wd_scr, out_v,
            h_scr, acc_scr, row_scr, col_scr, vt_scr, xh_scr, r_scr, st_scr, s0_scr, s1_scr,
            z_scr, zv_scr, new_scr, cc_scr, mod_scr, hn_scr, sem, *,
            n_groups, rep, ahead, ahp, kcp, oh, lw, dt, dl, rc2, marg, sub, cuts,
            mrows, dtm, cw, lt0, lsp, lst, lxp, lsc, cdl, wdl):
    _, d, s_len = xt_v.shape
    sk = kbuf.shape[1]
    gcols = rep * DH
    tg = GW // rep
    ng = s_len // tg
    nblk = s_len // LANES
    nlt = tg // LANES
    xw = s_len // NXC
    per = xw // tg
    lastg = n_groups - 1
    f = wg_v.shape[1]
    fw = 2 * wd_scr.shape[0] - f
    assert f % fw == 0 and f // fw <= n_groups - 3
    s_bufs = (s0_scr, s1_scr)
    cpad = (d // LANES + 1) * LANES
    assert d % LANES == LANES // 2 and n_groups >= 5 + 4 * d // (2 * LANES)
    qscale = (DH ** -0.5) * LOG2E

    def group_copies(g, slot):
        cols = pl.ds(pl.multiple_of(g * gcols, gcols), gcols)
        s = sem.at[NXC + 2 + slot]
        return (pltpu.make_async_copy(wq_hbm.at[:, cols], wqbuf.at[slot], s),
                pltpu.make_async_copy(k_hbm.at[g], kbuf.at[slot], s),
                pltpu.make_async_copy(v_hbm.at[g], vbuf.at[slot], s),
                pltpu.make_async_copy(wot_hbm.at[:, cols], wobuf.at[slot], s))

    def x_copy(j, s):
        cols = pl.ds(pl.multiple_of(j * xw, xw), xw)
        return pltpu.make_async_copy(xt_hbm.at[:, cols], xt_v.at[0, :, cols], sem.at[s])

    cp_z = pltpu.make_async_copy(zv_scr, z_scr, sem.at[0])
    cp_c = pltpu.make_async_copy(c_hbm, c_v, sem.at[0])
    cp_m0 = pltpu.make_async_copy(wmod_hbm.at[:, 0:2 * d], wmod_v.at[:, 0:2 * d], sem.at[1])
    cp_wql = pltpu.make_async_copy(wq_hbm.at[:, lastg * gcols:(lastg + 1) * gcols], wql_v,
                                   sem.at[2])
    cp_side = (pltpu.make_async_copy(wmod_hbm.at[:, 2 * d:6 * d], wmod_v.at[:, 2 * d:6 * d],
                                     sem.at[2]),
               pltpu.make_async_copy(wdt_hbm, wmod_v.at[:, 6 * d:6 * d + f], sem.at[2]))
    cp_wr = pltpu.make_async_copy(wr_hbm, wr_v, sem.at[0])
    cp_tail = (pltpu.make_async_copy(wg_hbm, wg_v, sem.at[0]),
               pltpu.make_async_copy(wu_hbm, wu_v, sem.at[0]))

    def out_start(rows, cols):
        pltpu.make_async_copy(out_v.at[rows, cols], out_hbm.at[rows, cols], sem.at[1]).start()

    def silu_c():
        cf = c_v[...].astype(F32)
        return (cf * jax.nn.sigmoid(cf)).astype(BF16)

    def mod_job(g):
        gate = yield
        mw = 2 * LANES
        lo = jnp.where(g < 2, 0, 2 * d + mw * jnp.minimum(g - 2, 4 * d // mw - 1))
        cols = pl.ds(pl.multiple_of(lo, LANES), mw)
        acc = jnp.zeros((8, mw), F32)
        for r0 in range(0, d, mrows):
            cc = jnp.concatenate([cc_scr[r0:r0 + mrows, :]] * 2, axis=1)
            prod = _by8(wmod_v[r0:r0 + mrows, cols].astype(F32) * cc)
            acc = gate(acc) + jnp.sum(prod, axis=0)
            if r0 + mrows == d:
                mod_scr[:, cols] = jnp.broadcast_to(jnp.sum(acc, axis=0, keepdims=True), (8, mw))
            gate = yield acc

    def col_job(j):
        gate = yield
        lo = pl.multiple_of((2 + j) * d // LANES * LANES, LANES)
        w = _rnd(gate(mod_scr[:, pl.ds(lo, cpad)]))
        row = jnp.where((2 + j) * d == lo, w[:, 0:d], w[:, cpad - d:cpad])
        row = jnp.where(j == 2, _rnd(1.0 + row), row)
        row_scr[j] = row
        col_scr[j] = to_col(row[0:1])
        gate = yield col_scr[0, 0:8, :], cdl

    def tspan(i, lo, n):
        if isinstance(i, int):
            return slice(i * tg + lo, i * tg + lo + n)
        return pl.ds(pl.multiple_of(i * tg + lo, n), n)

    def tcols(i):
        return tspan(i, 0, tg)

    def col(j, rows, tiles=nlt):
        return jnp.concatenate([col_scr[j, rows, :]] * tiles, axis=1)

    fch = [slice(lo, min(lo + LANES, d)) for lo in range(0, d, LANES)]

    def ln1_chunk(cols_of, mark=lambda v: None, stats=None):
        if stats is None:
            mo = _Moments()
            for r0 in range(0, d, 32):
                mo.add(xt_v[0, r0:r0 + 32, cols_of(0, xw)].astype(F32))
                mark(mo.s2)
            stats = mo.stats(d)
            mark(stats[1])
        mean, rinv = stats
        for b in range(0, xw, cw):
            for rows in fch:
                wide = lambda j: jnp.concatenate([col_scr[j, rows, :]] * (cw // LANES), axis=1)
                x = _by8(xt_v[z_scr[0, 0], rows, cols_of(b, cw)].astype(F32))
                y = ((x - mean[None, :, b:b + cw]) * rinv[None, :, b:b + cw]).reshape(-1, cw)
                h32 = pltpu.bitcast((y * wide(1) + wide(0)).astype(BF16).T, I32)
                hn_scr[b // 2:(b + cw) // 2, rows] = h32
                mark(h32[cw // 2 - 8:cw // 2])

    def to_col(row):
        return jnp.broadcast_to(row, (LANES, d)).T

    def project_q(tok, wq_ref, step, tail_first):
        half, full = LANES // 2, d // LANES * LANES
        hs = [pltpu.bitcast(h_scr[(tok * nlt + lt) * half:(tok * nlt + lt + 1) * half, :], BF16)
              for lt in range(nlt)]
        if tail_first:
            tails = [jnp.dot(h[:, full:], wq_ref[full:, :], preferred_element_type=F32) for h in hs]
            step(tails[0], LANES)
        parts = []
        for lt, h in enumerate(hs):
            if tail_first:
                q = jnp.dot(h[:, :full], wq_ref[:full, :], preferred_element_type=F32) + tails[lt]
                step(q, full * rep // 4)
            else:
                q = jnp.dot(h, wq_ref[...], preferred_element_type=F32)
                step(q, LANES * pl.cdiv(d, LANES) * rep // 4)
            parts.append((q * qscale).astype(BF16))
        return jnp.concatenate([p[:, r * DH:(r + 1) * DH] for r in range(rep) for p in parts],
                               axis=0)

    def ln2_job(i, n=2, rc=rc2):
        gate = yield
        cols, tiles = tspan(i, 0, n * tg), n * nlt
        mo = _Moments()
        mo.shift, mo.s1, mo.s2 = (st_scr[j, :, cols] for j in range(3))
        mean, rinv = mo.stats(d)
        racc = None
        for r0 in range(0, d, rc):
            rows = slice(r0, r0 + rc)
            x1 = xh_scr[d + r0:d + r0 + rc, cols].astype(F32)
            xc = (_by8(x1) - gate(mean)[None]).reshape(x1.shape)
            y = _rnd((_by8(_rnd(xc)) * rinv[None]).reshape(x1.shape))
            h2b = (_rnd(y * col(2, rows, tiles)) + col(1, rows, tiles)).astype(BF16)
            h2 = h2b.astype(F32)
            xh_scr[rows, cols] = h2b
            out_v[rows, cols] = (x1 + col(3, rows, tiles) * h2).astype(BF16)
            part = jnp.sum(_by8(h2 * col(4, rows, tiles)), axis=0)
            racc = part if racc is None else racc + part
            if r0 + rc == d:
                r = jnp.sum(racc, axis=0, keepdims=True)
                for lt in range(tiles):
                    r_scr[pl.ds(i * nlt + lt, 1), :] = r[:, lt * LANES:(lt + 1) * LANES]
            gate = yield racc

    def wd_job(g):
        gate = yield
        part = jnp.minimum(g - 2, f // fw - 1)
        src = jnp.where(g < 2, 0, 6 * d + part * fw)
        dst = jnp.where(g < 2, f // 2, part * (fw // 2))
        for f0 in range(0, fw, LANES):
            w32 = pltpu.bitcast(wmod_v[:, pl.ds(pl.multiple_of(src + f0, LANES), LANES)], I32)
            w32 = gate(_by8(w32)).reshape(w32.shape)
            wd = pltpu.bitcast(w32, BF16).T
            rows = pl.ds(pl.multiple_of(dst + f0 // 2, LANES // 2), LANES // 2)
            wd_scr[rows, :] = pltpu.bitcast(wd, I32)
            gate = yield wd_scr[f // 2:f // 2 + 8, 0:LANES], wdl

    def attention(slot, toks, sched, last=False, job=None, hook=None, dt=dt):
        wq_ref, k_ref, v_ref, wot_ref = (wqbuf.at[slot], kbuf.at[slot], vbuf.at[slot],
                                         wobuf.at[slot])
        zero = z_scr[0, 0]
        zvec = jnp.full((8, LANES), zero, I32)
        st = dict(clock=0, nxt=0, job=job)
        hist = []
        due = []
        if job is not None:
            next(job)

        def token(when):
            want = when - MXU_LAT
            for start, dur, res in reversed(hist):
                if start <= want:
                    row = min((want - start) * res.shape[0] // dur // 8 * 8, res.shape[0] - 8)
                    return pltpu.bitcast(res[row:row + 8, 0:LANES], I32) & zvec
            return None

        def tie(x, tok):
            if tok is None:
                return x
            if x.shape[-1] > LANES:
                tok = jnp.concatenate([tok] * (x.shape[-1] // LANES), axis=1)
            if x.ndim == 3:
                tok = tok[None]
            if x.dtype == I32:
                return x | tok
            return pltpu.bitcast(pltpu.bitcast(x, I32) | tok, x.dtype)

        def tie_due(x, now):
            while due and due[0][0] <= now:
                v = due.pop(0)[1]
                v = v if v.dtype == I32 else pltpu.bitcast(v, I32)
                bits = v[:, 0:LANES]
                for j in range(1, v.shape[1] // LANES):
                    bits = bits | v[:, j * LANES:(j + 1) * LANES]
                x = tie(x, bits & zvec)
            return x

        def side(upto):
            while st['job'] is not None and st['nxt'] <= upto:
                tok = token(st['nxt'] + MXU_LAT)
                try:
                    v = st['job'].send(lambda x, tok=tok: tie(x, tok))
                except StopIteration:
                    st['job'] = None
                    break
                v, extra = v if isinstance(v, tuple) else (v, 0)
                due.append((st['nxt'] + dl + extra, v))
                due.sort(key=lambda e: e[0])
                st['nxt'] += dt

        def step(result, dur, advance=None):
            hist.append((st['clock'], dur, result))
            st['clock'] += dur if advance is None else advance

        def scores(qg, buf, rows, cols, advance=None):
            s = jax.lax.dot_general(k_ref[rows, :], qg[cols], NT, preferred_element_type=F32)
            s_bufs[buf][zero, rows, cols] = s
            step(s, s.shape[0], advance)
            return s

        def max_fin(m):
            return jnp.broadcast_to(jnp.max(m, axis=0, keepdims=True), m.shape)

        def qk(qg, buf):
            m = None
            st['nxt'] = max(st['nxt'], st['clock'])
            stop = st['clock'] + sk - marg
            for j in range(4):
                t0 = st['clock']
                s = scores(qg, buf, slice(j * sk // 4, (j + 1) * sk // 4), slice(0, GW))
                blk = s.shape[0] if job is None else sub
                for r0 in range(0, s.shape[0], blk):
                    mj = jnp.max(_by8(s[r0:r0 + blk]), axis=0)
                    if m is not None:
                        m0 = tie_due(m[:, 0:LANES], t0 + r0)
                        mj = jnp.maximum(jnp.concatenate([m0, m[:, LANES:]], axis=1), mj)
                    m = mj
                    side(min(t0 + r0 + blk - 1, stop))
            return max_fin(m)

        def pv_unit(buf, m, u, kc, advance, lead):
            cs = slice(u * LANES, (u + 1) * LANES)
            o = l = None
            for j in range(sk // kc):
                when = st['clock'] - lead
                mu = tie_due(tie(m[:, cs], token(when)), when)
                p = jnp.exp2(_by8(s_bufs[buf][0, j * kc:(j + 1) * kc, cs]) - mu[None])
                lj = jnp.sum(p.reshape(kc // lw, lw, LANES), axis=0)
                oj = jnp.dot(pltpu.bitcast(vt_scr[0, :, j * kc:(j + 1) * kc], BF16),
                             p.reshape(kc, LANES).astype(BF16), preferred_element_type=F32)
                o = oj if o is None else o + oj
                l = lj if l is None else l + lj
                step(oj, DH, advance)
            return (o / jnp.sum(l, axis=0, keepdims=True)).astype(BF16)

        def heads_major(outs):
            return jnp.concatenate(
                [jnp.concatenate(outs[r * nlt:(r + 1) * nlt], axis=1) for r in range(rep)], axis=0)

        def pv(buf, m):
            return heads_major([pv_unit(buf, m, u, kcp, kcp // 4, ahp) for u in range(4)])

        def pv_qk(buf, m, qn, nbuf):
            outs, mns = [], []
            for half in range(2):
                s = scores(qn, nbuf, slice(0, sk), slice(half * GW // 2, (half + 1) * GW // 2), 0)
                mns.append(jnp.max(_by8(s), axis=0))
                outs += [pv_unit(buf, m, u, 2 * LANES, DH, ahead) for u in (2 * half, 2 * half + 1)]
            return heads_major(outs), max_fin(jnp.concatenate(mns, axis=1))

        def oproj(tok, ot):
            cols = tcols(tok)
            mo = _Moments()
            for r0 in range(0, d, oh):
                rows = slice(r0, r0 + oh)
                res = jnp.dot(wot_ref[rows, :], ot, preferred_element_type=F32)
                attn = res + acc_scr[rows, cols]
                if last:
                    x1b = (xt_v[0, rows, cols].astype(F32) + col(0, rows) * attn).astype(BF16)
                    xh_scr[d + r0:d + r0 + oh, cols] = x1b
                    mo.add(x1b.astype(F32))
                else:
                    acc_scr[rows, cols] = attn
                step(res, oh)
            if last:
                for j, v in enumerate((mo.shift, mo.s1, mo.s2)):
                    st_scr[j, :, cols] = v

        qs, ots, ms, bufs, free = {}, {}, {}, {}, [0, 1]
        for item in sched.split():
            kind, i = item[0], int(item[1:] or 0)
            if kind == '!':
                hook()
            elif kind == 'V':
                vt_scr[zero] = pltpu.bitcast(v_ref[...].T, I32)
            elif kind == 'Q':
                qs[i] = project_q(toks[i], wq_ref, step, i == 0)
            elif kind == 'L':
                qs[i] = q_scr[toks[i]]
            elif kind == 'K':
                bufs[i] = free.pop(0)
                ms[i] = qk(qs[i], bufs[i])
            elif kind == 'P':
                ots[i] = pv(bufs[i], ms[i])
                free.append(bufs[i])
            elif kind == 'S':
                bufs[i + 1] = free.pop(0)
                ots[i], ms[i + 1] = pv_qk(bufs[i], ms[i], qs[i + 1], bufs[i + 1])
                free.append(bufs[i])
            elif kind == 'O':
                oproj(toks[i], ots[i])
        if st['job'] is not None:
            _finish(st['job'])

    zv_scr[...] = jnp.zeros(zv_scr.shape, I32)
    for cp in ((cp_z, cp_c, cp_wr, x_copy(0, 0), cp_m0, cp_wql)
               + tuple(x_copy(j, j + 2) for j in range(1, NXC)) + group_copies(0, 0)):
        cp.start()

    def zero_body(j, carry):
        rows = pl.ds(pl.multiple_of(j * 32, 32), 32)
        acc_scr[rows, :] = jnp.zeros((32, s_len), F32)
        xh_scr[pl.ds(pl.multiple_of(d + j * 32, 32), 32), s_len - 2 * tg:s_len] = (
            jnp.zeros((32, 2 * tg), BF16))
        return carry

    jax.lax.fori_loop(0, d // 32, zero_body, 0)
    st_scr[:, :, s_len - 2 * tg:s_len] = jnp.zeros((3, 8, 2 * tg), F32)
    mod_scr[...] = jnp.zeros(mod_scr.shape, F32)
    cp_z.wait()
    cp_c.wait()
    cp_wr.wait()
    x_copy(0, 0).wait()

    mo0 = _Moments()
    for r0 in range(0, d, 32):
        mo0.add(xt_v[0, r0:r0 + 32, 0:xw].astype(F32))
    stats0 = mo0.stats(d)
    cc_scr[...] = to_col(silu_c()).astype(F32)
    mod_scr[:, 6 * d:7 * d] = jnp.broadcast_to(wr_v[...].astype(F32).reshape(1, d), (8, d))
    cp_m0.wait()
    mod = _rnd(jnp.dot(jnp.broadcast_to(silu_c(), (8, d)), wmod_v[:, 0:2 * d],
                       preferred_element_type=F32))
    col_scr[z_scr[0, 0]] = to_col(mod[0:1, 0:d])
    col_scr[z_scr[0, 0] + 1] = to_col(_rnd(1.0 + mod[0:1, d:2 * d]))
    ln1_chunk(lambda lo, n: slice(lo, lo + n), stats=stats0)
    cp_wql.wait()

    def ln1_body(j, carry):
        src = jnp.minimum(j + 1, NXC - 1)

        @pl.when(j + 1 < NXC)
        def _():
            x_copy(src, src + 2).wait()

        zvec = jnp.full((8, LANES), z_scr[0, 0], I32)
        nb = xw // LANES
        half = LANES // 2
        lhs = [hn_scr[b * half:(b + 1) * half, :] for b in range(nb)]
        for b in range(nb):
            h_scr[pl.ds(pl.multiple_of(j * (xw // 2) + b * half, half), half), :] = lhs[b]
        marks = []
        ln1_chunk(lambda lo, n: pl.ds(pl.multiple_of(src * xw + lo, n), n), marks.append)
        na = d // 32
        times = ([lt0 + lsp * i for i in range(na)] + [lt0 + lsp * na + lst]
                 + [lt0 + lsp * na + lst + lxp + lsc * i for i in range(len(marks) - na - 1)])
        dur = LANES * len(fch) * rep // 4
        ties = {}
        for t, v in zip(times, marks):
            b, off = t // dur, t % dur
            if off >= 2 * LANES:
                b, off = b + 1, 0
            if b < nb:
                v = v if v.dtype == I32 else pltpu.bitcast(v, I32)
                bits = v[:, 0:LANES] if v.shape[1] >= LANES else jnp.concatenate([v, v], axis=1)
                for c0 in range(LANES, v.shape[1], LANES):
                    bits = bits | v[:, c0:c0 + LANES]
                where = (b, off % LANES // 16, 0 if off < LANES else len(fch) - 1)
                ties[where] = bits if where not in ties else ties[where] | bits
        for b in range(nb):
            grid = [[lhs[b][r * 8:(r + 1) * 8, fs] for fs in fch] for r in range(half // 8)]
            for (bb, r, k), bits in ties.items():
                if bb == b:
                    grid[r][k] = grid[r][k] | (bits & zvec)[:, 0:grid[r][k].shape[1]]
            hb = jnp.concatenate([jnp.concatenate(row, axis=1) for row in grid], axis=0)
            q = jnp.dot(pltpu.bitcast(hb, BF16), wql_v[...], preferred_element_type=F32)
            q = (q * qscale).astype(BF16)
            for r in range(rep):
                lo = r * tg + (b % nlt) * LANES
                q_scr[j * per + b // nlt, lo:lo + LANES, :] = q[:, r * DH:(r + 1) * DH]
        return carry

    jax.lax.fori_loop(0, NXC, ln1_body, 0)

    steady = 'V Q0 Q1 K0 ! ' + ' '.join(
        ('O%d ' % (i - 2) if i >= 2 else '') + ('Q%d ' % (i + 2) if i + 2 < ng else '')
        + ('S%d' % i if i + 1 < ng else 'P%d' % i) for i in range(ng)
    ) + ' O%d O%d' % (ng - 2, ng - 1)

    def group_body(g, carry):
        slot = g & 1
        for cp in group_copies(g, slot):
            cp.wait()

        @pl.when(g == 2)
        def _():
            for cp in cp_side:
                cp.wait()

        def prefetch():
            for cp in group_copies(g + 1, 1 - slot):
                cp.start()
            for j, cp in zip((0, 0, 2, 3), cp_side + cp_tail):
                @pl.when(g == j)
                def _(cp=cp):
                    cp.start()

        attention(slot, list(range(ng)), steady, hook=prefetch, dt=dtm,
                  job=_chain(col_job(jnp.clip(g - (lastg - 5), 0, 4)), _mix(mod_job(g), wd_job(g), 2)))
        return carry

    jax.lax.fori_loop(0, lastg, group_body, 0)

    for cp in group_copies(lastg, lastg % 2) + cp_tail:
        cp.wait()
    npair = ng // 2

    def last_body(t, carry):
        prev = (t + npair - 1) % npair
        attention(lastg % 2, [2 * t, 2 * t + 1], 'V L0 L1 K0 K1 P0 P1 O0 O1', last=True,
                  job=ln2_job(2 * prev))
        return carry

    jax.lax.fori_loop(0, npair, last_body, 0)
    rest = ln2_job(ng - 2)
    next(rest)
    _finish(rest)

    ibits = (s_len - 1).bit_length()
    imask = (1 << ibits) - 1
    bits = pltpu.bitcast(_rnd(r_scr[...]), I32)
    pos = (jax.lax.broadcasted_iota(I32, bits.shape, 0) * LANES
           + jax.lax.broadcasted_iota(I32, bits.shape, 1))
    order = ((bits ^ ((bits >> 31) & 0x7FFFFFFF)) >> 16) + 0x8000
    key = pltpu.bitcast((order << ibits) + (imask - pos) + 0x20000000, F32)
    subl = jax.lax.broadcasted_iota(I32, (TOPC, LANES), 0)
    lane = jax.lax.broadcasted_iota(I32, (TOPC, LANES), 1)
    subd = jax.lax.broadcasted_iota(I32, (TOPC, d), 0)
    idxs, blks, bcols = [], [], []
    keyv = jnp.zeros((TOPC, LANES), I32)
    x_sel = jnp.zeros((TOPC, d), F32)
    x1_sel = jnp.zeros((TOPC, d), F32)
    for c in range(TOPC):
        top = jnp.max(jnp.max(key, axis=0, keepdims=True), axis=1, keepdims=True)
        key = jnp.where(key == top, 0.0, key)
        topi = pltpu.bitcast(jnp.broadcast_to(top, (TOPC, LANES)), I32)
        keyv = jnp.where(subl == c, topi, keyv)
        ixv = imask - (topi & imask)
        idxs.append(ixv[0, 0])
        blks.append(jnp.clip(idxs[c] >> (LANES.bit_length() - 1), 0, nblk - 1))
        bcols.append(pl.ds(pl.multiple_of(blks[c] * LANES, LANES), LANES))
        pick = jnp.where(lane == (ixv & (LANES - 1)), 1.0, 0.0).astype(BF16)
        take = lambda rows: jax.lax.dot_general(pick, xh_scr[rows, bcols[c]], NT,
                                                preferred_element_type=F32)
        x_sel = jnp.where(subd == c, take(slice(0, d)), x_sel)
        x1_sel = jnp.where(subd == c, take(slice(d, 2 * d)), x1_sel)

    for b in range(nblk):
        hit = blks[0] == b
        for bb in blks[1:]:
            hit = jnp.logical_or(hit, bb == b)

        @pl.when(jnp.logical_not(hit))
        def _(b=b):
            out_start(slice(0, d), slice(b * LANES, (b + 1) * LANES))

    final = []
    for c in range(TOPC):
        u = True
        for other in blks[c + 1:]:
            u = jnp.logical_and(u, other != blks[c])
        final.append(jnp.asarray(u))

    ob = (((keyv - 0x20000000) >> ibits) - 0x8000) << 16
    r_sel = pltpu.bitcast((ob ^ ((ob >> 31) & 0x7FFFFFFF)) & ~0xFFFF, F32)
    xs = x_sel.astype(BF16)
    gt = _rnd(jnp.dot(xs, wg_v[...], preferred_element_type=F32))
    gt = _rnd(gt * jax.nn.sigmoid(gt))
    up = _rnd(jnp.dot(xs, wu_v[...], preferred_element_type=F32))
    gu = (gt * up).astype(BF16)
    gate_r = jnp.concatenate([_rnd(jax.nn.sigmoid(r_sel))] * pl.cdiv(d, LANES), axis=1)

    def down(fs):
        y = _rnd(jnp.dot(gu, pltpu.bitcast(wd_scr[0:f // 2, fs], BF16), preferred_element_type=F32))
        y = _rnd(y * gate_r[:, fs])
        return x1_sel[:, fs] + _rnd(row_scr[3, :, fs] * _rnd(x_sel[:, fs] + y))

    def patch(fs, new):
        n = fs.stop - fs.start
        lane_d = jax.lax.broadcasted_iota(I32, (n // 2, LANES), 1)
        for c in range(TOPC):
            ln = idxs[c] & (LANES - 1)
            wide = jnp.broadcast_to(new[c:c + 1], (LANES, n)).astype(BF16).T
            moved = pltpu.bitcast(wide, I32)
            cur = pltpu.bitcast(out_v[fs, bcols[c]], I32)
            out_v[fs, bcols[c]] = pltpu.bitcast(jnp.where(lane_d == ln, moved, cur), BF16)

            @pl.when(final[c])
            def _(c=c):
                out_start(fs, bcols[c])

    pch = [slice(a, b) for a, b in zip((0,) + cuts, cuts + (d,))]
    new_scr[:, pch[0]] = down(pch[0])
    for j in range(len(pch)):
        @pl.when(z_scr[0, 0] == 0)
        def _(j=j):
            prev = new_scr[:, pch[j]]
            if j + 1 < len(pch):
                new_scr[:, pch[j + 1]] = down(pch[j + 1])
            patch(pch[j], prev)

    pltpu.make_async_copy(out_v, out_hbm, sem.at[1]).wait()


def _build(ahead=384, ahp=280, kcp=256, oh=144, lw=32, dt=100, dl=320, rc2=16,
          marg=128, sub=64, cuts=(256, 512), mrows=64, dtm=120, cw=256, lt0=40, lsp=28,
          lst=150, lxp=230, lsc=56, cdl=600, wdl=100):
    @jax.jit
    def pallas_adaLN_cond__gqa_block_cached__moe_arch_mod__prompt_kernel(
            A_x, A_k_cache, A_v_cache, A_wq, A_wo, B_x, B_w_r, B_w_gate, B_w_up, B_w_down, c, w_mod):
        b, s_len, d = A_x.shape
        assert b == 1
        hkv, sk = A_k_cache.shape[1], A_k_cache.shape[2]
        rep = HQ // hkv
        f = B_w_gate.shape[1]
        tg = GW // rep
        fw = LANES * pl.cdiv(f // LANES, hkv - 4)
        scratch = [
            pltpu.VMEM((1, d, s_len), BF16),
            pltpu.VMEM((2, sk, DH), BF16),
            pltpu.VMEM((2, sk, DH), BF16),
            pltpu.VMEM((2, d, rep * DH), BF16),
            pltpu.VMEM((2, d, rep * DH), BF16),
            pltpu.VMEM((d, rep * DH), BF16),
            pltpu.VMEM((s_len // tg, GW, DH), BF16),
            pltpu.VMEM((d,), BF16),
            pltpu.VMEM((1, d), BF16),
            pltpu.VMEM((d, 6 * d + f), BF16),
            pltpu.VMEM((d, f), BF16),
            pltpu.VMEM((d, f), BF16),
            pltpu.VMEM(((f + fw) // 2, d), I32),
            pltpu.VMEM((d, s_len), BF16),
            pltpu.VMEM((s_len // 2, d), I32),
            pltpu.VMEM((d, s_len), F32),
            pltpu.VMEM((5, 8, d), F32),
            pltpu.VMEM((5, d, LANES), F32),
            pltpu.VMEM((1, DH // 2, sk), I32),
            pltpu.VMEM((2 * d, s_len), BF16),
            pltpu.VMEM((s_len // LANES, LANES), F32),
            pltpu.VMEM((3, 8, s_len), F32),
            pltpu.VMEM((1, sk, GW), F32),
            pltpu.VMEM((1, sk, GW), F32),
            pltpu.SMEM((8, LANES), I32),
            pltpu.VMEM((8, LANES), I32),
            pltpu.VMEM((TOPC, d), F32),
            pltpu.VMEM((d, LANES), F32),
            pltpu.VMEM((8, 6 * d + (d // LANES + 1) * LANES), F32),
            pltpu.VMEM((s_len // NXC // 2, d), I32),
            pltpu.SemaphoreType.DMA((NXC + 4,)),
        ]
        out = pl.pallas_call(
            functools.partial(_kernel, n_groups=hkv, rep=rep, ahead=ahead,
                              ahp=ahp, kcp=kcp, oh=oh, lw=lw, dt=dt, dl=dl, rc2=rc2, marg=marg,
                              sub=sub, cuts=cuts, mrows=mrows, dtm=dtm, cw=cw, lt0=lt0, lsp=lsp,
                              lst=lst, lxp=lxp, lsc=lsc, cdl=cdl, wdl=wdl),
            in_specs=[pl.BlockSpec(memory_space=pl.ANY)] * 11,
            out_specs=pl.BlockSpec(memory_space=pl.ANY),
            out_shape=jax.ShapeDtypeStruct((d, s_len), BF16),
            scratch_shapes=scratch,
            compiler_params=pltpu.CompilerParams(vmem_limit_bytes=100 * 1024 * 1024),
        )(A_x.reshape(s_len, d).T, A_k_cache.reshape(hkv, sk, DH), A_v_cache.reshape(hkv, sk, DH),
          A_wq, A_wo.T, B_w_r, c, w_mod, B_w_gate, B_w_up, B_w_down.T)
        return out.T.reshape(b, s_len, d)
    return pallas_adaLN_cond__gqa_block_cached__moe_arch_mod__prompt_kernel


pallas_adaLN_cond__gqa_block_cached__moe_arch_mod__prompt_kernel = _build()
```
